```python
import jax
import jax.numpy as jnp

def _softmax(x, axis=-1):
    return jax.nn.softmax(x, axis=axis)
def _gelu(x):
    return jax.nn.gelu(x, approximate=True)
def _silu(x):
    return jax.nn.silu(x)
def _sigmoid(x):
    return jax.nn.sigmoid(x)
def _layernorm(x, axis=-1, eps=1e-5):
    m = jnp.mean(x, axis=axis, keepdims=True)
    v = jnp.var(x, axis=axis, keepdims=True)
    return (x - m) / jnp.sqrt(v + eps)
def _scatter_add(tgt, idx, src, axis=0):
    return tgt.at[idx].add(src)
def _segment_sum(src, seg, n):
    return jax.ops.segment_sum(src, seg, n)
class _Rng:
    def __init__(self, key):
        self._k = key
    def _next(self):
        self._k, sub = jax.random.split(self._k)
        return sub
    def normal(self, shape):
        return jax.random.normal(self._next(), shape, dtype=jnp.bfloat16)
    def randint(self, lo, hi, shape):
        return jax.random.randint(self._next(), shape, lo, hi, dtype=jnp.int32)
    def uniform(self, shape, lo=0.0, hi=1.0):
        return jax.random.uniform(self._next(), shape, jnp.bfloat16, lo, hi)
    def permutation(self, n):
        return jax.random.permutation(self._next(), n)


kernel_name = 'gated_mix__ssm_conv_h3__compressed_kv_cla__prompt'

def setup_inputs():
    _rng = _Rng(jax.random.key(int.from_bytes(__import__("os").urandom(4), "little")))
    _w = (lambda a: (lambda t: t.astype(jnp.bfloat16) if jnp.issubdtype(t.dtype, jnp.floating) else t)(jnp.asarray(a)))
    def _A_setup():
        B, S, D = 1, 2048, 1024
        ks = 4
        return {
            "q": _w((lambda *s: _rng.normal(s) * 0.05)(B, S, D)),
            "k": _w((lambda *s: _rng.normal(s) * 0.05)(B, S, D)),
            "v": _w((lambda *s: _rng.normal(s) * 0.05)(B, S, D)),
            "shift_k": _w((lambda *s: _rng.normal(s) * 0.05)(D, ks) * 0.5),
            "ssm_k": _w((lambda *s: _rng.normal(s) * 0.05)(D, S) * (1.0 / S ** 0.5)),
            "ssm_D": _w((lambda *s: _rng.normal(s) * 0.05)(D)),
        }
    _A_in = _A_setup()

    def _B_setup():
        B, H, Sq, Sk, D, M = 1, 32, 2048, 2048, 128, 1024
        Dc = 4 * D
        return {
            "x": _w((lambda *s: _rng.normal(s) * 0.05)(B, Sq, M)),
            "c_kv": _w((lambda *s: _rng.normal(s) * 0.05)(B, Sk, Dc)),
            "w_q": _w((lambda *s: _rng.normal(s) * 0.05)(M, H, D) * (M ** -0.5)),
            "w_uk": _w((lambda *s: _rng.normal(s) * 0.05)(Dc, H, D) * (Dc ** -0.5)),
            "w_uv": _w((lambda *s: _rng.normal(s) * 0.05)(Dc, H, D) * (Dc ** -0.5)),
            "w_o": _w((lambda *s: _rng.normal(s) * 0.05)(H, D, M) * ((H * D) ** -0.5)),
        }
    _B_in = _B_setup()

    return {
        "A_q": _A_in["q"],
        "A_k": _A_in["k"],
        "A_v": _A_in["v"],
        "A_shift_k": _A_in["shift_k"],
        "A_ssm_k": _A_in["ssm_k"],
        "A_ssm_D": _A_in["ssm_D"],
        "B_x": _B_in["x"],
        "B_c_kv": _B_in["c_kv"],
        "B_w_q": _B_in["w_q"],
        "B_w_uk": _B_in["w_uk"],
        "B_w_uv": _B_in["w_uv"],
        "B_w_o": _B_in["w_o"],
        "gate_w": _w((lambda *s: _rng.normal(s) * 0.05)(1024)),
    }

def reference(A_q, A_k, A_v, A_shift_k, A_ssm_k, A_ssm_D, B_x, B_c_kv, B_w_q, B_w_uk, B_w_uv, B_w_o, gate_w):
    def _A_ref(q, k, v, shift_k, ssm_k, ssm_D):
        B, S, D = q.shape
        ks = shift_k.shape[-1]
        k_pad = jnp.pad(k, ((0, 0), (ks - 1, 0), (0, 0)))
        k_shift = jnp.zeros_like(k)
        for t in range(ks):
            k_shift = k_shift + k_pad[:, t:t + S, :] * shift_k[:, ks - 1 - t][None, None, :]
        kv = k_shift * v
        L = 2 * S
        kv_pad = jnp.pad(kv, ((0, 0), (0, S), (0, 0)))
        kf_pad = jnp.pad(ssm_k, ((0, 0), (0, S)))
        kv_f = (lambda x, axes=(-2,-1): jnp.fft.rfft2(x.astype(jnp.float32), axes=axes))(kv_pad[:, None, :, :], axes=(1, 2))
        kf_f = (lambda x, axes=(-2,-1): jnp.fft.rfft2(x.astype(jnp.float32), axes=axes))(kf_pad[:, None, :], axes=(1, 2))
        kf_f = (lambda x, *d: x.transpose(*d))(kf_f, 1, 2, 0)
        y_f = kv_f * kf_f[None, :, :, :]
        y = (lambda x, s, axes=(-2,-1): jnp.fft.irfft2(x, s=s, axes=axes).astype(jnp.bfloat16))(y_f, (1, L), axes=(1, 2))[:, 0, :S, :]
        y = y + kv * ssm_D[None, None, :]
        return q * y

    def _B_ref(x, c_kv, w_q, w_uk, w_uv, w_o):
        B, Sq, M = x.shape[0], x.shape[1], x.shape[2]
        Sk = c_kv.shape[1]
        H, D = w_q.shape[1], w_q.shape[2]
        q = jnp.einsum("bqm,mhd->bhqd", x, w_q)
        k = jnp.einsum("bkc,chd->bhkd", c_kv, w_uk)
        v = jnp.einsum("bkc,chd->bhkd", c_kv, w_uv)
        scores = jnp.einsum("bhqd,bhkd->bhqk", q, k) * (D ** -0.5)
        off = Sk - Sq
        qi = jnp.arange(Sq)[:, None]
        kj = jnp.arange(Sk)[None, :]
        cmask = kj <= (qi + off)
        scores = jnp.where(cmask[None, None], scores, -1e9)
        p = _softmax(scores, axis=-1)
        ctx = jnp.einsum("bhqk,bhkd->bhqd", p, v)
        return jnp.einsum("bhqd,hdm->bqm", ctx, w_o)

    x = A_q
    g = _sigmoid((x * gate_w).sum(-1, keepdims=True))
    a = _A_ref(x, A_k, A_v, A_shift_k, A_ssm_k, A_ssm_D)
    b = _B_ref(x, B_c_kv, B_w_q, B_w_uk, B_w_uv, B_w_o)
    return g * a + (1 - g) * b
```

```python
import jax
import jax.numpy as jnp
import numpy as np
from jax import lax
import jax.experimental.pallas as pl
import jax.experimental.pallas.tpu as pltpu

S = 2048
DM = 1024
H = 32
DH = 128
DC = 512
T = 128
NB = S // T
KS = 4
PR = 1024

F32 = jnp.float32
BF16 = jnp.bfloat16
NT = (((1,), (1,)), ((), ()))


def _dft_matrices():
    ks = np.concatenate([np.arange(0, T, 2), np.arange(1, T, 2)]).reshape(NB, 8)
    n = np.arange(T)
    theta = 2.0 * np.pi * (ks[:, :, None] + 0.5) * n[None, None, :] / (2 * T)
    fwd = np.concatenate([np.cos(theta), -np.sin(theta)], axis=1).reshape(2 * T, T)
    inv = fwd.T / T
    return fwd.astype(np.float32), inv.astype(np.float32)


def _head_group_weights(raw_ref, g, rows):
    words = raw_ref.bitcast(jnp.uint32)
    win = words.at[pl.ds(pl.multiple_of(g * 4, 4), rows * (H // 2) - 12)]
    cols = []
    for b in range(4):
        w = win[pl.ds(b, rows, stride=H // 2), :]
        cols.append(pltpu.bitcast(w << 16, F32).astype(BF16))
        cols.append(pltpu.bitcast(w & jnp.uint32(0xFFFF0000), F32).astype(BF16))
    return jnp.concatenate(cols, axis=1)


def _project(src_ref, raw_ref, dst_ref, scale=None):
    rows = src_ref.shape[1]
    steps = S // PR

    def body(t, carry):
        g = t // steps
        r0 = pl.multiple_of((t % steps) * PR, PR)
        w = _head_group_weights(raw_ref, g, rows)
        y = jnp.dot(src_ref[pl.ds(r0, PR), :], w, preferred_element_type=F32)
        if scale is not None:
            y = y * scale
        y = y.astype(BF16)
        for j in range(8):
            dst_ref[g * 8 + j, pl.ds(r0, PR), :] = y[:, j * DH:(j + 1) * DH]
        return carry

    lax.fori_loop(0, (H // 8) * steps, body, 0)


def _attention_head(h, q_ref, k_ref, v_ref):
    row = lax.broadcasted_iota(jnp.int32, (T, T), 0)
    col = lax.broadcasted_iota(jnp.int32, (T, T), 1)
    causal = col <= row

    def scores(r):
        n = (r + 1) * T
        s = lax.dot_general(q_ref[h, r * T:n, :], k_ref[h, 0:n, :], NT,
                            preferred_element_type=F32)
        diag = jnp.where(causal, s[:, r * T:], -1e9)
        s = diag if r == 0 else jnp.concatenate([s[:, :r * T], diag], axis=1)
        return s, jnp.max(s, axis=1, keepdims=True)

    def context(r, s, m):
        n = (r + 1) * T
        p = jnp.exp2(s - m)
        l = jnp.sum(p, axis=1, keepdims=True)
        o = jnp.dot(p.astype(BF16), v_ref[h, 0:n, :], preferred_element_type=F32)
        q_ref[h, r * T:n, :] = (o * (1.0 / l)).astype(BF16)

    last = scores(NB - 1)
    prev = scores(0)
    for r in range(1, NB - 1):
        cur = scores(r)
        context(r - 1, *prev)
        prev = cur
    context(NB - 2, *prev)
    context(NB - 1, *last)


def _mix_tile(c, ctx_ref, wo_ref, x_ref, ak_ref, av_ref, hk_ref, shift_ref, skip_ref,
              gate_ref, fwd_ref, inv_ref, kpad_ref, u_ref, uf_ref, hf_ref, zf_ref,
              b_ref, out_ref):
    cols = pl.ds(pl.multiple_of(c * T, T), T)
    fwd = fwd_ref[...]

    kpad_ref[8:, :] = ak_ref[:, cols].astype(F32)
    taps = shift_ref[:, cols]
    for j in range(NB):
        ksh = kpad_ref[pl.ds(8 + j * T, T), :] * taps[0:1]
        for t in range(1, KS):
            ksh = ksh + kpad_ref[pl.ds(8 + j * T - t, T), :] * taps[t:t + 1]
        u = (ksh * av_ref[j * T:(j + 1) * T, cols].astype(F32)).astype(BF16)
        u_ref[j * T:(j + 1) * T, :] = u
        uf_ref[j] = jnp.dot(fwd, u, preferred_element_type=F32)

    before = None
    for d in range(NB):
        cur = lax.dot_general(fwd, hk_ref[cols, d * T:(d + 1) * T], NT,
                              preferred_element_type=F32)
        if before is None:
            hf_ref[d] = cur
        else:
            parts = []
            for f in range(NB):
                re, im = slice(16 * f, 16 * f + 8), slice(16 * f + 8, 16 * f + 16)
                if f < NB // 2:
                    parts += [cur[re] - before[im], cur[im] + before[re]]
                else:
                    parts += [cur[re] + before[im], cur[im] - before[re]]
            hf_ref[d] = jnp.concatenate(parts, axis=0)
        before = cur

    def spectrum_products(f):
        re, im = slice(16 * f, 16 * f + 8), slice(16 * f + 8, 16 * f + 16)
        for i0 in range(0, NB, 4):
            acc = {}
            for j0 in range(0, i0 + 4, 4):
                us = {j: (uf_ref[j, re, :], uf_ref[j, im, :]) for j in range(j0, j0 + 4)}
                lo = max(i0 - j0 - 3, 0)
                hs = {d: (hf_ref[d, re, :], hf_ref[d, im, :])
                      for d in range(lo, i0 - j0 + 4)}
                for i in range(i0, i0 + 4):
                    for j in range(j0, min(j0 + 4, i + 1)):
                        (ur, ui), (hr, hi) = us[j], hs[i - j]
                        zr, zi = ur * hr - ui * hi, ur * hi + ui * hr
                        acc[i] = (zr, zi) if i not in acc else (acc[i][0] + zr, acc[i][1] + zi)
            for i in range(i0, i0 + 4):
                zf_ref[i, 16 * f:16 * f + 16, :] = jnp.concatenate(acc[i], axis=0).astype(BF16)

    wo = wo_ref[:, cols]
    rows = 2 * T
    for r in range(S // rows):
        ctx = jnp.concatenate([ctx_ref[h, r * rows:(r + 1) * rows, :] for h in range(H)], axis=1)
        b_ref[r * rows:(r + 1) * rows, :] = jnp.dot(ctx, wo, preferred_element_type=F32)
        spectrum_products(2 * r)
        spectrum_products(2 * r + 1)

    inv = inv_ref[...]
    skip = skip_ref[:, cols]
    for i in range(NB):
        blk = slice(i * T, (i + 1) * T)
        y = jnp.dot(inv, zf_ref[i], preferred_element_type=F32)
        a = x_ref[blk, cols].astype(F32) * (y + u_ref[blk, :].astype(F32) * skip)
        g = gate_ref[blk, :]
        out_ref[blk, cols] = (g * a + (1.0 - g) * b_ref[blk, :]).astype(BF16)


def _kernel(x_hbm, ak_hbm, av_hbm, shift_in, hk_hbm, skip_in, c_hbm, wq_hbm, wuk_hbm,
            wuv_hbm, wo_hbm, gw_in, fwd_in, inv_in, out_hbm,
            x_ref, ak_ref, av_ref, hk_ref, c_ref, wq_ref, wuk_ref, wuv_ref, wo_ref,
            q_ref, k_ref, v_ref, gate_ref, shift_ref, skip_ref, fwd_ref, inv_ref,
            kpad_ref, u_ref, uf_ref, hf_ref, zf_ref, b_ref, out_ref, in_sem, out_sem):
    pairs = [(c_hbm, c_ref), (wuk_hbm, wuk_ref), (wuv_hbm, wuv_ref), (x_hbm, x_ref),
             (wq_hbm, wq_ref), (wo_hbm, wo_ref), (ak_hbm, ak_ref), (av_hbm, av_ref),
             (hk_hbm, hk_ref)]
    copies = [pltpu.make_async_copy(s, d, in_sem.at[i]) for i, (s, d) in enumerate(pairs)]
    cp_c, cp_wuk, cp_wuv, cp_x, cp_wq = copies[:5]

    cp_c.start()
    cp_wuk.start()
    shift_ref[...] = shift_in[...].astype(F32)
    skip_ref[...] = skip_in[...].astype(F32).reshape(1, DM)
    fwd_ref[...] = fwd_in[...].astype(BF16)
    inv_ref[...] = inv_in[...].astype(BF16)
    kpad_ref[0:8, :] = jnp.zeros((8, T), F32)
    cp_c.wait()
    cp_wuk.wait()
    cp_wuv.start()
    cp_x.start()
    cp_wq.start()
    _project(c_ref, wuk_ref, k_ref)
    cp_wuv.wait()
    cp_x.wait()
    cp_wq.wait()
    for cp in copies[5:]:
        cp.start()
    _project(c_ref, wuv_ref, v_ref)
    _project(x_ref, wq_ref, q_ref, scale=DH ** -0.5 * np.log2(np.e))

    gw = gw_in[...].astype(F32).reshape(1, DM)
    gr = S // H

    def head(h, carry):
        _attention_head(h, q_ref, k_ref, v_ref)
        rows = pl.ds(pl.multiple_of(h * gr, gr), gr)
        z = jnp.sum(x_ref[rows, :].astype(F32) * gw, axis=1, keepdims=True)
        gate_ref[rows, :] = jnp.broadcast_to(1.0 / (1.0 + jnp.exp(-z)), (gr, T))
        return carry

    lax.fori_loop(0, H, head, 0)

    for cp in copies[5:]:
        cp.wait()

    def out_copy(c):
        cols = pl.ds(pl.multiple_of(c * T, T), T)
        return pltpu.make_async_copy(out_ref.at[:, cols], out_hbm.at[:, cols], out_sem.at[c])

    def tile(c, carry):
        _mix_tile(c, q_ref, wo_ref, x_ref, ak_ref, av_ref, hk_ref, shift_ref, skip_ref,
                  gate_ref, fwd_ref, inv_ref, kpad_ref, u_ref, uf_ref, hf_ref, zf_ref,
                  b_ref, out_ref)
        out_copy(c).start()
        return carry

    lax.fori_loop(0, DM // T, tile, 0)
    for c in range(DM // T):
        out_copy(c).wait()


@jax.jit
def pallas_gated_mix__ssm_conv_h3__compressed_kv_cla__prompt_kernel(
    A_q: jax.Array,
    A_k: jax.Array,
    A_v: jax.Array,
    A_shift_k: jax.Array,
    A_ssm_k: jax.Array,
    A_ssm_D: jax.Array,
    B_x: jax.Array,
    B_c_kv: jax.Array,
    B_w_q: jax.Array,
    B_w_uk: jax.Array,
    B_w_uv: jax.Array,
    B_w_o: jax.Array,
    gate_w: jax.Array,
):
    del B_x
    fwd, inv = _dft_matrices()
    hbm = pl.BlockSpec(memory_space=pl.ANY)
    vmem = pl.BlockSpec(memory_space=pltpu.VMEM)
    out = pl.pallas_call(
        _kernel,
        out_shape=jax.ShapeDtypeStruct((S, DM), BF16),
        in_specs=[hbm, hbm, hbm, vmem, hbm, vmem, hbm, hbm, hbm, hbm, hbm, vmem, vmem, vmem],
        out_specs=hbm,
        scratch_shapes=[
            pltpu.VMEM((S, DM), BF16),
            pltpu.VMEM((S, DM), BF16),
            pltpu.VMEM((S, DM), BF16),
            pltpu.VMEM((DM, S), BF16),
            pltpu.VMEM((S, DC), BF16),
            pltpu.VMEM((DM * H, DH), BF16),
            pltpu.VMEM((DC * H, DH), BF16),
            pltpu.VMEM((DC * H, DH), BF16),
            pltpu.VMEM((H * DH, DM), BF16),
            pltpu.VMEM((H, S, DH), BF16),
            pltpu.VMEM((H, S, DH), BF16),
            pltpu.VMEM((H, S, DH), BF16),
            pltpu.VMEM((S, T), F32),
            pltpu.VMEM((KS, DM), F32),
            pltpu.VMEM((1, DM), F32),
            pltpu.VMEM((2 * T, T), BF16),
            pltpu.VMEM((T, 2 * T), BF16),
            pltpu.VMEM((8 + S, T), F32),
            pltpu.VMEM((S, T), BF16),
            pltpu.VMEM((NB, 2 * T, T), F32),
            pltpu.VMEM((NB, 2 * T, T), F32),
            pltpu.VMEM((NB, 2 * T, T), BF16),
            pltpu.VMEM((S, T), F32),
            pltpu.VMEM((S, DM), BF16),
            pltpu.SemaphoreType.DMA((9,)),
            pltpu.SemaphoreType.DMA((DM // T,)),
        ],
        compiler_params=pltpu.CompilerParams(vmem_limit_bytes=124 * 2**20),
    )(
        A_q.reshape(S, DM), A_k.reshape(S, DM), A_v.reshape(S, DM), A_shift_k.T,
        A_ssm_k, A_ssm_D, B_c_kv.reshape(S, DC), B_w_q.reshape(DM * H, DH),
        B_w_uk.reshape(DC * H, DH), B_w_uv.reshape(DC * H, DH),
        B_w_o.reshape(H * DH, DM), gate_w, fwd, inv,
    )
    return out.reshape(1, S, DM)
```

```python
import jax
import jax.numpy as jnp
import numpy as np
from jax import lax
import jax.experimental.pallas as pl
import jax.experimental.pallas.tpu as pltpu

S = 2048
DM = 1024
H = 32
DH = 128
DC = 512
T = 128
NB = S // T
NP = H // 2
KS = 4
CH = 4
W = T // 2

F32 = jnp.float32
BF16 = jnp.bfloat16
U32 = jnp.uint32
NT = (((1,), (1,)), ((), ()))


def _dft_matrices():
    ks = np.concatenate([np.arange(0, T, 2), np.arange(1, T, 2)]).reshape(NB, 8)
    n = np.arange(T)
    theta = 2.0 * np.pi * (ks[:, :, None] + 0.5) * n[None, None, :] / (2 * T)
    fwd = np.concatenate([np.cos(theta), -np.sin(theta)], axis=1).reshape(2 * T, T)
    inv = fwd.T / T
    return fwd.astype(np.float32), inv.astype(np.float32)


def _mm(a, b):
    return jnp.dot(a, b, preferred_element_type=F32)


def _pack(v):
    return pltpu.bitcast(v.astype(BF16), U32)


def _unpack(w):
    return pltpu.bitcast(w, BF16)


def _left(a11, a12, a21, a22):
    return [a11 + a22, a21 + a22, a11, a22, a11 + a12, a21 - a11, a12 - a22]


def _right(b11, b12, b21, b22):
    return [b11 + b22, b11, b12 - b22, b21 - b11, b22, b11 + b12, b21 + b22]


def _combine(m):
    return (m[0] + m[3] - m[4] + m[6], m[2] + m[4], m[1] + m[3], m[0] - m[1] + m[2] + m[5])


def _pair_weights(words):
    half = words.shape[0] // 2
    first = pltpu.bitcast(words << 16, F32)
    second = pltpu.bitcast(words & jnp.uint32(0xFFFF0000), F32)
    ops = _right(first[:half], second[:half], first[half:], second[half:])
    return [v.astype(BF16) for v in ops]


def _store_left(src_ref, dst_ref, e):
    half = src_ref.shape[1] // 2
    v = src_ref[pl.ds(pl.multiple_of(e * 2 * T, 2 * T), 2 * T), :].astype(F32)
    ops = _left(v[:T, :half], v[:T, half:], v[T:, :half], v[T:, half:])
    for i in range(7):
        dst_ref[i, pl.ds(pl.multiple_of(e * W, W), W), :] = _pack(ops[i])
    return v


def _project_kv(t, cs_ref, wkv_ref, kv_ref):
    base = pl.multiple_of((t >> 2) * S, S)
    for b in range(4):
        w = _pair_weights(wkv_ref[t * 4 + b])
        pair = (t & 3) * 4 + b
        for e in range(0, NB // 2, 2):
            c = _combine([_mm(_unpack(cs_ref[i, e * W:(e + 2) * W, :]), w[i]) for i in range(7)])
            for k in range(2):
                for odd in range(2):
                    for head in range(2):
                        r0 = head * (S // 2) + (2 * (e + k) + odd) * W
                        kv_ref[pair, pl.ds(base + r0, W), :] = _pack(
                            c[2 * odd + head][k * T:(k + 1) * T])


def _attend_pair(p, xs_ref, wq_ref, kv_ref):
    row = lax.broadcasted_iota(jnp.int32, (T, T), 0)
    col = lax.broadcasted_iota(jnp.int32, (T, T), 1)
    causal = col <= row
    scale = DH ** -0.5 * np.log2(np.e)
    w = _pair_weights(wq_ref[p])
    q, s, ctx = {}, {}, {}

    def chunks(r):
        return [(j, min(j + CH, r + 1)) for j in range(0, r + 1, CH)]

    def tiles(region, j0, j1):
        r0 = region * (S // 2)
        return _unpack(kv_ref[p, r0 + j0 * W:r0 + j1 * W, :])

    def queries(e):
        c = _combine([_mm(_unpack(xs_ref[i, e * W:(e + 1) * W, :]), w[i]) for i in range(7)])
        for odd in range(2):
            for head in range(2):
                q[2 * e + odd, head] = (c[2 * odd + head] * scale).astype(BF16)

    def scores(r, head):
        parts, m = [], None
        for j0, j1 in chunks(r):
            d = lax.dot_general(q[r, head], tiles(head, j0, j1), NT, preferred_element_type=F32)
            for j in range(j0, j1):
                t = d[:, (j - j0) * T:(j - j0 + 1) * T]
                if j == r:
                    t = jnp.where(causal, t, -1e9)
                parts.append(t)
                m = t if m is None else jnp.maximum(m, t)
        s[r, head] = parts, jnp.max(m, axis=1, keepdims=True)

    def context(r, head):
        parts, m = s.pop((r, head))
        l, o = None, None
        for j0, j1 in chunks(r):
            ps = [jnp.exp2(parts[j] - m) for j in range(j0, j1)]
            for e in ps:
                l = e if l is None else l + e
            e = ps[0] if len(ps) == 1 else jnp.concatenate(ps, axis=1)
            d = _mm(e.astype(BF16), tiles(2 + head, j0, j1))
            o = d if o is None else o + d
        l = jnp.sum(l, axis=1, keepdims=True)
        inv = pltpu.reciprocal(l, approx=True)
        inv = inv * (2.0 - l * inv)
        ctx[r, head] = o * inv

    def emit(e):
        ops = _left(*[ctx.pop((2 * e + odd, head)) for odd in range(2) for head in range(2)])
        for i in range(7):
            r0 = (i // 2) * (S // 2) + e * T + (i % 2) * W
            kv_ref[p, r0:r0 + W, :] = _pack(ops[i])

    todo = [(r, head) for r in range(NB - 1, -1, -1) for head in range(2)]
    next_q, next_s, lead = NB // 2 - 1, 0, 0
    for r, head in todo:
        while next_s < len(todo) and lead < LEAD + r + 1:
            rs, hs = todo[next_s]
            while next_q >= 0 and next_q >= rs // 2 - 1:
                queries(next_q)
                next_q -= 1
            scores(rs, hs)
            lead += rs + 1
            next_s += 1
        context(r, head)
        lead -= r + 1
        if head == 1 and r % 2 == 0:
            emit(r // 2)


LEAD = 12


def _mix_pair(c, kv_ref, wo_ref, x_ref, ak_ref, av_ref, hk_ref, shift_ref, skip_ref,
              gate_ref, fwd_ref, inv_ref, kpad_ref, uf_ref, hf_ref, out_ref):
    cols = [pl.ds(pl.multiple_of((2 * c + n) * T, T), T) for n in range(2)]
    fwd = fwd_ref[...]
    inv = inv_ref[...]
    for n in range(2):
        kpad_ref[n, 8:, :] = ak_ref[:, cols[n]].astype(F32)
    taps = [shift_ref[:, cols[n]] for n in range(2)]
    skip = [skip_ref[:, cols[n]] for n in range(2)]

    def heads(odd, n):
        return jnp.concatenate(
            [wo_ref[h * DH:(h + 1) * DH, cols[n]].astype(F32) for h in range(odd, H, 2)], axis=0)

    w = [v.astype(BF16) for v in _right(heads(0, 0), heads(0, 1), heads(1, 0), heads(1, 1))]
    before, u, a = {}, {}, {}

    def signal_spectrum(j, n):
        ksh = kpad_ref[n, pl.ds(8 + j * T, T), :] * taps[n][0:1]
        for t in range(1, KS):
            ksh = ksh + kpad_ref[n, pl.ds(8 + j * T - t, T), :] * taps[n][t:t + 1]
        u[j, n] = (ksh * av_ref[j * T:(j + 1) * T, cols[n]].astype(F32)).astype(BF16)
        uf_ref[n, j] = _mm(fwd, u[j, n])

    def filter_spectrum(d, n):
        cur = lax.dot_general(fwd, hk_ref[cols[n], d * T:(d + 1) * T], NT,
                              preferred_element_type=F32)
        for f in range(NB):
            re, im = slice(16 * f, 16 * f + 8), slice(16 * f + 8, 16 * f + 16)
            if d == 0:
                hr, hi = cur[re], cur[im]
            elif f < NB // 2:
                hr, hi = cur[re] - before[n][im], cur[im] + before[n][re]
            else:
                hr, hi = cur[re] + before[n][im], cur[im] - before[n][re]
            hf_ref[n, d, re, :] = hr
            hf_ref[n, d, im, :] = hi
        before[n] = cur

    def conv_block(i, n):
        z = []
        for f in range(NB):
            re, im = slice(16 * f, 16 * f + 8), slice(16 * f + 8, 16 * f + 16)
            zr, zi = None, None
            for j in range(i + 1):
                ur, ui = uf_ref[n, j, re, :], uf_ref[n, j, im, :]
                hr, hi = hf_ref[n, i - j, re, :], hf_ref[n, i - j, im, :]
                pr, pi = ur * hr - ui * hi, ur * hi + ui * hr
                zr, zi = (pr, pi) if zr is None else (zr + pr, zi + pi)
            z += [zr, zi]
        y = _mm(inv, jnp.concatenate(z, axis=0).astype(BF16))
        blk = slice(i * T, (i + 1) * T)
        a[i, n] = x_ref[blk, cols[n]].astype(F32) * (y + u.pop((i, n)).astype(F32) * skip[n])

    def product(e, i):
        r0 = (i // 2) * (S // 2) + e * T + (i % 2) * W
        left = jnp.concatenate([kv_ref[p, r0:r0 + W, :] for p in range(NP)], axis=1)
        return _mm(_unpack(left), w[i])

    for e in range(NB // 2):
        m = []
        for odd in range(2):
            for n in range(2):
                filter_spectrum(2 * e + odd, n)
                signal_spectrum(2 * e + odd, n)
            m.append(product(e, len(m)))
        m.append(product(e, 2))
        for odd in range(2):
            for n in range(2):
                conv_block(2 * e + odd, n)
                m.append(product(e, len(m)))
        b = _combine(m)
        for odd in range(2):
            blk = slice((2 * e + odd) * T, (2 * e + odd + 1) * T)
            g = gate_ref[blk, :]
            for n in range(2):
                out_ref[blk, cols[n]] = (
                    g * a.pop((2 * e + odd, n)) + (1.0 - g) * b[2 * odd + n]).astype(BF16)


def _kernel(x_hbm, ak_hbm, av_hbm, shift_in, hk_hbm, skip_in, c_hbm, wq_hbm, wuk_hbm,
            wuv_hbm, wo_hbm, gw_in, fwd_in, inv_in, out_hbm,
            x_ref, ak_ref, av_ref, hk_ref, c_ref, wq_ref, wkv_ref, wo_ref, cs_ref, xs_ref,
            kv_ref, gate_ref, shift_ref, skip_ref, fwd_ref, inv_ref, kpad_ref, uf_ref, hf_ref,
            out_ref, c_sem, wkv_sem, x_sem, late_sem, out_sem):
    steps = NB // 2
    late = [(ak_hbm, ak_ref), (av_hbm, av_ref), (hk_hbm, hk_ref), (wo_hbm, wo_ref)]

    def pair_copy(w_hbm, p, dst, sem):
        return pltpu.make_async_copy(w_hbm.bitcast(U32).at[:, p, :], dst, sem)

    def rows_copy(src, dst, t, sem):
        n = src.shape[0] // steps
        rows = pl.ds(pl.multiple_of(t * n, n), n)
        return pltpu.make_async_copy(src.at[rows], dst.at[rows], sem)

    def wait_filled(buf, sem):
        pltpu.make_async_copy(buf, buf, sem).wait()

    def fetch_step(w_hbm, t):
        for b in range(4):
            pair_copy(w_hbm, (t & 3) * 4 + b, wkv_ref.at[t * 4 + b], wkv_sem.at[t]).start()
        rows_copy(x_hbm, x_ref, t, x_sem.at[t]).start()

    c_copy = pltpu.make_async_copy(c_hbm, c_ref, c_sem)
    c_copy.start()
    fetch_step(wuk_hbm, 0)
    shift_ref[...] = shift_in[...].astype(F32)
    skip_ref[...] = skip_in[...].astype(F32).reshape(1, DM)
    fwd_ref[...] = fwd_in[...].astype(BF16)
    inv_ref[...] = inv_in[...].astype(BF16)
    kpad_ref[:, 0:8, :] = jnp.zeros((2, 8, T), F32)
    gw = gw_in[...].astype(F32).reshape(1, DM)
    c_copy.wait()
    for e in range(steps):
        _store_left(c_ref, cs_ref, e)

    def kv_step(t, carry):
        pl.when(t < 3)(lambda: fetch_step(wuk_hbm, t + 1))
        pl.when((t >= 3) & (t < steps - 1))(lambda: fetch_step(wuv_hbm, t + 1))
        for k in range(2):
            pair_copy(wq_hbm, 2 * t + k, wq_ref.at[2 * t + k], late_sem.at[4]).start()
        for k, (src, dst) in enumerate(late):
            rows_copy(src, dst, t, late_sem.at[k]).start()
        wait_filled(wkv_ref.at[pl.ds(t * 4, 4)], wkv_sem.at[t])
        rows_copy(x_hbm, x_ref, t, x_sem.at[t]).wait()
        _project_kv(t, cs_ref, wkv_ref, kv_ref)
        x = _store_left(x_ref, xs_ref, t)
        z = jnp.sum(x * gw, axis=1, keepdims=True)
        gate_ref[pl.ds(pl.multiple_of(t * 2 * T, 2 * T), 2 * T), :] = jnp.broadcast_to(
            1.0 / (1.0 + jnp.exp(-z)), (2 * T, T))
        return carry

    lax.fori_loop(0, steps, kv_step, 0)

    wait_filled(wq_ref, late_sem.at[4])

    def pair_step(p, carry):
        _attend_pair(p, xs_ref, wq_ref, kv_ref)
        return carry

    lax.fori_loop(0, NP, pair_step, 0)

    for k, (_, dst) in enumerate(late):
        wait_filled(dst, late_sem.at[k])

    def out_copy(c):
        cols = pl.ds(pl.multiple_of(c * 2 * T, 2 * T), 2 * T)
        return pltpu.make_async_copy(out_ref.at[:, cols], out_hbm.at[:, cols], out_sem.at[c])

    def mix_step(c, carry):
        _mix_pair(c, kv_ref, wo_ref, x_ref, ak_ref, av_ref, hk_ref, shift_ref, skip_ref,
                  gate_ref, fwd_ref, inv_ref, kpad_ref, uf_ref, hf_ref, out_ref)
        out_copy(c).start()
        return carry

    lax.fori_loop(0, DM // (2 * T), mix_step, 0)
    for c in range(DM // (2 * T)):
        out_copy(c).wait()


@jax.jit
def pallas_gated_mix__ssm_conv_h3__compressed_kv_cla__prompt_kernel(
    A_q: jax.Array,
    A_k: jax.Array,
    A_v: jax.Array,
    A_shift_k: jax.Array,
    A_ssm_k: jax.Array,
    A_ssm_D: jax.Array,
    B_x: jax.Array,
    B_c_kv: jax.Array,
    B_w_q: jax.Array,
    B_w_uk: jax.Array,
    B_w_uv: jax.Array,
    B_w_o: jax.Array,
    gate_w: jax.Array,
):
    del B_x
    fwd, inv = _dft_matrices()
    hbm = pl.BlockSpec(memory_space=pl.ANY)
    vmem = pl.BlockSpec(memory_space=pltpu.VMEM)
    out = pl.pallas_call(
        _kernel,
        out_shape=jax.ShapeDtypeStruct((S, DM), BF16),
        in_specs=[hbm, hbm, hbm, vmem, hbm, vmem, hbm, hbm, hbm, hbm, hbm, vmem, vmem, vmem],
        out_specs=hbm,
        scratch_shapes=[
            pltpu.VMEM((S, DM), BF16),
            pltpu.VMEM((S, DM), BF16),
            pltpu.VMEM((S, DM), BF16),
            pltpu.VMEM((DM, S), BF16),
            pltpu.VMEM((S, DC), BF16),
            pltpu.VMEM((NP, DM, DH), U32),
            pltpu.VMEM((2 * NP, DC, DH), U32),
            pltpu.VMEM((H * DH, DM), BF16),
            pltpu.VMEM((7, S // 4, DC // 2), U32),
            pltpu.VMEM((7, S // 4, DM // 2), U32),
            pltpu.VMEM((NP, 2 * S, DH), U32),
            pltpu.VMEM((S, T), F32),
            pltpu.VMEM((KS, DM), F32),
            pltpu.VMEM((1, DM), F32),
            pltpu.VMEM((2 * T, T), BF16),
            pltpu.VMEM((T, 2 * T), BF16),
            pltpu.VMEM((2, 8 + S, T), F32),
            pltpu.VMEM((2, NB, 2 * T, T), F32),
            pltpu.VMEM((2, NB, 2 * T, T), F32),
            pltpu.VMEM((S, DM), BF16),
            pltpu.SemaphoreType.DMA,
            pltpu.SemaphoreType.DMA((NB // 2,)),
            pltpu.SemaphoreType.DMA((NB // 2,)),
            pltpu.SemaphoreType.DMA((5,)),
            pltpu.SemaphoreType.DMA((DM // (2 * T),)),
        ],
        compiler_params=pltpu.CompilerParams(vmem_limit_bytes=124 * 2**20),
    )(
        A_q.reshape(S, DM), A_k.reshape(S, DM), A_v.reshape(S, DM), A_shift_k.T,
        A_ssm_k, A_ssm_D, B_c_kv.reshape(S, DC), B_w_q, B_w_uk, B_w_uv,
        B_w_o.reshape(H * DH, DM), gate_w, fwd, inv,
    )
    return out.reshape(1, S, DM)
```

```python
import functools

import jax
import jax.numpy as jnp
import numpy as np
from jax import lax
import jax.experimental.pallas as pl
import jax.experimental.pallas.tpu as pltpu

S = 2048
DM = 1024
H = 32
DH = 128
DC = 512
T = 128
NB = S // T
NP = H // 2
KS = 4
CH = 4
W = T // 2

F32 = jnp.float32
BF16 = jnp.bfloat16
U32 = jnp.uint32
NT = (((1,), (1,)), ((), ()))
import os
OPT = dict(a.split('=') for a in os.environ.get('OPT', '').split())
LEAD = int(OPT.get('lead', 12))
LAG = int(OPT.get('lag', 2))
PH = OPT.get('ph', '123')
LC, LX, LG = 0, DC // 2, DC // 2 + DM // 2


def _dft_matrices():
    ks = np.concatenate([np.arange(0, T, 2), np.arange(1, T, 2)]).reshape(NB, 8)
    n = np.arange(T)
    theta = 2.0 * np.pi * (ks[:, :, None] + 0.5) * n[None, None, :] / (2 * T)
    fwd = np.concatenate([np.cos(theta), -np.sin(theta)], axis=1).reshape(2 * T, T)
    inv = fwd.T / T
    return fwd.astype(np.float32), inv.astype(np.float32)


def _mm(a, b):
    return jnp.dot(a, b, preferred_element_type=F32)


def _pack(v):
    return pltpu.pack_elementwise([v[:W], v[W:]], packed_dtype=BF16)


def _halves(words):
    return [pltpu.unpack_elementwise(words, index=i, packed_dtype=BF16, unpacked_dtype=F32)
            for i in range(2)]


def _unpack(words):
    return pltpu.bitcast(words, BF16)


def _after(v, earlier):
    return jnp.maximum(v, jnp.minimum(earlier, v))


def _left(a11, a12, a21, a22):
    return [a11 + a22, a21 + a22, a11, a22, a11 + a12, a21 - a11, a12 - a22]


def _right_operand(i, b):
    first, sign, second = (
        ((0, 0), 1, (1, 1)), ((0, 0), 0, None), ((0, 1), -1, (1, 1)), ((1, 0), -1, (0, 0)),
        ((1, 1), 0, None), ((0, 0), 1, (0, 1)), ((1, 0), 1, (1, 1)))[i]
    if sign == 0:
        return b(*first)
    return b(*first) + b(*second) if sign > 0 else b(*first) - b(*second)


def _combine(m):
    return (m[0] + m[3] - m[4] + m[6], m[2] + m[4], m[1] + m[3], m[0] - m[1] + m[2] + m[5])


def _pair_weights(words):
    half = words.shape[0] // 2
    heads = _halves(words)
    return [_right_operand(i, lambda r, c: heads[c][r * half:(r + 1) * half]).astype(BF16)
            for i in range(7)]


def _store_left(src_ref, dst_ref, lane, e):
    half = src_ref.shape[1] // 2
    v = src_ref[pl.ds(pl.multiple_of(e * 2 * T, 2 * T), 2 * T), :]
    even, odd = _halves(pltpu.bitcast(v, U32))
    top = jnp.concatenate([even[:W], odd[:W]], axis=0)
    bottom = jnp.concatenate([even[W:], odd[W:]], axis=0)
    ops = _left(top[:, :half], top[:, half:], bottom[:, :half], bottom[:, half:])
    for i in range(7):
        dst_ref[i, pl.ds(pl.multiple_of(e * W, W), W), lane:lane + half] = pltpu.bitcast(
            ops[i].astype(BF16), U32)
    return v


def _project_kv(t, left_ref, wkv_ref, kv_ref, meanwhile):
    base = pl.multiple_of((t >> 2) * S, S)
    for b in range(4):
        if b == int(OPT.get('mw', 2)):
            meanwhile()
        w = _pair_weights(wkv_ref[t * 4 + b])
        pair = (t & 3) * 4 + b
        for e in range(0, NB // 2, 2):
            c = _combine([_mm(_unpack(left_ref[i, e * W:(e + 2) * W, LC:LX]), w[i]) for i in range(7)])
            for k in range(2):
                for odd in range(2):
                    for head in range(2):
                        r0 = head * (S // 2) + (2 * (e + k) + odd) * W
                        kv_ref[pair, pl.ds(base + r0, W), :] = _pack(
                            c[2 * odd + head][k * T:(k + 1) * T])


def _operand_row(e, i):
    return (i // 2) * (S // 2) + (2 * e + i % 2) * W


def _attend_pair(p, left_ref, wq_ref, kv_ref):
    row = lax.broadcasted_iota(jnp.int32, (T, T), 0)
    col = lax.broadcasted_iota(jnp.int32, (T, T), 1)
    causal = col <= jnp.where(row < W, 2 * row, 2 * (row - W) + 1)
    scale = DH ** -0.5 * np.log2(np.e)
    w = _pair_weights(wq_ref[p])
    q, s, ctx, sums, done = {}, {}, {}, [], []
    zero = lax.shift_right_logical(p, 8)

    def chunks(r):
        return [(j, min(j + CH, r + 1)) for j in range(0, r + 1, CH)]

    def tiles(region, j0, j1):
        r0 = region * (S // 2)
        return _unpack(kv_ref[p, r0 + j0 * W:r0 + j1 * W, :])

    def queries(e):
        c = _combine([_mm(_unpack(left_ref[i, e * W:(e + 1) * W, LX:LG]), w[i]) for i in range(7)])
        for odd in range(2):
            for head in range(2):
                q[2 * e + odd, head] = (c[2 * odd + head] * scale).astype(BF16)

    def scores(r, head):
        parts, m = [], None
        for j0, j1 in chunks(r):
            d = lax.dot_general(q[r, head], tiles(head, j0, j1), NT, preferred_element_type=F32)
            for j in range(j0, j1):
                t = d[:, (j - j0) * T:(j - j0 + 1) * T]
                if j == r:
                    t = jnp.where(causal, t, -1e9)
                parts.append(t)
                m = t if m is None else jnp.maximum(m, t)
        s[r, head] = parts, jnp.max(m, axis=1, keepdims=True)

    def context(r, head):
        parts, top = s.pop((r, head))
        top = jnp.broadcast_to(top, (T, T))
        l, o = None, None
        for j0, j1 in chunks(r):
            m = top
            if 'l' in OPT.get('pin', 'x') and len(sums) >= LAG:
                m = _after(m, sums[-LAG])
            if 'o' in OPT.get('pin', 'x') and j0 == 0 and len(done) >= 2:
                m = _after(m, done[-2])
            ps = [jnp.exp2(parts[j] - m) for j in range(j0, j1)]
            G = int(OPT.get('g', 4))
            for k in range(0, len(ps), G):
                t = ps[k]
                for e in ps[k + 1:k + G]:
                    t = t + e
                if len(ps[k:k + G]) > 1:
                    last = min(k + G, len(ps)) - 1
                    ps[last] = jnp.minimum(ps[last], t)
                l = t if l is None else l + t
            sums.append(l)
            if 'p' in OPT.get('pin', 'x'):
                ps[-1] = jnp.minimum(ps[-1], l)
            if 'q' in OPT.get('pin', 'x'):
                ps[0] = jnp.minimum(ps[0], l)
            e = ps[0] if len(ps) == 1 else jnp.concatenate(ps, axis=1)
            d = _mm(e.astype(BF16), tiles(2 + head, j0, j1))
            o = d if o is None else o + d
        l = jnp.sum(l, axis=1, keepdims=True)
        inv = pltpu.reciprocal(l, approx=True)
        inv = inv * (2.0 - l * inv)
        ctx[r, head] = o * inv
        done.append(ctx[r, head])

    def emit(e):
        ops = _left(*[ctx.pop((2 * e + odd, head)) for odd in range(2) for head in range(2)])
        for i in range(7):
            r0 = _operand_row(e, i)
            if 'z' not in OPT:
                kv_ref[p, r0:r0 + W, :] = _pack(ops[i])
            else:
                kv_ref[p, pl.ds(pl.multiple_of(zero * W + r0, W), W), :] = _pack(ops[i])

    todo = [(r, head) for r in range(NB - 1, -1, -1) for head in range(2)]
    if 'seq' in OPT:
        todo = [(r, head) for head in range(2) for r in range(NB - 1, -1, -1)]
    if 'one' in OPT:
        todo = [(r, head) for head in range(1) for r in range(NB - 1, -1, -1)]
    next_q, next_s, lead, ready = NB // 2 - 1, 0, 0, []
    for r, head in todo:
        while next_s < len(todo) and lead < LEAD + r + 1:
            rs, hs = todo[next_s]
            while next_q >= 0 and next_q >= rs // 2 - 1:
                queries(next_q)
                next_q -= 1
            scores(rs, hs)
            lead += rs + 1
            next_s += 1
        context(r, head)
        lead -= r + 1
        ready.append(r // 2 if head == 1 and r % 2 == 0 else None)
        if len(ready) > int(OPT.get('ed', 1)):
            e = ready.pop(0)
            if e is not None:
                emit(e)
    for e in ready:
        if e is not None:
            emit(e)


def _mix_step(c, half, kv_ref, wo_ref, x_ref, ak_ref, av_ref, hk_ref, shift_ref, skip_ref,
              left_ref, fwd_ref, inv_ref, kpad_ref, uf_ref, hf_ref, held_ref, out_ref):
    cols = [pl.ds(pl.multiple_of((2 * c + n) * T, T), T) for n in range(2)]
    own = cols[half]
    fwd = fwd_ref[...]
    inv = inv_ref[...]
    kpad_ref[8:, :] = ak_ref[:, own].astype(F32)
    taps = shift_ref[:, own]
    skip = skip_ref[:, own]

    def heads(odd, n, i):
        lanes = pl.ds(pl.multiple_of((2 * c + n + lax.shift_right_logical(c, 24 + i)) * T, T), T)
        return jnp.concatenate(
            [wo_ref[h * DH:(h + 1) * DH, lanes].astype(F32) for h in range(odd, H, 2)], axis=0)

    w = [_right_operand(i, functools.partial(heads, i=i)).astype(BF16) for i in range(7)]
    zero = jnp.full((8, T), lax.shift_right_logical(c, 8), jnp.int32).astype(U32)
    before, u, z, parts, due = [], {}, {}, {}, {}

    def gate(j):
        return pltpu.bitcast(_gate_rows(left_ref, j)[...], F32)

    def deliver(j, n, v):
        blk = slice(j * T, (j + 1) * T)
        if n == half and j // 8 == half:
            if (j, n) not in parts:
                parts[j, n] = v
                return
            v = v + parts.pop((j, n))
        elif half == 0:
            held_ref[c, blk, :] = v
            return
        else:
            v = v + held_ref[c, blk, :]
        out_ref[blk, cols[n]] = v.astype(BF16)

    def spectra(j):
        cur = lax.dot_general(fwd, hk_ref[own, j * T:(j + 1) * T], NT, preferred_element_type=F32)
        for f in range(NB):
            re, im = slice(16 * f, 16 * f + 8), slice(16 * f + 8, 16 * f + 16)
            if j == 0:
                hr, hi = cur[re], cur[im]
            elif f < NB // 2:
                hr, hi = cur[re] - before[-1][im], cur[im] + before[-1][re]
            else:
                hr, hi = cur[re] + before[-1][im], cur[im] - before[-1][re]
            hf_ref[j, re, :] = hr
            hf_ref[j, im, :] = hi
        before.append(cur)
        ksh = kpad_ref[pl.ds(8 + j * T, T), :] * taps[0:1]
        for t in range(1, KS):
            ksh = ksh + kpad_ref[pl.ds(8 + j * T - t, T), :] * taps[t:t + 1]
        u[j] = (ksh * av_ref[j * T:(j + 1) * T, own].astype(F32)).astype(BF16)
        uf_ref[j] = _mm(fwd, u[j])

    def products(i0, i1, start, step):
        base = lax.shift_right_logical(c, 8 + i0)
        rows = {i: [] for i in range(i0, i1)}
        for f in range(NB):
            re, im = slice(16 * f, 16 * f + 8), slice(16 * f + 8, 16 * f + 16)
            acc = {}
            for j in range(i1):
                ur, ui = uf_ref[base + j, re, :], uf_ref[base + j, im, :]
                for i in range(max(i0, j), i1):
                    hr, hi = hf_ref[base + i - j, re, :], hf_ref[base + i - j, im, :]
                    pr, pi = ur * hr - ui * hi, ur * hi + ui * hr
                    acc[i] = (pr, pi) if j == 0 else (acc[i][0] + pr, acc[i][1] + pi)
            bits = None
            for i in range(i0, i1):
                rows[i] += acc[i]
                for v in acc[i]:
                    v = pltpu.bitcast(v, U32)
                    bits = v if bits is None else bits | v
            due[int(start + f * step)] = bits & zero
        for i in range(i0, i1):
            z[i] = jnp.concatenate(rows[i], axis=0).astype(BF16)

    def convolved(i):
        y = _mm(inv, z.pop(i)) + u.pop(i).astype(F32) * skip
        deliver(i, half, gate(i) * (x_ref[i * T:(i + 1) * T, own].astype(F32) * y))

    def product(e, i):
        r0 = _operand_row(e, i)
        left = [kv_ref[p, r0:r0 + W, :] for p in range(NP)]
        for p in range(0, NP, 4):
            at = 32 * i + 2 * p
            if any(at + k in due for k in range(8)):
                rows = [left[p][8 * k:8 * k + 8] for k in range(8)]
                left[p] = jnp.concatenate(
                    [v | due.pop(at + k) if at + k in due else v for k, v in enumerate(rows)],
                    axis=0)
        return _mm(_unpack(jnp.concatenate(left, axis=1)), w[i])

    groups = [((0, 2), (2, 4)), ((4, 6), (14, 16)), ((6, 8), (12, 14)), ((8, 10), (10, 12))]
    if half == 1:
        groups = [groups[0], groups[3], groups[2][::-1], groups[1][::-1]]
    t0 = eval(OPT.get('t0', '((64,3),(130,4))'))
    t1 = eval(OPT.get('t1', '((4,7.5),(130,5.8))'))
    sp = list(eval(OPT.get('sp', '6,8,10,12,14,16')))
    for step, pair in enumerate(groups):
        e = 4 * half + step
        m = []
        for k, (i0, i1) in enumerate(pair):
            if step == 0 and k == 0:
                for j in range(int(OPT.get('s0', 4))):
                    spectra(j)
            products(i0, i1, *(t0 if step == 0 else t1)[k])
            for _ in range(4 - k):
                m.append(product(e, len(m)))
                for j in range(len(before), sp.pop(0) if sp else 0):
                    spectra(j)
            for i in range(i0, i1):
                convolved(i)
        b = _combine(m)
        for odd in range(2):
            for n in range(2):
                deliver(2 * e + odd, n, (1.0 - gate(2 * e + odd)) * b[2 * odd + n])


def _gate_rows(left_ref, j):
    return left_ref.at[j // 4, (j % 4) * T:(j % 4 + 1) * T, LG:]


def _kernel(x_hbm, ak_hbm, av_hbm, shift_in, hk_hbm, skip_in, c_hbm, wq_hbm, wuk_hbm,
            wuv_hbm, wo_hbm, gw_in, fwd_in, inv_in, out_hbm,
            x_ref, ak_ref, av_ref, hk_ref, c_ref, wq_ref, wkv_ref, wo_ref, left_ref,
            kv_ref, shift_ref, skip_ref, fwd_ref, inv_ref, kpad_ref, uf_ref, hf_ref, held_ref,
            out_ref, in_sem, wkv_sem, wq_sem, out_sem):
    steps = NB // 2

    def pair_copy(w_hbm, p, dst, sem):
        return pltpu.make_async_copy(w_hbm.bitcast(U32).at[:, p, :], dst, sem)

    def wait_filled(buf, sem):
        pltpu.make_async_copy(buf, buf, sem).wait()

    def fetch_group(t):
        for b in range(4):
            pair_copy(wuk_hbm if t < 4 else wuv_hbm, (t % 4) * 4 + b,
                      wkv_ref.at[t * 4 + b], wkv_sem.at[t]).start()

    first, rest = pl.ds(0, 2 * T), pl.ds(2 * T, S - 2 * T)
    plain = [(c_hbm, c_ref), (x_hbm.at[first], x_ref.at[first]),
             (x_hbm.at[rest], x_ref.at[rest]), (wo_hbm, wo_ref), (ak_hbm, ak_ref),
             (av_hbm, av_ref), (hk_hbm, hk_ref)]
    copies = [pltpu.make_async_copy(s, d, in_sem.at[k]) for k, (s, d) in enumerate(plain)]

    def fetch_ahead(t):
        if t == 0:
            copies[2].start()
        fetch_group(t + 2)
        if 1 <= t <= 4:
            for p in range(4 * t - 4, 4 * t):
                pair_copy(wq_hbm, p, wq_ref.at[p], wq_sem).start()
        if t == 5:
            for cp in copies[3:]:
                cp.start()

    copies[0].start()
    fetch_group(0)
    copies[1].start()
    fetch_group(1)
    shift_ref[...] = shift_in[...].astype(F32)
    skip_ref[...] = skip_in[...].astype(F32).reshape(1, DM)
    fwd_ref[...] = fwd_in[...].astype(BF16)
    inv_ref[...] = inv_in[...].astype(BF16)
    kpad_ref[0:8, :] = jnp.zeros((8, T), F32)
    copies[0].wait()

    def left_step(e, carry):
        _store_left(c_ref, left_ref, LC, e)
        return carry

    lax.fori_loop(0, steps, left_step, 0)

    def kv_step(t, carry):
        for k in range(steps - 2):
            pl.when(t == k)(functools.partial(fetch_ahead, k))
        pl.when(t == 0)(copies[1].wait)
        pl.when(t == 1)(copies[2].wait)
        wait_filled(wkv_ref.at[pl.ds(t * 4, 4)], wkv_sem.at[t])

        def meanwhile():
            x = _store_left(x_ref, left_ref, LX, t)
            z = jnp.sum(x.astype(F32) * gw_in[...].astype(F32).reshape(1, DM), axis=1, keepdims=True)
            g = jnp.broadcast_to(1.0 / (1.0 + jnp.exp(-z)), (2 * T, T))
            rows = pl.ds(pl.multiple_of((t & 1) * 2 * T, 2 * T), 2 * T)
            left_ref[t >> 1, rows, LG:] = pltpu.bitcast(g, U32)

        _project_kv(t, left_ref, wkv_ref, kv_ref, meanwhile)
        return carry

    if '1' in PH:
        lax.fori_loop(0, steps, kv_step, 0)

    wait_filled(wq_ref, wq_sem)

    def pair_step(p, carry):
        _attend_pair(p, left_ref, wq_ref, kv_ref)
        return carry

    if '2' in PH:
        lax.fori_loop(0, NP, pair_step, 0)

    for cp in copies[3:]:
        cp.wait()

    def out_copy(c):
        cols = pl.ds(pl.multiple_of(c * 2 * T, 2 * T), 2 * T)
        return pltpu.make_async_copy(out_ref.at[:, cols], out_hbm.at[:, cols], out_sem.at[c])

    for half in range(2):
        def mix_step(c, carry):
            _mix_step(c, half, kv_ref, wo_ref, x_ref, ak_ref, av_ref, hk_ref, shift_ref,
                      skip_ref, left_ref, fwd_ref, inv_ref, kpad_ref, uf_ref, hf_ref, held_ref,
                      out_ref)
            if half == 1:
                out_copy(c).start()
            return carry

        if '3' in PH and str(half) in OPT.get('half', '01'):
            lax.fori_loop(0, DM // (2 * T), mix_step, 0)
    for c in range(DM // (2 * T)):
        out_copy(c).wait()


@jax.jit
def pallas_gated_mix__ssm_conv_h3__compressed_kv_cla__prompt_kernel(
    A_q: jax.Array,
    A_k: jax.Array,
    A_v: jax.Array,
    A_shift_k: jax.Array,
    A_ssm_k: jax.Array,
    A_ssm_D: jax.Array,
    B_x: jax.Array,
    B_c_kv: jax.Array,
    B_w_q: jax.Array,
    B_w_uk: jax.Array,
    B_w_uv: jax.Array,
    B_w_o: jax.Array,
    gate_w: jax.Array,
):
    del B_x
    fwd, inv = _dft_matrices()
    hbm = pl.BlockSpec(memory_space=pl.ANY)
    vmem = pl.BlockSpec(memory_space=pltpu.VMEM)
    out = pl.pallas_call(
        _kernel,
        out_shape=jax.ShapeDtypeStruct((S, DM), BF16),
        in_specs=[hbm, hbm, hbm, vmem, hbm, vmem, hbm, hbm, hbm, hbm, hbm, vmem, vmem, vmem],
        out_specs=hbm,
        scratch_shapes=[
            pltpu.VMEM((S, DM), BF16),
            pltpu.VMEM((S, DM), BF16),
            pltpu.VMEM((S, DM), BF16),
            pltpu.VMEM((DM, S), BF16),
            pltpu.VMEM((S, DC), BF16),
            pltpu.VMEM((NP, DM, DH), U32),
            pltpu.VMEM((2 * NP, DC, DH), U32),
            pltpu.VMEM((H * DH, DM), BF16),
            pltpu.VMEM((7, S // 4, LG + T), U32),
            pltpu.VMEM((NP, 2 * S, DH), U32),
            pltpu.VMEM((KS, DM), F32),
            pltpu.VMEM((1, DM), F32),
            pltpu.VMEM((2 * T, T), BF16),
            pltpu.VMEM((T, 2 * T), BF16),
            pltpu.VMEM((8 + S, T), F32),
            pltpu.VMEM((NB, 2 * T, T), F32),
            pltpu.VMEM((NB, 2 * T, T), F32),
            pltpu.VMEM((DM // (2 * T), S, T), F32),
            pltpu.VMEM((S, DM), BF16),
            pltpu.SemaphoreType.DMA((7,)),
            pltpu.SemaphoreType.DMA((NB // 2,)),
            pltpu.SemaphoreType.DMA,
            pltpu.SemaphoreType.DMA((DM // (2 * T),)),
        ],
        compiler_params=pltpu.CompilerParams(vmem_limit_bytes=127 * 2**20),
    )(
        A_q.reshape(S, DM), A_k.reshape(S, DM), A_v.reshape(S, DM), A_shift_k.T,
        A_ssm_k, A_ssm_D, B_c_kv.reshape(S, DC), B_w_q, B_w_uk, B_w_uv,
        B_w_o.reshape(H * DH, DM), gate_w, fwd, inv,
    )
    return out.reshape(1, S, DM)
```

```python
import functools

import jax
import jax.numpy as jnp
import numpy as np
from jax import lax
import jax.experimental.pallas as pl
import jax.experimental.pallas.tpu as pltpu

S = 2048
DM = 1024
H = 32
DH = 128
DC = 512
T = 128
NB = S // T
NP = H // 2
KS = 4
CH = 4
W = T // 2

F32 = jnp.float32
BF16 = jnp.bfloat16
U32 = jnp.uint32
NT = (((1,), (1,)), ((), ()))
import os
OPT = dict(a.split('=') for a in os.environ.get('OPT', '').split())
LEAD = int(OPT.get('lead', 12))
LAG = int(OPT.get('lag', 2))
PH = OPT.get('ph', '123')


def _dft_matrices():
    ks = np.concatenate([np.arange(0, T, 2), np.arange(1, T, 2)]).reshape(NB, 8)
    n = np.arange(T)
    theta = 2.0 * np.pi * (ks[:, :, None] + 0.5) * n[None, None, :] / (2 * T)
    fwd = np.concatenate([np.cos(theta), -np.sin(theta)], axis=1).reshape(2 * T, T)
    inv = fwd.T / T
    return fwd.astype(np.float32), inv.astype(np.float32)


def _mm(a, b):
    return jnp.dot(a, b, preferred_element_type=F32)


def _pack(v):
    return pltpu.pack_elementwise([v[:W], v[W:]], packed_dtype=BF16)


def _halves(words):
    return [pltpu.unpack_elementwise(words, index=i, packed_dtype=BF16, unpacked_dtype=F32)
            for i in range(2)]


def _unpack(words):
    return pltpu.bitcast(words, BF16)


def _after(v, earlier):
    return jnp.maximum(v, jnp.minimum(earlier, v))


def _zero_word(i):
    return jnp.full((8, T), lax.shift_right_logical(i, 8), jnp.int32).astype(U32)


def _left(a11, a12, a21, a22):
    return [a11 + a22, a21 + a22, a11, a22, a11 + a12, a21 - a11, a12 - a22]


def _right_operand(i, b):
    first, sign, second = (
        ((0, 0), 1, (1, 1)), ((0, 0), 0, None), ((0, 1), -1, (1, 1)), ((1, 0), -1, (0, 0)),
        ((1, 1), 0, None), ((0, 0), 1, (0, 1)), ((1, 0), 1, (1, 1)))[i]
    if sign == 0:
        return b(*first)
    return b(*first) + b(*second) if sign > 0 else b(*first) - b(*second)


def _combine(m):
    return (m[0] + m[3] - m[4] + m[6], m[2] + m[4], m[1] + m[3], m[0] - m[1] + m[2] + m[5])


def _pair_weights(words):
    half = words.shape[0] // 2
    heads = _halves(words)
    return [_right_operand(i, lambda r, c: heads[c][r * half:(r + 1) * half]).astype(BF16)
            for i in range(7)]


def _store_left(src_ref, half, cols, dst_ref, e, r0, r1):
    parts = []
    for j in range(2):
        for c0 in (0, half):
            v = src_ref[pl.ds(pl.multiple_of((2 * e + j) * T + r0, 32), r1 - r0),
                        c0 + cols.start:c0 + cols.stop]
            parts.append(_halves(pltpu.bitcast(v, U32)))
    stored = []
    for odd in range(2):
        rows = pl.ds(pl.multiple_of(e * W + odd * (W // 2) + r0 // 4, 8), (r1 - r0) // 4)
        for i, v in enumerate(_left(*[part[odd] for part in parts])):
            stored.append(pltpu.bitcast(v.astype(BF16), U32))
            dst_ref[i, rows, cols] = stored[-1]
    return stored


def _project_kv(t, cs_ref, wkv_ref, kv_ref, meanwhile):
    base = pl.multiple_of((t >> 2) * S, S)
    for b in range(4):
        w = _pair_weights(wkv_ref[t * 4 + b])
        pair = (t & 3) * 4 + b
        for e in range(0, NB // 2, 2):
            left = [cs_ref[i, e * W:(e + 2) * W, :] for i in range(7)]
            at = int(OPT.get('mw', 2))
            tie = meanwhile(b, e // 2)
            left[at] = jnp.concatenate(
                [left[at][:8] | jnp.concatenate([tie, tie], axis=1), left[at][8:]], axis=0)
            c = _combine([_mm(_unpack(left[i]), w[i]) for i in range(7)])
            for k in range(2):
                for odd in range(2):
                    for head in range(2):
                        r0 = head * (S // 2) + (2 * (e + k) + odd) * W
                        kv_ref[pair, pl.ds(base + r0, W), :] = _pack(
                            c[2 * odd + head][k * T:(k + 1) * T])


def _operand_row(e, i):
    return (i // 2) * (S // 2) + (2 * e + i % 2) * W


def _attend_pair(p, xs_ref, wq_ref, kv_ref):
    row = lax.broadcasted_iota(jnp.int32, (T, T), 0)
    col = lax.broadcasted_iota(jnp.int32, (T, T), 1)
    causal = col <= jnp.where(row < W, 2 * row, 2 * (row - W) + 1)
    scale = DH ** -0.5 * np.log2(np.e)
    w = _pair_weights(wq_ref[p])
    q, s, ctx, sums, done = {}, {}, {}, [], []
    zero = lax.shift_right_logical(p, 8)

    def chunks(r):
        return [(j, min(j + CH, r + 1)) for j in range(0, r + 1, CH)]

    def tiles(region, j0, j1):
        r0 = region * (S // 2)
        return _unpack(kv_ref[p, r0 + j0 * W:r0 + j1 * W, :])

    def queries(e):
        c = _combine([_mm(_unpack(xs_ref[i, e * W:(e + 1) * W, :]), w[i]) for i in range(7)])
        for odd in range(2):
            for head in range(2):
                q[2 * e + odd, head] = (c[2 * odd + head] * scale).astype(BF16)

    def scores(r, head):
        parts, m = [], None
        for j0, j1 in chunks(r):
            d = lax.dot_general(q[r, head], tiles(head, j0, j1), NT, preferred_element_type=F32)
            for j in range(j0, j1):
                t = d[:, (j - j0) * T:(j - j0 + 1) * T]
                if j == r:
                    t = jnp.where(causal, t, -1e9)
                parts.append(t)
                m = t if m is None else jnp.maximum(m, t)
        s[r, head] = parts, jnp.max(m, axis=1, keepdims=True)

    def context(r, head):
        parts, top = s.pop((r, head))
        top = jnp.broadcast_to(top, (T, T))
        l, o = None, None
        for j0, j1 in chunks(r):
            m = top
            if 'l' in OPT.get('pin', 'x') and len(sums) >= LAG:
                m = _after(m, sums[-LAG])
            if 'o' in OPT.get('pin', 'x') and j0 == 0 and len(done) >= 2:
                m = _after(m, done[-2])
            ps = [jnp.exp2(parts[j] - m) for j in range(j0, j1)]
            G = int(OPT.get('g', 4))
            for k in range(0, len(ps), G):
                t = ps[k]
                for e in ps[k + 1:k + G]:
                    t = t + e
                if len(ps[k:k + G]) > 1:
                    last = min(k + G, len(ps)) - 1
                    ps[last] = jnp.minimum(ps[last], t)
                l = t if l is None else l + t
            sums.append(l)
            if 'p' in OPT.get('pin', 'x'):
                ps[-1] = jnp.minimum(ps[-1], l)
            if 'q' in OPT.get('pin', 'x'):
                ps[0] = jnp.minimum(ps[0], l)
            e = ps[0] if len(ps) == 1 else jnp.concatenate(ps, axis=1)
            d = _mm(e.astype(BF16), tiles(2 + head, j0, j1))
            o = d if o is None else o + d
        l = jnp.sum(l, axis=1, keepdims=True)
        inv = pltpu.reciprocal(l, approx=True)
        inv = inv * (2.0 - l * inv)
        ctx[r, head] = o * inv
        done.append(ctx[r, head])

    def emit(e):
        ops = _left(*[ctx.pop((2 * e + odd, head)) for odd in range(2) for head in range(2)])
        for i in range(7):
            r0 = _operand_row(e, i)
            if 'z' not in OPT:
                kv_ref[p, r0:r0 + W, :] = _pack(ops[i])
            else:
                kv_ref[p, pl.ds(pl.multiple_of(zero * W + r0, W), W), :] = _pack(ops[i])

    todo = [(r, head) for r in range(NB - 1, -1, -1) for head in range(2)]
    if 'seq' in OPT:
        todo = [(r, head) for head in range(2) for r in range(NB - 1, -1, -1)]
    if 'one' in OPT:
        todo = [(r, head) for head in range(1) for r in range(NB - 1, -1, -1)]
    next_q, next_s, lead, ready = NB // 2 - 1, 0, 0, []
    for r, head in todo:
        while next_s < len(todo) and lead < LEAD + r + 1:
            rs, hs = todo[next_s]
            while next_q >= 0 and next_q >= rs // 2 - 1:
                queries(next_q)
                next_q -= 1
            scores(rs, hs)
            lead += rs + 1
            next_s += 1
        context(r, head)
        lead -= r + 1
        ready.append(r // 2 if head == 1 and r % 2 == 0 else None)
        if len(ready) > int(OPT.get('ed', 1)):
            e = ready.pop(0)
            if e is not None:
                emit(e)
    for e in ready:
        if e is not None:
            emit(e)


def _mix_step(c, half, kv_ref, wo_ref, x_ref, ak_ref, av_ref, hk_ref, shift_ref, skip_ref,
              gate_ref, fwd_ref, inv_ref, uf_ref, hf_ref, held_ref, out_ref):
    cols = [pl.ds(pl.multiple_of((2 * c + n) * T, T), T) for n in range(2)]
    own = cols[half]
    fwd = fwd_ref[...]
    inv = inv_ref[...]
    taps = shift_ref[:, own]
    keys = ak_ref[:, own].astype(F32)
    shifted = keys * taps[KS - 1:KS]
    for t in range(KS - 2, -1, -1):
        shifted = jnp.concatenate([jnp.zeros((1, T), F32), shifted[:-1]], axis=0)
        shifted = shifted + keys * taps[t:t + 1]
    skip = skip_ref[:, own]

    def heads(odd, n, i):
        lanes = pl.ds(pl.multiple_of((2 * c + n + lax.shift_right_logical(c, 24 + i)) * T, T), T) if 'oh' in OPT else cols[n]
        return jnp.concatenate(
            [wo_ref[h * DH:(h + 1) * DH, lanes].astype(F32) for h in range(odd, H, 2)], axis=0)

    w = [_right_operand(i, functools.partial(heads, i=i)).astype(BF16) for i in range(7)]
    zero = _zero_word(c)
    before, u, z, parts, due = [], {}, {}, {}, {}

    def gate(j):
        return gate_ref[j * T:(j + 1) * T, :]

    def deliver(j, n, v):
        blk = slice(j * T, (j + 1) * T)
        if n == half and j // 8 == half:
            if (j, n) not in parts:
                parts[j, n] = v
                return
            v = v + parts.pop((j, n))
        elif half == 0:
            held_ref[c, blk, :] = v
            return
        else:
            v = v + held_ref[c, blk, :]
        out_ref[blk, cols[n]] = v.astype(BF16)

    def spectra(j):
        cur = lax.dot_general(fwd, hk_ref[own, j * T:(j + 1) * T], NT, preferred_element_type=F32)
        for f in range(NB):
            re, im = slice(16 * f, 16 * f + 8), slice(16 * f + 8, 16 * f + 16)
            if j == 0:
                hr, hi = cur[re], cur[im]
            elif f < NB // 2:
                hr, hi = cur[re] - before[-1][im], cur[im] + before[-1][re]
            else:
                hr, hi = cur[re] + before[-1][im], cur[im] - before[-1][re]
            hf_ref[j, re, :] = hr
            hf_ref[j, im, :] = hi
        before.append(cur)
        blk = slice(j * T, (j + 1) * T)
        u[j] = (shifted[blk] * av_ref[blk, own].astype(F32)).astype(BF16)
        uf_ref[j, :2 * T] = _mm(fwd, u[j])

    def products(i0, i1, start, step):
        base = 0 if 'sb' in OPT else lax.shift_right_logical(c, 8 + i0)
        rows = {i: [] for i in range(i0, i1)}
        for f in range(NB):
            re, im = slice(16 * f, 16 * f + 8), slice(16 * f + 8, 16 * f + 16)
            acc = {}
            for j in range(1 if 'nc' in OPT else i1):
                ur, ui = uf_ref[base + j, re, :], uf_ref[base + j, im, :]
                for i in range(max(i0, j), i1):
                    hr, hi = hf_ref[base + i - j, re, :], hf_ref[base + i - j, im, :]
                    pr, pi = ur * hr - ui * hi, ur * hi + ui * hr
                    acc[i] = (pr, pi) if j == 0 else (acc[i][0] + pr, acc[i][1] + pi)
            bits = None
            for i in range(i0, i1):
                rows[i] += acc[i]
                for v in acc[i]:
                    v = pltpu.bitcast(v, U32)
                    bits = v if bits is None else bits | v
            if 'nl' not in OPT: due[int(start + f * step)] = bits & zero
        for i in range(i0, i1):
            z[i] = jnp.concatenate(rows[i], axis=0).astype(BF16)

    def convolved(i):
        y = _mm(inv, z.pop(i)) + u.pop(i).astype(F32) * skip
        deliver(i, half, gate(i) * (x_ref[i * T:(i + 1) * T, own].astype(F32) * y))

    def product(e, i):
        r0 = _operand_row(e, i)
        left = [kv_ref[p, r0:r0 + W, :] for p in range(NP)]
        for p in range(0, NP, 4):
            at = 32 * i + 2 * p
            if any(at + k in due for k in range(8)):
                rows = [left[p][8 * k:8 * k + 8] for k in range(8)]
                left[p] = jnp.concatenate(
                    [v | due.pop(at + k) if at + k in due else v for k, v in enumerate(rows)],
                    axis=0)
        return _mm(_unpack(jnp.concatenate(left, axis=1)), w[i])

    groups = [((0, 2), (2, 4)), ((4, 6), (14, 16)), ((6, 8), (12, 14)), ((8, 10), (10, 12))]
    if half == 1:
        groups = [groups[0], groups[3], groups[2][::-1], groups[1][::-1]]
    t0 = eval(OPT.get('t0', '((64,3),(130,4))'))
    t1 = eval(OPT.get('t1', '((4,7.5),(130,5.8))'))
    sp = list(eval(OPT.get('sp', '6,8,10,12,14,16')))
    for step, pair in enumerate(groups):
        e = 4 * half + step
        m = []
        for k, (i0, i1) in enumerate(pair):
            if step == 0 and k == 0:
                for j in range(int(OPT.get('s0', 4))):
                    spectra(j)
            products(i0, i1, *(t0 if step == 0 else t1)[k])
            for _ in range(4 - k):
                m.append(product(e, len(m)))
                for j in range(len(before), sp.pop(0) if sp else 0):
                    spectra(j)
            for i in range(i0, i1):
                convolved(i)
        b = _combine(m)
        for odd in range(2):
            for n in range(2):
                deliver(2 * e + odd, n, (1.0 - gate(2 * e + odd)) * b[2 * odd + n])


def _kernel(x_hbm, ak_hbm, av_hbm, shift_in, hk_hbm, skip_in, c_hbm, wq_hbm, wuk_hbm,
            wuv_hbm, wo_hbm, gw_in, fwd_in, inv_in, out_hbm,
            x_ref, ak_ref, av_ref, hk_ref, c_ref, wq_ref, wkv_ref, wo_ref, cs_ref, xs_ref, gate_ref,
            kv_ref, shift_ref, skip_ref, fwd_ref, inv_ref, uf_ref, hf_ref, held_ref,
            out_ref, in_sem, out_sem):
    steps = NB // 2

    def pair_copy(w_hbm, p, dst, sem):
        return pltpu.make_async_copy(w_hbm.bitcast(U32).at[:, p, :], dst, sem)

    def wait_filled(buf, sem):
        pltpu.make_async_copy(buf, buf, sem).wait()

    def fetch_group(t):
        for b in range(4):
            pair_copy(wuk_hbm if t < 4 else wuv_hbm, (t % 4) * 4 + b,
                      wkv_ref.at[t * 4 + b], in_sem.at[8 + t]).start()

    first, rest = pl.ds(0, 2 * T), pl.ds(2 * T, S - 2 * T)
    plain = [(c_hbm, c_ref), (x_hbm.at[first], x_ref.at[first]),
             (x_hbm.at[rest], x_ref.at[rest]), (wo_hbm, wo_ref), (ak_hbm, ak_ref),
             (av_hbm, av_ref), (hk_hbm, hk_ref)]
    copies = [pltpu.make_async_copy(s, d, in_sem.at[k]) for k, (s, d) in enumerate(plain)]

    def fetch_ahead(t):
        if t == 0:
            copies[2].start()
        fetch_group(t + 2)
        if 1 <= t <= 4:
            for p in range(4 * t - 4, 4 * t):
                pair_copy(wq_hbm, p, wq_ref.at[p], in_sem.at[7]).start()

    copies[0].start()
    fetch_group(0)
    copies[1].start()
    fetch_group(1)
    shift_ref[...] = shift_in[...].astype(F32)
    skip_ref[...] = skip_in[...].astype(F32).reshape(1, DM)
    fwd_ref[...] = fwd_in[...].astype(BF16)
    inv_ref[...] = inv_in[...].astype(BF16)
    copies[0].wait()

    def left_step(e, carry):
        _store_left(c_ref, DC // 2, slice(0, DC // 2), cs_ref, e, 0, T)
        return carry

    lax.fori_loop(0, steps, left_step, 0)

    def kv_step(t, carry):
        for k in range(steps - 2):
            pl.when(t == k)(functools.partial(fetch_ahead, k))
        pl.when(t == 0)(copies[1].wait)
        pl.when(t == 1)(copies[2].wait)
        wait_filled(wkv_ref.at[pl.ds(t * 4, 4)], in_sem.at[8 + t])

        def meanwhile(b, k):
            done = _store_left(x_ref, DM // 2, slice(b * T, (b + 1) * T), xs_ref, t,
                               32 * k, 32 * k + 32)
            rows = pl.ds(pl.multiple_of(t * 2 * T + (4 * b + k) * 16, 16), 16)
            z = jnp.sum(x_ref[rows, :].astype(F32) * gw, axis=1, keepdims=True)
            g = jnp.broadcast_to(1.0 / (1.0 + jnp.exp(-z)), (16, T))
            gate_ref[rows, :] = g
            done += [pltpu.bitcast(g[:8], U32), pltpu.bitcast(g[8:], U32)]
            return functools.reduce(jnp.bitwise_or, done) & _zero_word(t)

        gw = gw_in[...].astype(F32).reshape(1, DM)
        _project_kv(t, cs_ref, wkv_ref, kv_ref, meanwhile)
        return carry

    if '1' in PH:
        lax.fori_loop(0, steps, kv_step, 0)

    for cp in copies[3:]:
        cp.start()
    wait_filled(wq_ref, in_sem.at[7])

    def pair_step(p, carry):
        _attend_pair(p, xs_ref, wq_ref, kv_ref)
        return carry

    if '2' in PH:
        lax.fori_loop(0, NP, pair_step, 0)

    for cp in copies[3:]:
        cp.wait()

    def out_copy(c):
        cols = pl.ds(pl.multiple_of(c * 2 * T, 2 * T), 2 * T)
        return pltpu.make_async_copy(out_ref.at[:, cols], out_hbm.at[:, cols], out_sem.at[c])

    for half in range(2):
        def mix_step(c, carry):
            _mix_step(c, half, kv_ref, wo_ref, x_ref, ak_ref, av_ref, hk_ref, shift_ref,
                      skip_ref, gate_ref, fwd_ref, inv_ref, uf_ref, hf_ref, held_ref,
                      out_ref)
            if half == 1:
                out_copy(c).start()
            return carry

        if '3' in PH and str(half) in OPT.get('half', '01'):
            lax.fori_loop(0, DM // (2 * T), mix_step, 0)
    for c in range(DM // (2 * T)):
        out_copy(c).wait()


@jax.jit
def pallas_gated_mix__ssm_conv_h3__compressed_kv_cla__prompt_kernel(
    A_q: jax.Array,
    A_k: jax.Array,
    A_v: jax.Array,
    A_shift_k: jax.Array,
    A_ssm_k: jax.Array,
    A_ssm_D: jax.Array,
    B_x: jax.Array,
    B_c_kv: jax.Array,
    B_w_q: jax.Array,
    B_w_uk: jax.Array,
    B_w_uv: jax.Array,
    B_w_o: jax.Array,
    gate_w: jax.Array,
):
    del B_x
    fwd, inv = _dft_matrices()
    hbm = pl.BlockSpec(memory_space=pl.ANY)
    vmem = pl.BlockSpec(memory_space=pltpu.VMEM)
    out = pl.pallas_call(
        _kernel,
        out_shape=jax.ShapeDtypeStruct((S, DM), BF16),
        in_specs=[hbm, hbm, hbm, vmem, hbm, vmem, hbm, hbm, hbm, hbm, hbm, vmem, vmem, vmem],
        out_specs=hbm,
        scratch_shapes=[
            pltpu.VMEM((S, DM), BF16),
            pltpu.VMEM((S, DM), BF16),
            pltpu.VMEM((S, DM), BF16),
            pltpu.VMEM((DM, S), BF16),
            pltpu.VMEM((S, DC), BF16),
            pltpu.VMEM((NP, DM, DH), U32),
            pltpu.VMEM((2 * NP, DC, DH), U32),
            pltpu.VMEM((H * DH, DM), BF16),
            pltpu.VMEM((7, S // 4, DC // 2), U32),
            pltpu.VMEM((7, S // 4, DM // 2), U32),
            pltpu.VMEM((S, T), F32),
            pltpu.VMEM((NP, 2 * S, DH), U32),
            pltpu.VMEM((KS, DM), F32),
            pltpu.VMEM((1, DM), F32),
            pltpu.VMEM((2 * T, T), BF16),
            pltpu.VMEM((T, 2 * T), BF16),
            pltpu.VMEM((NB, 2 * T + int(OPT.get('pu', 0)), T), F32),
            pltpu.VMEM((NB, 2 * T + int(OPT.get('ph_', 0)), T), F32),
            pltpu.VMEM((DM // (2 * T), S, T), F32),
            pltpu.VMEM((S, DM), BF16),
            pltpu.SemaphoreType.DMA((16,)),
            pltpu.SemaphoreType.DMA((DM // (2 * T),)),
        ],
        compiler_params=pltpu.CompilerParams(vmem_limit_bytes=127 * 2**20),
    )(
        A_q.reshape(S, DM), A_k.reshape(S, DM), A_v.reshape(S, DM), A_shift_k.T,
        A_ssm_k, A_ssm_D, B_c_kv.reshape(S, DC), B_w_q, B_w_uk, B_w_uv,
        B_w_o.reshape(H * DH, DM), gate_w, fwd, inv,
    )
    return out.reshape(1, S, DM)
```

```python
import functools

import jax
import jax.numpy as jnp
import numpy as np
from jax import lax
import jax.experimental.pallas as pl
import jax.experimental.pallas.tpu as pltpu

S = 2048
DM = 1024
H = 32
DH = 128
DC = 512
T = 128
NB = S // T
NP = H // 2
KS = 4
CH = 4
W = T // 2

F32 = jnp.float32
BF16 = jnp.bfloat16
U32 = jnp.uint32
NT = (((1,), (1,)), ((), ()))
import os
OPT = dict(a.split('=') for a in os.environ.get('OPT', '').split())
LEAD = int(OPT.get('lead', 12))
LAG = int(OPT.get('lag', 2))
PH = OPT.get('ph', '123')


def _dft_matrices():
    ks = np.concatenate([np.arange(0, T, 2), np.arange(1, T, 2)]).reshape(NB, 8)
    n = np.arange(T)
    theta = 2.0 * np.pi * (ks[:, :, None] + 0.5) * n[None, None, :] / (2 * T)
    fwd = np.concatenate([np.cos(theta), -np.sin(theta)], axis=1).reshape(2 * T, T)
    inv = fwd.T / T
    return fwd.astype(np.float32), inv.astype(np.float32)


def _mm(a, b):
    return jnp.dot(a, b, preferred_element_type=F32)


def _pack(v):
    return pltpu.pack_elementwise([v[:W], v[W:]], packed_dtype=BF16)


def _halves(words):
    return [pltpu.unpack_elementwise(words, index=i, packed_dtype=BF16, unpacked_dtype=F32)
            for i in range(2)]


def _unpack(words):
    return pltpu.bitcast(words, BF16)


def _after(v, earlier):
    return jnp.maximum(v, jnp.minimum(earlier, v))


def _zero_word(i):
    return jnp.full((8, T), lax.shift_right_logical(i, 8), jnp.int32).astype(U32)


def _left(a11, a12, a21, a22):
    return [a11 + a22, a21 + a22, a11, a22, a11 + a12, a21 - a11, a12 - a22]


def _right_operand(i, b):
    first, sign, second = (
        ((0, 0), 1, (1, 1)), ((0, 0), 0, None), ((0, 1), -1, (1, 1)), ((1, 0), -1, (0, 0)),
        ((1, 1), 0, None), ((0, 0), 1, (0, 1)), ((1, 0), 1, (1, 1)))[i]
    if sign == 0:
        return b(*first)
    return b(*first) + b(*second) if sign > 0 else b(*first) - b(*second)


def _combine(m):
    return (m[0] + m[3] - m[4] + m[6], m[2] + m[4], m[1] + m[3], m[0] - m[1] + m[2] + m[5])


def _pair_weights(words):
    half = words.shape[0] // 2
    heads = _halves(words)
    return [_right_operand(i, lambda r, c: heads[c][r * half:(r + 1) * half]).astype(BF16)
            for i in range(7)]


def _store_left(src_ref, half, cols, dst_ref, e, r0, r1):
    parts = []
    for j in range(2):
        for c0 in (0, half):
            v = src_ref[pl.ds(pl.multiple_of((2 * e + j) * T + r0, 32), r1 - r0),
                        c0 + cols.start:c0 + cols.stop]
            parts.append(_halves(pltpu.bitcast(v, U32)))
    stored = []
    for odd in range(2):
        rows = pl.ds(pl.multiple_of(e * W + odd * (W // 2) + r0 // 4, 8), (r1 - r0) // 4)
        for i, v in enumerate(_left(*[part[odd] for part in parts])):
            stored.append(pltpu.bitcast(v.astype(BF16), U32))
            dst_ref[i, rows, cols] = stored[-1]
    return stored


def _project_kv(t, cs_ref, wkv_ref, kv_ref, meanwhile):
    base = pl.multiple_of((t >> 2) * S, S)
    for b in range(4):
        w = _pair_weights(wkv_ref[t * 4 + b])
        pair = (t & 3) * 4 + b
        for e in range(0, NB // 2, 2):
            left = [cs_ref[i, e * W:(e + 2) * W, :] for i in range(7)]
            at = int(OPT.get('mw', 2))
            tie = meanwhile(b, e // 2)
            left[at] = jnp.concatenate(
                [left[at][:8] | jnp.concatenate([tie, tie], axis=1), left[at][8:]], axis=0)
            c = _combine([_mm(_unpack(left[i]), w[i]) for i in range(7)])
            for k in range(2):
                for odd in range(2):
                    for head in range(2):
                        r0 = head * (S // 2) + (2 * (e + k) + odd) * W
                        kv_ref[pair, pl.ds(base + r0, W), :] = _pack(
                            c[2 * odd + head][k * T:(k + 1) * T])


def _operand_row(e, i):
    return (i // 2) * (S // 2) + (2 * e + i % 2) * W


def _attend_pair(p, xs_ref, wq_ref, kv_ref):
    row = lax.broadcasted_iota(jnp.int32, (T, T), 0)
    col = lax.broadcasted_iota(jnp.int32, (T, T), 1)
    causal = col <= jnp.where(row < W, 2 * row, 2 * (row - W) + 1)
    scale = DH ** -0.5 * np.log2(np.e)
    w = _pair_weights(wq_ref[p])
    q, s, ctx, sums, done = {}, {}, {}, [], []
    zero = lax.shift_right_logical(p, 8)

    def chunks(r):
        return [(j, min(j + CH, r + 1)) for j in range(0, r + 1, CH)]

    def tiles(region, j0, j1):
        r0 = region * (S // 2)
        return _unpack(kv_ref[p, r0 + j0 * W:r0 + j1 * W, :])

    def queries(e):
        c = _combine([_mm(_unpack(xs_ref[i, e * W:(e + 1) * W, :]), w[i]) for i in range(7)])
        for odd in range(2):
            for head in range(2):
                q[2 * e + odd, head] = (c[2 * odd + head] * scale).astype(BF16)

    def scores(r, head):
        parts, m = [], None
        for j0, j1 in chunks(r):
            d = lax.dot_general(q[r, head], tiles(head, j0, j1), NT, preferred_element_type=F32)
            for j in range(j0, j1):
                t = d[:, (j - j0) * T:(j - j0 + 1) * T]
                if j == r:
                    t = jnp.where(causal, t, -1e9)
                parts.append(t)
                m = t if m is None else jnp.maximum(m, t)
        s[r, head] = parts, jnp.max(m, axis=1, keepdims=True)

    def context(r, head):
        parts, top = s.pop((r, head))
        top = jnp.broadcast_to(top, (T, T))
        l, o = None, None
        for j0, j1 in chunks(r):
            m = top
            if 'l' in OPT.get('pin', 'x') and len(sums) >= LAG:
                m = _after(m, sums[-LAG])
            if 'o' in OPT.get('pin', 'x') and j0 == 0 and len(done) >= 2:
                m = _after(m, done[-2])
            ps = [jnp.exp2(parts[j] - m) for j in range(j0, j1)]
            G = int(OPT.get('g', 4))
            for k in range(0, len(ps), G):
                t = ps[k]
                for e in ps[k + 1:k + G]:
                    t = t + e
                if len(ps[k:k + G]) > 1:
                    last = min(k + G, len(ps)) - 1
                    ps[last] = jnp.minimum(ps[last], t)
                l = t if l is None else l + t
            sums.append(l)
            if 'p' in OPT.get('pin', 'x'):
                ps[-1] = jnp.minimum(ps[-1], l)
            if 'q' in OPT.get('pin', 'x'):
                ps[0] = jnp.minimum(ps[0], l)
            e = ps[0] if len(ps) == 1 else jnp.concatenate(ps, axis=1)
            d = _mm(e.astype(BF16), tiles(2 + head, j0, j1))
            o = d if o is None else o + d
        l = jnp.sum(l, axis=1, keepdims=True)
        inv = pltpu.reciprocal(l, approx=True)
        inv = inv * (2.0 - l * inv)
        ctx[r, head] = o * inv
        done.append(ctx[r, head])

    def emit(e):
        ops = _left(*[ctx.pop((2 * e + odd, head)) for odd in range(2) for head in range(2)])
        for i in range(7):
            r0 = _operand_row(e, i)
            if 'z' not in OPT:
                kv_ref[p, r0:r0 + W, :] = _pack(ops[i])
            else:
                kv_ref[p, pl.ds(pl.multiple_of(zero * W + r0, W), W), :] = _pack(ops[i])

    todo = [(r, head) for r in range(NB - 1, -1, -1) for head in range(2)]
    if 'seq' in OPT:
        todo = [(r, head) for head in range(2) for r in range(NB - 1, -1, -1)]
    if 'one' in OPT:
        todo = [(r, head) for head in range(1) for r in range(NB - 1, -1, -1)]
    next_q, next_s, lead, ready = NB // 2 - 1, 0, 0, []
    for r, head in todo:
        while next_s < len(todo) and lead < LEAD + r + 1:
            rs, hs = todo[next_s]
            while next_q >= 0 and next_q >= rs // 2 - 1:
                queries(next_q)
                next_q -= 1
            scores(rs, hs)
            lead += rs + 1
            next_s += 1
        context(r, head)
        lead -= r + 1
        ready.append(r // 2 if head == 1 and r % 2 == 0 else None)
        if len(ready) > int(OPT.get('ed', 1)):
            e = ready.pop(0)
            if e is not None:
                emit(e)
    for e in ready:
        if e is not None:
            emit(e)


def _mix_step(c, half, kv_ref, wo_ref, x_ref, ak_ref, av_ref, hk_ref, shift_ref, skip_ref,
              gate_ref, fwd_ref, inv_ref, uf_ref, hf_ref, held_ref, out_ref):
    tile = 2 * c + half
    own = pl.ds(pl.multiple_of(tile * T, T), T)
    fwd = fwd_ref[...]
    inv = inv_ref[...]
    taps = shift_ref[:, own].astype(F32)
    keys = ak_ref[tile].astype(F32)
    shifted = keys * taps[KS - 1:KS]
    for t in range(KS - 2, -1, -1):
        shifted = jnp.concatenate([jnp.zeros((1, T), F32), shifted[:-1]], axis=0)
        shifted = shifted + keys * taps[t:t + 1]
    skip = skip_ref[pl.ds(pl.multiple_of(c * 2 * T, 2 * T), 2 * T)].astype(F32).reshape(1, 2 * T)
    skip = skip[:, half * T:(half + 1) * T]

    def heads(odd, n):
        return jnp.concatenate([wo_ref[2 * c + n, h * DH:(h + 1) * DH, :].astype(F32)
                                for h in range(odd, H, 2)], axis=0)

    w = [_right_operand(i, heads).astype(BF16) for i in range(7)]
    zero = _zero_word(c)
    before, u, z, parts, due = [], {}, {}, {}, {}

    def gate(j):
        return gate_ref[j * T:(j + 1) * T, :]

    def deliver(j, n, v):
        blk = slice(j * T, (j + 1) * T)
        if n == half and j // 8 == half:
            if (j, n) not in parts:
                parts[j, n] = v
                return
            v = v + parts.pop((j, n))
        elif half == 0:
            held_ref[c, blk, :] = v
            return
        else:
            v = v + held_ref[c, blk, :]
        out_ref[2 * c + n, blk, :] = v.astype(BF16)

    def spectra(j):
        cur = lax.dot_general(fwd, hk_ref[own, j * T:(j + 1) * T], NT, preferred_element_type=F32)
        for f in range(NB):
            re, im = slice(16 * f, 16 * f + 8), slice(16 * f + 8, 16 * f + 16)
            if j == 0:
                hr, hi = cur[re], cur[im]
            elif f < NB // 2:
                hr, hi = cur[re] - before[-1][im], cur[im] + before[-1][re]
            else:
                hr, hi = cur[re] + before[-1][im], cur[im] - before[-1][re]
            hf_ref[j, re, :] = hr
            hf_ref[j, im, :] = hi
        before.append(cur)
        blk = slice(j * T, (j + 1) * T)
        u[j] = (shifted[blk] * av_ref[tile, blk, :].astype(F32)).astype(BF16)
        uf_ref[j, :2 * T] = _mm(fwd, u[j])

    def products(i0, i1, start, step):
        base = 0 if 'sb' in OPT else lax.shift_right_logical(c, 8 + i0)
        rows = {i: [] for i in range(i0, i1)}
        for f in range(NB):
            re, im = slice(16 * f, 16 * f + 8), slice(16 * f + 8, 16 * f + 16)
            acc = {}
            for j in range(1 if 'nc' in OPT else i1):
                bu = 0 if 'su' in OPT else base
                ur, ui = uf_ref[bu + j, re, :], uf_ref[bu + j, im, :]
                for i in range(max(i0, j), i1):
                    bh = 0
                    hr, hi = hf_ref[bh + i - j, re, :], hf_ref[bh + i - j, im, :]
                    pr, pi = ur * hr - ui * hi, ur * hi + ui * hr
                    acc[i] = (pr, pi) if j == 0 else (acc[i][0] + pr, acc[i][1] + pi)
            bits = None
            for i in range(i0, i1):
                rows[i] += acc[i]
                for v in acc[i]:
                    v = pltpu.bitcast(v, U32)
                    bits = v if bits is None else bits | v
            if 'nl' not in OPT: due[int(start + f * step)] = bits & zero
        for i in range(i0, i1):
            z[i] = jnp.concatenate(rows[i], axis=0).astype(BF16)

    def convolved(i):
        y = _mm(inv, z.pop(i)) + u.pop(i).astype(F32) * skip
        deliver(i, half, gate(i) * (x_ref[i * T:(i + 1) * T, own].astype(F32) * y))

    def product(e, i):
        r0 = _operand_row(e, i)
        left = [kv_ref[p, r0:r0 + W, :] for p in range(NP)]
        for p in range(0, NP, 4):
            at = 32 * i + 2 * p
            if any(at + k in due for k in range(8)):
                rows = [left[p][8 * k:8 * k + 8] for k in range(8)]
                left[p] = jnp.concatenate(
                    [v | due.pop(at + k) if at + k in due else v for k, v in enumerate(rows)],
                    axis=0)
        return _mm(_unpack(jnp.concatenate(left, axis=1)), w[i])

    groups = [((0, 2), (2, 4)), ((4, 6), (14, 16)), ((6, 8), (12, 14)), ((8, 10), (10, 12))]
    if half == 1:
        groups = [groups[0], groups[3], groups[2][::-1], groups[1][::-1]]
    t0 = eval(OPT.get('t0', '((64,3),(130,4))'))
    t1 = eval(OPT.get('t1', '((4,7.5),(130,5.8))'))
    sp = list(eval(OPT.get('sp', '6,8,10,12,14,16')))
    for step, pair in enumerate(groups):
        e = 4 * half + step
        m = []
        for k, (i0, i1) in enumerate(pair):
            if step == 0 and k == 0:
                for j in range(int(OPT.get('s0', 4))):
                    spectra(j)
            products(i0, i1, *(t0 if step == 0 else t1)[k])
            for _ in range(4 - k):
                m.append(product(e, len(m)))
                for j in range(len(before), sp.pop(0) if sp else 0):
                    spectra(j)
            for i in range(i0, i1):
                convolved(i)
        b = _combine(m)
        for odd in range(2):
            for n in range(2):
                deliver(2 * e + odd, n, (1.0 - gate(2 * e + odd)) * b[2 * odd + n])


def _kernel(x_hbm, ak_hbm, av_hbm, shift_hbm, hk_hbm, skip_hbm, c_hbm, wq_hbm, wuk_hbm,
            wuv_hbm, wo_hbm, gw_hbm, fwd_hbm, inv_hbm, out_hbm,
            x_ref, ak_ref, av_ref, hk_ref, c_ref, wq_ref, wkv_ref, wo_ref, cs_ref, xs_ref,
            gate_ref, kv_ref, uf_ref, hf_ref, held_ref, out_ref, fwd_ref, inv_ref, shift_ref,
            skip_ref, gw_ref, in_sem, out_sem):
    steps = NB // 2

    def pair_copy(w_hbm, p, dst, sem):
        return pltpu.make_async_copy(w_hbm.bitcast(U32).at[:, p, :], dst, sem)

    def wait_filled(buf, sem):
        pltpu.make_async_copy(buf, buf, sem).wait()

    def fetch_group(t):
        for b in range(4):
            pair_copy(wuk_hbm if t < 4 else wuv_hbm, (t % 4) * 4 + b,
                      wkv_ref.at[t * 4 + b], in_sem.at[t]).start()

    def c_copy(e):
        rows = pl.ds(pl.multiple_of(e * 2 * T, 2 * T), 2 * T)
        return pltpu.make_async_copy(c_hbm.at[rows], c_ref.at[rows], in_sem.at[steps + e])

    wq_sem = in_sem.at[2 * steps]
    first, rest = pl.ds(0, 2 * T), pl.ds(2 * T, S - 2 * T)
    plain = [(gw_hbm, gw_ref), (x_hbm.at[first], x_ref.at[first]),
             (x_hbm.at[rest], x_ref.at[rest]), (hk_hbm, hk_ref), (shift_hbm, shift_ref),
             (skip_hbm, skip_ref), (fwd_hbm, fwd_ref), (inv_hbm, inv_ref)]
    tiled = [(wo_hbm, wo_ref), (ak_hbm, ak_ref), (av_hbm, av_ref)]
    tile_sem = 2 * steps + 1 + len(plain)
    gw_copy, x_first, x_rest, *late = [
        pltpu.make_async_copy(src, dst, in_sem.at[2 * steps + 1 + k])
        for k, (src, dst) in enumerate(plain)]

    def fetch_ahead(t):
        if t == 0:
            x_rest.start()
        fetch_group(t + 1)
        if 1 <= t <= 4:
            for p in range(4 * t - 4, 4 * t):
                pair_copy(wq_hbm, p, wq_ref.at[p], wq_sem).start()

    gw_copy.start()
    fetch_group(0)
    x_first.start()
    for e in range(steps):
        c_copy(e).start()

    def left_step(e, carry):
        c_copy(e).wait()
        _store_left(c_ref, DC // 2, slice(0, DC // 2), cs_ref, e, 0, T)
        return carry

    lax.fori_loop(0, steps, left_step, 0)
    gw_copy.wait()
    x_first.wait()

    def kv_step(t, carry):
        for k in range(steps - 1):
            pl.when(t == k)(functools.partial(fetch_ahead, k))
        pl.when(t == 1)(x_rest.wait)
        wait_filled(wkv_ref.at[pl.ds(t * 4, 4)], in_sem.at[t])

        def meanwhile(b, k):
            done = _store_left(x_ref, DM // 2, slice(b * T, (b + 1) * T), xs_ref, t,
                               32 * k, 32 * k + 32)
            rows = pl.ds(pl.multiple_of(t * 2 * T + (4 * b + k) * 16, 16), 16)
            z = jnp.sum(x_ref[rows, :].astype(F32) * gw, axis=1, keepdims=True)
            g = jnp.broadcast_to(1.0 / (1.0 + jnp.exp(-z)), (16, T))
            gate_ref[rows, :] = g
            done += [pltpu.bitcast(g[:8], U32), pltpu.bitcast(g[8:], U32)]
            return functools.reduce(jnp.bitwise_or, done) & _zero_word(t)

        gw = gw_ref[...].astype(F32).reshape(1, DM)
        _project_kv(t, cs_ref, wkv_ref, kv_ref, meanwhile)
        return carry

    if '1' in PH:
        lax.fori_loop(0, steps, kv_step, 0)

    for cp in late:
        cp.start()
    wait_filled(wq_ref, wq_sem)

    def pair_step(p, carry):
        @pl.when(p < DM // T)
        def _():
            cols = pl.ds(pl.multiple_of(p * T, T), T)
            for k, (src, dst) in enumerate(tiled):
                pltpu.make_async_copy(src.at[:, cols], dst.at[p], in_sem.at[tile_sem + k]).start()

        _attend_pair(p, xs_ref, wq_ref, kv_ref)
        return carry

    if '2' in PH:
        lax.fori_loop(0, NP, pair_step, 0)

    for cp in late:
        cp.wait()
    for k, (_, dst) in enumerate(tiled):
        wait_filled(dst, in_sem.at[tile_sem + k])

    def out_copy(c, part):
        rows, n = ((pl.ds(0, S // 2), 0), (pl.ds(S // 2, S // 2), 0), (pl.ds(0, S), 1))[part]
        cols = pl.ds(pl.multiple_of((2 * c + n) * T, T), T)
        return pltpu.make_async_copy(
            out_ref.at[2 * c + n, rows], out_hbm.at[rows, cols], out_sem.at[3 * c + part])

    for half in range(2):
        def mix_step(c, carry):
            _mix_step(c, half, kv_ref, wo_ref, x_ref, ak_ref, av_ref, hk_ref, shift_ref,
                      skip_ref, gate_ref, fwd_ref, inv_ref, uf_ref, hf_ref, held_ref, out_ref)
            for part in ((0,), (1, 2))[half]:
                out_copy(c, part).start()
            return carry

        if '3' in PH and str(half) in OPT.get('half', '01'):
            lax.fori_loop(0, DM // (2 * T), mix_step, 0)
    for c in range(DM // (2 * T)):
        for part in range(3):
            out_copy(c, part).wait()


@jax.jit
def pallas_gated_mix__ssm_conv_h3__compressed_kv_cla__prompt_kernel(
    A_q: jax.Array,
    A_k: jax.Array,
    A_v: jax.Array,
    A_shift_k: jax.Array,
    A_ssm_k: jax.Array,
    A_ssm_D: jax.Array,
    B_x: jax.Array,
    B_c_kv: jax.Array,
    B_w_q: jax.Array,
    B_w_uk: jax.Array,
    B_w_uv: jax.Array,
    B_w_o: jax.Array,
    gate_w: jax.Array,
):
    del B_x
    fwd, inv = _dft_matrices()
    hbm = pl.BlockSpec(memory_space=pl.ANY)
    out = pl.pallas_call(
        _kernel,
        out_shape=jax.ShapeDtypeStruct((S, DM), BF16),
        in_specs=[hbm] * 14,
        out_specs=hbm,
        scratch_shapes=[
            pltpu.VMEM((S, DM), BF16),
            pltpu.VMEM((DM // T, S, T), BF16),
            pltpu.VMEM((DM // T, S, T), BF16),
            pltpu.VMEM((DM, S), BF16),
            pltpu.VMEM((S, DC), BF16),
            pltpu.VMEM((NP, DM, DH), U32),
            pltpu.VMEM((2 * NP, DC, DH), U32),
            pltpu.VMEM((DM // T, H * DH, T), BF16),
            pltpu.VMEM((7, S // 4, DC // 2), U32),
            pltpu.VMEM((7, S // 4, DM // 2), U32),
            pltpu.VMEM((S + 8 * int(OPT.get('p1', 0)), T), F32),
            pltpu.VMEM((NP, 2 * S, DH), U32),
            pltpu.VMEM((NB, 2 * T, T), F32),
            pltpu.VMEM((NB, 2 * T, T), F32),
            pltpu.VMEM((DM // (2 * T), S, T), F32),
            pltpu.VMEM((DM // T, S, T), BF16),
            pltpu.VMEM((2 * T, T), BF16),
            pltpu.VMEM((T, 2 * T), BF16),
            pltpu.VMEM((KS, DM), BF16),
            pltpu.VMEM((DM,), BF16),
            pltpu.VMEM((DM,), BF16),
            pltpu.SemaphoreType.DMA((NB + 12,)),
            pltpu.SemaphoreType.DMA((3 * DM // (2 * T),)),
        ],
        compiler_params=pltpu.CompilerParams(vmem_limit_bytes=127 * 2**20),
    )(
        A_q.reshape(S, DM), A_k.reshape(S, DM), A_v.reshape(S, DM), A_shift_k.T,
        A_ssm_k, A_ssm_D, B_c_kv.reshape(S, DC), B_w_q, B_w_uk, B_w_uv,
        B_w_o.reshape(H * DH, DM), gate_w, fwd.astype(BF16), inv.astype(BF16),
    )
    return out.reshape(1, S, DM)
```

```python
import functools

import jax
import jax.numpy as jnp
import numpy as np
from jax import lax
import jax.experimental.pallas as pl
import jax.experimental.pallas.tpu as pltpu

S = 2048
DM = 1024
H = 32
DH = 128
DC = 512
KS = 4
T = 128
W = T // 2
NB = S // T
NP = H // 2
NC = DM // T
LEAD = 12

F32 = jnp.float32
BF16 = jnp.bfloat16
U32 = jnp.uint32
NT = (((1,), (1,)), ((), ()))
LOG2E = float(np.log2(np.e))


def _dft_matrices():
    ks = np.concatenate([np.arange(0, T, 2), np.arange(1, T, 2)]).reshape(NB, 8)
    n = np.arange(T)
    theta = 2.0 * np.pi * (ks[:, :, None] + 0.5) * n[None, None, :] / (2 * T)
    fwd = np.concatenate([np.cos(theta), -np.sin(theta)], axis=1).reshape(2 * T, T)
    return fwd.astype(BF16), (fwd.T / T).astype(BF16)


def _mm(a, b):
    return jnp.dot(a, b, preferred_element_type=F32)


def _pack(v):
    return pltpu.pack_elementwise([v[:W], v[W:]], packed_dtype=BF16)


def _unpack(words):
    return pltpu.bitcast(words, BF16)


def _halves(words):
    return [pltpu.unpack_elementwise(words, index=i, packed_dtype=BF16, unpacked_dtype=F32)
            for i in range(2)]


def _zero(i):
    return lax.shift_right_logical(i, 8)


def _zero_after(values, i):
    bits = functools.reduce(jnp.bitwise_or, [pltpu.bitcast(v, U32) for v in values])
    return bits & jnp.full(bits.shape, _zero(i), jnp.int32).astype(U32)


def _left(a11, a12, a21, a22):
    return [a11 + a22, a21 + a22, a11, a22, a11 + a12, a21 - a11, a12 - a22]


def _right(b11, b12, b21, b22):
    return [b11 + b22, b11, b12 - b22, b21 - b11, b22, b11 + b12, b21 + b22]


def _combine(m):
    return (m[0] + m[3] - m[4] + m[6], m[2] + m[4], m[1] + m[3], m[0] - m[1] + m[2] + m[5])


def _pair_weights(words):
    half = words.shape[0] // 2
    first, second = _halves(words)
    return [v.astype(BF16)
            for v in _right(first[:half], second[:half], first[half:], second[half:])]


def _store_left(src_ref, cols, dst_ref, e, r0, r1):
    half = src_ref.shape[1] // 2
    parts = []
    for j in range(2):
        rows = pl.ds(pl.multiple_of((2 * e + j) * T + r0, 32), r1 - r0)
        for c0 in (0, half):
            v = src_ref[rows, c0 + cols.start:c0 + cols.stop]
            parts.append(_halves(pltpu.bitcast(v, U32)))
    stored = []
    for odd in range(2):
        rows = pl.ds(pl.multiple_of(e * W + odd * (W // 2) + r0 // 4, 8), (r1 - r0) // 4)
        for i, v in enumerate(_left(*[part[odd] for part in parts])):
            stored.append(pltpu.bitcast(v.astype(BF16), U32))
            dst_ref[i, rows, cols] = stored[-1]
    return stored


def _project_kv(t, cs_ref, wkv_ref, kv_ref, meanwhile):
    base = pl.multiple_of((t >> 2) * S, S)
    for b in range(4):
        w = _pair_weights(wkv_ref[t * 4 + b])
        pair = (t & 3) * 4 + b
        for e in range(0, NB // 2, 2):
            left = [cs_ref[i, e * W:(e + 2) * W, :] for i in range(7)]
            zero = meanwhile(b, e // 2)
            left[2] = jnp.concatenate(
                [left[2][:8] | jnp.concatenate([zero, zero], axis=1), left[2][8:]], axis=0)
            c = _combine([_mm(_unpack(left[i]), w[i]) for i in range(7)])
            for k in range(2):
                for odd in range(2):
                    for head in range(2):
                        r0 = head * (S // 2) + (2 * (e + k) + odd) * W
                        kv_ref[pair, pl.ds(base + r0, W), :] = _pack(
                            c[2 * odd + head][k * T:(k + 1) * T])


def _operand_row(e, i):
    return (i // 2) * (S // 2) + (2 * e + i % 2) * W


def _attend_pair(p, xs_ref, wq_ref, kv_ref):
    row = lax.broadcasted_iota(jnp.int32, (T, T), 0)
    col = lax.broadcasted_iota(jnp.int32, (T, T), 1)
    causal = col <= jnp.where(row < W, 2 * row, 2 * (row - W) + 1)
    w = _pair_weights(wq_ref[p])
    q, s, ctx = {}, {}, {}

    def blocks(region, n):
        r0 = region * (S // 2)
        return _unpack(kv_ref[p, r0:r0 + n * W, :])

    def queries(e):
        c = _combine([_mm(_unpack(xs_ref[i, e * W:(e + 1) * W, :]), w[i]) for i in range(7)])
        for odd in range(2):
            for head in range(2):
                q[2 * e + odd, head] = (c[2 * odd + head] * (DH ** -0.5 * LOG2E)).astype(BF16)

    def scores(r, head):
        d = lax.dot_general(q.pop((r, head)), blocks(head, r + 1), NT,
                            preferred_element_type=F32)
        tiles = [d[:, j * T:(j + 1) * T] for j in range(r + 1)]
        tiles[r] = jnp.where(causal, tiles[r], -1e9 * LOG2E)
        top = jnp.max(functools.reduce(jnp.maximum, tiles), axis=1, keepdims=True)
        s[r, head] = tiles, top

    def context(r, head):
        tiles, top = s.pop((r, head))
        top = jnp.broadcast_to(top, (T, T))
        tiles = [jnp.exp2(v - top) for v in tiles]
        total = functools.reduce(jnp.add, tiles)
        if r > 0:
            tiles[r] = jnp.minimum(tiles[r], total)
        o = _mm(jnp.concatenate(tiles, axis=1).astype(BF16), blocks(2 + head, r + 1))
        total = jnp.sum(total, axis=1, keepdims=True)
        inv = pltpu.reciprocal(total, approx=True)
        inv = inv * (2.0 - total * inv)
        ctx[r, head] = o * inv

    def emit(e):
        ops = _left(*[ctx.pop((2 * e + odd, head)) for odd in range(2) for head in range(2)])
        for i in range(7):
            r0 = _operand_row(e, i)
            kv_ref[p, r0:r0 + W, :] = _pack(ops[i])

    order = [(r, head) for r in range(NB - 1, -1, -1) for head in range(2)]
    scored, lead = 0, 0
    for r, head in order:
        while scored < len(order) and lead < LEAD + r + 1:
            if order[scored] not in q:
                queries(order[scored][0] // 2)
            scores(*order[scored])
            lead += order[scored][0] + 1
            scored += 1
        context(r, head)
        lead -= r + 1
        if head == 1 and r % 2 == 0:
            emit(r // 2)


def _mix_step(c, half, kv_ref, wo_ref, x_ref, ak_ref, av_ref, hk_ref, shift_ref, skip_ref,
              gate_ref, fwd_ref, inv_ref, uf_ref, hf_ref, held_ref, out_ref):
    tile = 2 * c + half
    own = pl.ds(pl.multiple_of(tile * T, T), T)
    fwd = fwd_ref[...]
    inv = inv_ref[...]
    skip = skip_ref[pl.ds(pl.multiple_of(c * 2 * T, 2 * T), 2 * T)]
    skip = skip.astype(F32).reshape(1, 2 * T)[:, half * T:(half + 1) * T]

    taps = shift_ref[:, own].astype(F32)
    keys = ak_ref[tile].astype(F32)
    shifted = keys * taps[KS - 1:KS]
    for t in range(KS - 2, -1, -1):
        shifted = jnp.concatenate([jnp.zeros((1, T), F32), shifted[:-1]], axis=0)
        shifted = shifted + keys * taps[t:t + 1]

    def heads(odd, n):
        return jnp.concatenate([wo_ref[2 * c + n, h * DH:(h + 1) * DH, :].astype(F32)
                                for h in range(odd, H, 2)], axis=0)

    w = [v.astype(BF16) for v in _right(heads(0, 0), heads(0, 1), heads(1, 0), heads(1, 1))]
    plain, u, z, parts, due = [], {}, {}, {}, {}

    def deliver(j, n, v):
        blk = slice(j * T, (j + 1) * T)
        if n == half and j // 8 == half:
            if (j, n) not in parts:
                parts[j, n] = v
                return
            v = v + parts.pop((j, n))
        elif half == 0:
            held_ref[c, blk, :] = v
            return
        else:
            v = v + held_ref[c, blk, :]
        out_ref[2 * c + n, blk, :] = v.astype(BF16)

    def spectra(j):
        blk = slice(j * T, (j + 1) * T)
        cur = lax.dot_general(fwd, hk_ref[own, blk], NT, preferred_element_type=F32)
        for f in range(NB):
            re, im = slice(16 * f, 16 * f + 8), slice(16 * f + 8, 16 * f + 16)
            if j == 0:
                hr, hi = cur[re], cur[im]
            elif f < NB // 2:
                hr, hi = cur[re] - plain[-1][im], cur[im] + plain[-1][re]
            else:
                hr, hi = cur[re] + plain[-1][im], cur[im] - plain[-1][re]
            hf_ref[j, re, :] = hr
            hf_ref[j, im, :] = hi
        plain.append(cur)
        u[j] = (shifted[blk] * av_ref[tile, blk, :].astype(F32)).astype(BF16)
        uf_ref[j] = _mm(fwd, u[j])

    def multiply(i0, start, step):
        base = _zero(c >> i0)
        rows = {i0: [], i0 + 1: []}
        for f in range(NB):
            re, im = slice(16 * f, 16 * f + 8), slice(16 * f + 8, 16 * f + 16)
            acc = {}
            for j in range(i0 + 2):
                ur, ui = uf_ref[base + j, re, :], uf_ref[base + j, im, :]
                for i in range(max(i0, j), i0 + 2):
                    hr, hi = hf_ref[i - j, re, :], hf_ref[i - j, im, :]
                    pr, pi = ur * hr - ui * hi, ur * hi + ui * hr
                    acc[i] = (pr, pi) if j == 0 else (acc[i][0] + pr, acc[i][1] + pi)
            for i in rows:
                rows[i] += acc[i]
            due[int(start + f * step)] = _zero_after(acc[i0] + acc[i0 + 1], c)
        for i in rows:
            z[i] = jnp.concatenate(rows[i], axis=0).astype(BF16)

    def convolved(i):
        blk = slice(i * T, (i + 1) * T)
        y = _mm(inv, z.pop(i)) + u.pop(i).astype(F32) * skip
        deliver(i, half, gate_ref[blk, :] * (x_ref[blk, own].astype(F32) * y))

    def product(e, i):
        r0 = _operand_row(e, i)
        left = [kv_ref[p, r0:r0 + W, :] for p in range(NP)]
        for p in range(0, NP, 4):
            at = 32 * i + 2 * p
            if any(at + k in due for k in range(8)):
                rows = [left[p][8 * k:8 * k + 8] for k in range(8)]
                left[p] = jnp.concatenate(
                    [v | due.pop(at + k) if at + k in due else v for k, v in enumerate(rows)],
                    axis=0)
        return _mm(_unpack(jnp.concatenate(left, axis=1)), w[i])

    groups = [(0, 2), (4, 14), (6, 12), (8, 10)] if half == 0 else [
        (0, 2), (8, 10), (12, 6), (14, 4)]
    for j in range(4):
        spectra(j)
    for step, pair in enumerate(groups):
        e = 4 * half + step
        pace = ((64, 3), (130, 4)) if step == 0 else ((4, 7.5), (130, 5.8))
        m = []
        for k, i0 in enumerate(pair):
            multiply(i0, *pace[k])
            for _ in range(4 - k):
                m.append(product(e, len(m)))
                for j in range(len(plain), min(len(plain) + 2, NB)):
                    spectra(j)
            convolved(i0)
            convolved(i0 + 1)
        b = _combine(m)
        for odd in range(2):
            j = 2 * e + odd
            for n in range(2):
                deliver(j, n, (1.0 - gate_ref[j * T:(j + 1) * T, :]) * b[2 * odd + n])


def _kernel(x_hbm, ak_hbm, av_hbm, shift_hbm, hk_hbm, skip_hbm, c_hbm, wq_hbm, wuk_hbm,
            wuv_hbm, wo_hbm, gw_hbm, fwd_hbm, inv_hbm, out_hbm,
            x_ref, ak_ref, av_ref, hk_ref, c_ref, wq_ref, wkv_ref, wo_ref, cs_ref, xs_ref,
            gate_ref, kv_ref, uf_ref, hf_ref, held_ref, out_ref, fwd_ref, inv_ref, shift_ref,
            skip_ref, gw_ref, in_sem, out_sem):
    steps = NB // 2
    wq_sem = in_sem.at[2 * steps]
    first, rest = pl.ds(0, 2 * T), pl.ds(2 * T, S - 2 * T)
    whole = [(gw_hbm, gw_ref), (x_hbm.at[first], x_ref.at[first]),
             (x_hbm.at[rest], x_ref.at[rest]), (hk_hbm, hk_ref), (shift_hbm, shift_ref),
             (skip_hbm, skip_ref), (fwd_hbm, fwd_ref), (inv_hbm, inv_ref)]
    gw_copy, x_first, x_rest, *late = [
        pltpu.make_async_copy(src, dst, in_sem.at[2 * steps + 1 + k])
        for k, (src, dst) in enumerate(whole)]
    tiled = [(src, dst, in_sem.at[2 * steps + 1 + len(whole) + k])
             for k, (src, dst) in enumerate(
                 [(wo_hbm, wo_ref), (ak_hbm, ak_ref), (av_hbm, av_ref)])]

    def pair_copy(w_hbm, p, dst, sem):
        return pltpu.make_async_copy(w_hbm.bitcast(U32).at[:, p, :], dst, sem)

    def wait_filled(buf, sem):
        pltpu.make_async_copy(buf, buf, sem).wait()

    def fetch_group(t):
        for b in range(4):
            pair_copy(wuk_hbm if t < 4 else wuv_hbm, (t % 4) * 4 + b,
                      wkv_ref.at[t * 4 + b], in_sem.at[t]).start()

    def fetch_ahead(t):
        if t == 0:
            x_rest.start()
        fetch_group(t + 1)
        if 1 <= t <= 4:
            for p in range(4 * t - 4, 4 * t):
                pair_copy(wq_hbm, p, wq_ref.at[p], wq_sem).start()

    def c_copy(e):
        rows = pl.ds(pl.multiple_of(e * 2 * T, 2 * T), 2 * T)
        return pltpu.make_async_copy(c_hbm.at[rows], c_ref.at[rows], in_sem.at[steps + e])

    def out_copy(c, part):
        rows, n = ((pl.ds(0, S // 2), 0), (pl.ds(S // 2, S // 2), 0), (pl.ds(0, S), 1))[part]
        cols = pl.ds(pl.multiple_of((2 * c + n) * T, T), T)
        return pltpu.make_async_copy(
            out_ref.at[2 * c + n, rows], out_hbm.at[rows, cols], out_sem.at[3 * c + part])

    for e in range(steps):
        c_copy(e).start()
    fetch_group(0)
    x_first.start()
    gw_copy.start()

    def left_step(e, carry):
        c_copy(e).wait()
        _store_left(c_ref, slice(0, DC // 2), cs_ref, e, 0, T)
        return carry

    lax.fori_loop(0, steps, left_step, 0)
    gw_copy.wait()
    x_first.wait()

    def kv_step(t, carry):
        for k in range(steps - 1):
            pl.when(t == k)(functools.partial(fetch_ahead, k))
        pl.when(t == 1)(x_rest.wait)
        wait_filled(wkv_ref.at[pl.ds(t * 4, 4)], in_sem.at[t])
        gw = gw_ref[...].astype(F32).reshape(1, DM)

        def meanwhile(b, k):
            done = _store_left(x_ref, slice(b * T, (b + 1) * T), xs_ref, t, 32 * k, 32 * k + 32)
            rows = pl.ds(pl.multiple_of(t * 2 * T + (4 * b + k) * 16, 16), 16)
            logit = jnp.sum(x_ref[rows, :].astype(F32) * gw, axis=1, keepdims=True)
            g = jnp.broadcast_to(1.0 / (1.0 + jnp.exp(-logit)), (16, T))
            gate_ref[rows, :] = g
            return _zero_after(done + [g[:8], g[8:]], t)

        _project_kv(t, cs_ref, wkv_ref, kv_ref, meanwhile)
        return carry

    lax.fori_loop(0, steps, kv_step, 0)

    for copy in late:
        copy.start()
    wait_filled(wq_ref, wq_sem)

    def pair_step(p, carry):
        @pl.when(p < NC)
        def _():
            cols = pl.ds(pl.multiple_of(p * T, T), T)
            for src, dst, sem in tiled:
                pltpu.make_async_copy(src.at[:, cols], dst.at[p], sem).start()

        _attend_pair(p, xs_ref, wq_ref, kv_ref)
        return carry

    lax.fori_loop(0, NP, pair_step, 0)

    for copy in late:
        copy.wait()
    for _, dst, sem in tiled:
        wait_filled(dst, sem)

    for half in range(2):
        def mix_step(c, carry):
            _mix_step(c, half, kv_ref, wo_ref, x_ref, ak_ref, av_ref, hk_ref, shift_ref,
                      skip_ref, gate_ref, fwd_ref, inv_ref, uf_ref, hf_ref, held_ref, out_ref)
            for part in ((0,), (1, 2))[half]:
                out_copy(c, part).start()
            return carry

        lax.fori_loop(0, NC // 2, mix_step, 0)

    for c in range(NC // 2):
        for part in range(3):
            out_copy(c, part).wait()


@jax.jit
def pallas_gated_mix__ssm_conv_h3__compressed_kv_cla__prompt_kernel(
    A_q: jax.Array,
    A_k: jax.Array,
    A_v: jax.Array,
    A_shift_k: jax.Array,
    A_ssm_k: jax.Array,
    A_ssm_D: jax.Array,
    B_x: jax.Array,
    B_c_kv: jax.Array,
    B_w_q: jax.Array,
    B_w_uk: jax.Array,
    B_w_uv: jax.Array,
    B_w_o: jax.Array,
    gate_w: jax.Array,
):
    del B_x
    fwd, inv = _dft_matrices()
    hbm = pl.BlockSpec(memory_space=pl.ANY)
    out = pl.pallas_call(
        _kernel,
        out_shape=jax.ShapeDtypeStruct((S, DM), BF16),
        in_specs=[hbm] * 14,
        out_specs=hbm,
        scratch_shapes=[
            pltpu.VMEM((S, DM), BF16),
            pltpu.VMEM((NC, S, T), BF16),
            pltpu.VMEM((NC, S, T), BF16),
            pltpu.VMEM((DM, S), BF16),
            pltpu.VMEM((S, DC), BF16),
            pltpu.VMEM((NP, DM, DH), U32),
            pltpu.VMEM((2 * NP, DC, DH), U32),
            pltpu.VMEM((NC, H * DH, T), BF16),
            pltpu.VMEM((7, S // 4, DC // 2), U32),
            pltpu.VMEM((7, S // 4, DM // 2), U32),
            pltpu.VMEM((S, T), F32),
            pltpu.VMEM((NP, 2 * S, DH), U32),
            pltpu.VMEM((NB, 2 * T, T), F32),
            pltpu.VMEM((NB, 2 * T, T), F32),
            pltpu.VMEM((NC // 2, S, T), F32),
            pltpu.VMEM((NC, S, T), BF16),
            pltpu.VMEM((2 * T, T), BF16),
            pltpu.VMEM((T, 2 * T), BF16),
            pltpu.VMEM((KS, DM), BF16),
            pltpu.VMEM((DM,), BF16),
            pltpu.VMEM((DM,), BF16),
            pltpu.SemaphoreType.DMA((NB + 12,)),
            pltpu.SemaphoreType.DMA((3 * NC // 2,)),
        ],
        compiler_params=pltpu.CompilerParams(vmem_limit_bytes=124 * 2**20),
    )(
        A_q.reshape(S, DM), A_k.reshape(S, DM), A_v.reshape(S, DM), A_shift_k.T,
        A_ssm_k, A_ssm_D, B_c_kv.reshape(S, DC), B_w_q, B_w_uk, B_w_uv,
        B_w_o.reshape(H * DH, DM), gate_w, fwd, inv,
    )
    return out.reshape(1, S, DM)
```

```python
import functools

import jax
import jax.numpy as jnp
import numpy as np
from jax import lax
import jax.experimental.pallas as pl
import jax.experimental.pallas.tpu as pltpu

S = 2048
DM = 1024
H = 32
DH = 128
DC = 512
KS = 4
T = 128
W = T // 2
NB = S // T
NP = H // 2
NC = DM // T
LEAD = 12

F32 = jnp.float32
BF16 = jnp.bfloat16
U32 = jnp.uint32
NT = (((1,), (1,)), ((), ()))
LOG2E = float(np.log2(np.e))


def _dft_matrices():
    ks = np.concatenate([np.arange(0, T, 2), np.arange(1, T, 2)]).reshape(NB, 8)
    n = np.arange(T)
    theta = 2.0 * np.pi * (ks[:, :, None] + 0.5) * n[None, None, :] / (2 * T)
    fwd = np.concatenate([np.cos(theta), -np.sin(theta)], axis=1).reshape(2 * T, T)
    return fwd.astype(BF16), (fwd.T / T).astype(BF16)


def _mm(a, b):
    return jnp.dot(a, b, preferred_element_type=F32)


def _pack(v):
    return pltpu.pack_elementwise([v[:W], v[W:]], packed_dtype=BF16)


def _unpack(words):
    return pltpu.bitcast(words, BF16)


def _halves(words):
    return [pltpu.unpack_elementwise(words, index=i, packed_dtype=BF16, unpacked_dtype=F32)
            for i in range(2)]


def _zero(i):
    return lax.shift_right_logical(i, 8)


def _zero_after(values, i):
    bits = functools.reduce(jnp.bitwise_or, [pltpu.bitcast(v, U32) for v in values])
    return bits & jnp.full(bits.shape, _zero(i), jnp.int32).astype(U32)


def _left(a11, a12, a21, a22):
    return [a11 + a22, a21 + a22, a11, a22, a11 + a12, a21 - a11, a12 - a22]


def _right(b):
    return [b(0, 0, 0) + b(0, 1, 1), b(1, 0, 0), b(2, 0, 1) - b(2, 1, 1),
            b(3, 1, 0) - b(3, 0, 0), b(4, 1, 1), b(5, 0, 0) + b(5, 0, 1),
            b(6, 1, 0) + b(6, 1, 1)]


def _combine(m):
    return (m[0] + m[3] - m[4] + m[6], m[2] + m[4], m[1] + m[3], m[0] - m[1] + m[2] + m[5])


def _pair_weights(words):
    half = words.shape[0] // 2
    heads = _halves(words)
    return [v.astype(BF16)
            for v in _right(lambda i, r, c: heads[c][r * half:(r + 1) * half])]


def _store_left(src_ref, cols, dst_ref, e, r0, r1):
    half = src_ref.shape[1] // 2
    parts = []
    for j in range(2):
        rows = pl.ds(pl.multiple_of((2 * e + j) * T + r0, 32), r1 - r0)
        for c0 in (0, half):
            v = src_ref[rows, c0 + cols.start:c0 + cols.stop]
            parts.append(_halves(pltpu.bitcast(v, U32)))
    stored = []
    for odd in range(2):
        rows = pl.ds(pl.multiple_of(e * W + odd * (W // 2) + r0 // 4, 8), (r1 - r0) // 4)
        for i, v in enumerate(_left(*[part[odd] for part in parts])):
            stored.append(pltpu.bitcast(v.astype(BF16), U32))
            dst_ref[i, rows, cols] = stored[-1]
    return stored


def _project_kv(t, order, cs_ref, wkv_ref, kv_ref, meanwhile):
    base = pl.multiple_of((t >> 2) * S, S)
    w = [_pair_weights(wkv_ref[t * 4 + b]) for b in range(4)]
    for b, quarter in order:
        e = 2 * quarter
        zero = meanwhile(b, quarter)
        left = [cs_ref[i, e * W:(e + 2) * W, :] for i in range(7)]
        if zero is not None:
            left[2] = jnp.concatenate(
                [left[2][:8] | jnp.concatenate([zero, zero], axis=1), left[2][8:]], axis=0)
        c = _combine([_mm(_unpack(left[i]), w[b][i]) for i in range(7)])
        for k in range(2):
            for odd in range(2):
                for head in range(2):
                    r0 = head * (S // 2) + (2 * (e + k) + odd) * W
                    kv_ref[(t & 3) * 4 + b, pl.ds(base + r0, W), :] = _pack(
                        c[2 * odd + head][k * T:(k + 1) * T])


def _operand_row(e, i):
    return (i // 2) * (S // 2) + (2 * e + i % 2) * W


def _attend_pair(p, xs_ref, wq_ref, kv_ref):
    row = lax.broadcasted_iota(jnp.int32, (T, T), 0)
    col = lax.broadcasted_iota(jnp.int32, (T, T), 1)
    causal = col <= jnp.where(row < W, 2 * row, 2 * (row - W) + 1)
    w = _pair_weights(wq_ref[p])
    q, s, ctx = {}, {}, {}

    def blocks(region, n):
        r0 = region * (S // 2)
        return _unpack(kv_ref[p, r0:r0 + n * W, :])

    def queries(e):
        c = _combine([_mm(_unpack(xs_ref[i, e * W:(e + 1) * W, :]), w[i]) for i in range(7)])
        for odd in range(2):
            for head in range(2):
                q[2 * e + odd, head] = (c[2 * odd + head] * (DH ** -0.5 * LOG2E)).astype(BF16)

    def scores(r, head):
        d = lax.dot_general(q.pop((r, head)), blocks(head, r + 1), NT,
                            preferred_element_type=F32)
        tiles = [d[:, j * T:(j + 1) * T] for j in range(r + 1)]
        tiles[r] = jnp.where(causal, tiles[r], -1e9 * LOG2E)
        top = jnp.max(functools.reduce(jnp.maximum, tiles), axis=1, keepdims=True)
        s[r, head] = tiles, top

    def context(r, head):
        tiles, top = s.pop((r, head))
        top = jnp.broadcast_to(top, (T, T))
        tiles = [jnp.exp2(v - top) for v in tiles]
        total = functools.reduce(jnp.add, tiles)
        if r > 0:
            tiles[r] = jnp.minimum(tiles[r], total)
        o = _mm(jnp.concatenate(tiles, axis=1).astype(BF16), blocks(2 + head, r + 1))
        total = jnp.sum(total, axis=1, keepdims=True)
        inv = pltpu.reciprocal(total, approx=True)
        inv = inv * (2.0 - total * inv)
        ctx[r, head] = o * inv

    def emit(e):
        ops = _left(*[ctx.pop((2 * e + odd, head)) for odd in range(2) for head in range(2)])
        for i in range(7):
            r0 = _operand_row(e, i)
            kv_ref[p, r0:r0 + W, :] = _pack(ops[i])

    order = [(r, head) for r in range(NB - 1, -1, -1) for head in range(2)]
    scored, lead = 0, 0
    for r, head in order:
        while scored < len(order) and lead < LEAD + r + 1:
            if order[scored] not in q:
                queries(order[scored][0] // 2)
            scores(*order[scored])
            lead += order[scored][0] + 1
            scored += 1
        context(r, head)
        lead -= r + 1
        if head == 1 and r % 2 == 0:
            emit(r // 2)


def _mix_step(c, half, kv_ref, wo_ref, x_ref, ak_ref, av_ref, hk_ref, shift_ref, skip_ref,
              gate_ref, fwd_ref, inv_ref, uf_ref, hf_ref, held_ref, out_ref):
    tile = 2 * c + half
    own = pl.ds(pl.multiple_of(tile * T, T), T)
    fwd = fwd_ref[...]
    inv = inv_ref[...]
    skip = skip_ref[pl.ds(pl.multiple_of(c * 2 * T, 2 * T), 2 * T)]
    skip = skip.astype(F32).reshape(1, 2 * T)[:, half * T:(half + 1) * T]

    taps = shift_ref[:, own].astype(F32)
    keys = ak_ref[tile].astype(F32)
    shifted = keys * taps[KS - 1:KS]
    for t in range(KS - 2, -1, -1):
        shifted = jnp.concatenate([jnp.zeros((1, T), F32), shifted[:-1]], axis=0)
        shifted = shifted + keys * taps[t:t + 1]

    def heads(i, odd, n):
        at = 2 * c + n + _zero(c >> i)
        return jnp.concatenate([wo_ref[at, h * DH:(h + 1) * DH, :].astype(F32)
                                for h in range(odd, H, 2)], axis=0)

    w = [v.astype(BF16) for v in _right(heads)]
    plain, u, z, parts, due = [], {}, {}, {}, {}

    def deliver(j, n, v):
        blk = slice(j * T, (j + 1) * T)
        if n == half and j // 8 == half:
            if (j, n) not in parts:
                parts[j, n] = v
                return
            v = v + parts.pop((j, n))
        elif half == 0:
            held_ref[c, blk, :] = v
            return
        else:
            v = v + held_ref[c, blk, :]
        out_ref[2 * c + n, blk, :] = v.astype(BF16)

    def spectra(j):
        blk = slice(j * T, (j + 1) * T)
        cur = lax.dot_general(fwd, hk_ref[own, blk], NT, preferred_element_type=F32)
        for f in range(NB):
            re, im = slice(16 * f, 16 * f + 8), slice(16 * f + 8, 16 * f + 16)
            if j == 0:
                hr, hi = cur[re], cur[im]
            elif f < NB // 2:
                hr, hi = cur[re] - plain[-1][im], cur[im] + plain[-1][re]
            else:
                hr, hi = cur[re] + plain[-1][im], cur[im] - plain[-1][re]
            hf_ref[j, re, :] = hr
            hf_ref[j, im, :] = hi
        plain.append(cur)
        u[j] = (shifted[blk] * av_ref[tile, blk, :].astype(F32)).astype(BF16)
        uf_ref[j] = _mm(fwd, u[j])

    def multiply(i0, start, step):
        base = _zero(c >> i0)
        rows = {i0: [], i0 + 1: []}
        for f in range(NB):
            re, im = slice(16 * f, 16 * f + 8), slice(16 * f + 8, 16 * f + 16)
            acc = {}
            for j in range(i0 + 2):
                ur, ui = uf_ref[base + j, re, :], uf_ref[base + j, im, :]
                for i in range(max(i0, j), i0 + 2):
                    hr, hi = hf_ref[i - j, re, :], hf_ref[i - j, im, :]
                    pr, pi = ur * hr - ui * hi, ur * hi + ui * hr
                    acc[i] = (pr, pi) if j == 0 else (acc[i][0] + pr, acc[i][1] + pi)
            for i in rows:
                rows[i] += acc[i]
            due[int(start + f * step)] = _zero_after(acc[i0] + acc[i0 + 1], c)
        for i in rows:
            z[i] = jnp.concatenate(rows[i], axis=0).astype(BF16)

    def convolved(i):
        blk = slice(i * T, (i + 1) * T)
        y = _mm(inv, z.pop(i)) + u.pop(i).astype(F32) * skip
        deliver(i, half, gate_ref[blk, :] * (x_ref[blk, own].astype(F32) * y))

    def product(e, i):
        r0 = _operand_row(e, i)
        left = [kv_ref[p, r0:r0 + W, :] for p in range(NP)]
        for p in range(0, NP, 4):
            at = 32 * i + 2 * p
            if any(at + k in due for k in range(8)):
                rows = [left[p][8 * k:8 * k + 8] for k in range(8)]
                left[p] = jnp.concatenate(
                    [v | due.pop(at + k) if at + k in due else v for k, v in enumerate(rows)],
                    axis=0)
        return _mm(_unpack(jnp.concatenate(left, axis=1)), w[i])

    groups = [(0, 2), (4, 14), (6, 12), (8, 10)] if half == 0 else [
        (0, 2), (8, 10), (12, 6), (14, 4)]
    for j in range(4):
        spectra(j)
    for step, pair in enumerate(groups):
        e = 4 * half + step
        pace = ((64, 3), (130, 4)) if step == 0 else ((4, 7.5), (130, 5.8))
        m = []
        for k, i0 in enumerate(pair):
            multiply(i0, *pace[k])
            for _ in range(4 - k):
                m.append(product(e, len(m)))
                for j in range(len(plain), min(len(plain) + 2, NB)):
                    spectra(j)
            convolved(i0)
            convolved(i0 + 1)
        b = _combine(m)
        for odd in range(2):
            j = 2 * e + odd
            for n in range(2):
                deliver(j, n, (1.0 - gate_ref[j * T:(j + 1) * T, :]) * b[2 * odd + n])


def _kernel(x_hbm, ak_hbm, av_hbm, shift_hbm, hk_hbm, skip_hbm, c_hbm, wq_hbm, wuk_hbm,
            wuv_hbm, wo_hbm, gw_hbm, fwd_hbm, inv_hbm, out_hbm,
            x_ref, ak_ref, av_ref, hk_ref, c_ref, wq_ref, wkv_ref, wo_ref, cs_ref, xs_ref,
            gate_ref, kv_ref, uf_ref, hf_ref, held_ref, out_ref, fwd_ref, inv_ref, shift_ref,
            skip_ref, gw_ref, in_sem, out_sem):
    steps = NB // 2
    wq_sem = in_sem.at[steps]
    first, rest = pl.ds(0, 2 * T), pl.ds(2 * T, S - 2 * T)
    upper, lower = pl.ds(0, S // 2), pl.ds(S // 2, S // 2)
    whole = [(c_hbm.at[upper], c_ref.at[upper]), (c_hbm.at[lower], c_ref.at[lower]),
             (gw_hbm, gw_ref), (x_hbm.at[first], x_ref.at[first]),
             (x_hbm.at[rest], x_ref.at[rest]), (hk_hbm, hk_ref), (shift_hbm, shift_ref),
             (skip_hbm, skip_ref), (fwd_hbm, fwd_ref), (inv_hbm, inv_ref)]
    c_upper, c_lower, gw_copy, x_first, x_rest, *late = [
        pltpu.make_async_copy(src, dst, in_sem.at[steps + 1 + k])
        for k, (src, dst) in enumerate(whole)]
    tiled = [(src, dst, in_sem.at[steps + 1 + len(whole) + k])
             for k, (src, dst) in enumerate(
                 [(wo_hbm, wo_ref), (ak_hbm, ak_ref), (av_hbm, av_ref)])]

    def pair_copy(w_hbm, p, dst, sem):
        return pltpu.make_async_copy(w_hbm.bitcast(U32).at[:, p, :], dst, sem)

    def wait_filled(buf, sem):
        pltpu.make_async_copy(buf, buf, sem).wait()

    def fetch_group(t):
        for b in range(4):
            pair_copy(wuk_hbm if t < 4 else wuv_hbm, (t % 4) * 4 + b,
                      wkv_ref.at[t * 4 + b], in_sem.at[t]).start()

    def fetch_ahead(t):
        fetch_group(t + 1)
        if 1 <= t <= 4:
            for p in range(4 * t - 4, 4 * t):
                pair_copy(wq_hbm, p, wq_ref.at[p], wq_sem).start()

    def out_copy(c, part):
        rows, n = ((pl.ds(0, S // 2), 0), (pl.ds(S // 2, S // 2), 0), (pl.ds(0, S), 1))[part]
        return pltpu.make_async_copy(
            out_ref.at[2 * c + n, rows], out_hbm.at[rows, pl.ds((2 * c + n) * T, T)],
            out_sem.at[3 * c + part])

    def prepare_x(t, b, k):
        done = _store_left(x_ref, slice(b * T, (b + 1) * T), xs_ref, t, 32 * k, 32 * k + 32)
        rows = pl.ds(pl.multiple_of(t * 2 * T + (4 * b + k) * 16, 16), 16)
        gw = gw_ref[...].astype(F32).reshape(1, DM)
        logit = jnp.sum(x_ref[rows, :].astype(F32) * gw, axis=1, keepdims=True)
        g = jnp.broadcast_to(1.0 / (1.0 + jnp.exp(-logit)), (16, T))
        gate_ref[rows, :] = g
        return _zero_after(done + [g[:8], g[8:]], t)

    def prepare_c(e0):
        for e in range(e0, e0 + steps // 2):
            _store_left(c_ref, slice(0, DC // 2), cs_ref, e, 0, T)

    def first_step(t, carry):
        def meanwhile(b, quarter):
            if (b, quarter) == (0, 1):
                c_lower.wait()
                x_first.wait()
                gw_copy.wait()
                prepare_c(steps // 2)
            if quarter >= 2:
                return prepare_x(t, b, 2 * quarter - 4) | prepare_x(t, b, 2 * quarter - 3)

        c_upper.wait()
        prepare_c(0)
        wait_filled(wkv_ref.at[pl.ds(0, 4)], in_sem.at[0])
        _project_kv(t, [(b, quarter) for quarter in range(4) for b in range(4)],
                    cs_ref, wkv_ref, kv_ref, meanwhile)
        return carry

    def kv_step(t, carry):
        for k in range(1, steps - 1):
            pl.when(t == k)(functools.partial(fetch_ahead, k))
        pl.when(t == 1)(x_rest.wait)
        wait_filled(wkv_ref.at[pl.ds(t * 4, 4)], in_sem.at[t])
        _project_kv(t, [(b, quarter) for b in range(4) for quarter in range(4)],
                    cs_ref, wkv_ref, kv_ref, functools.partial(prepare_x, t))
        return carry

    c_upper.start()
    fetch_group(0)
    c_lower.start()
    x_first.start()
    gw_copy.start()
    fetch_group(1)
    x_rest.start()
    first_step(jnp.int32(0), 0)
    lax.fori_loop(1, steps, kv_step, 0)

    for copy in late:
        copy.start()
    wait_filled(wq_ref, wq_sem)

    def pair_step(p, carry):
        @pl.when(p < NC)
        def _():
            cols = pl.ds(pl.multiple_of(p * T, T), T)
            for src, dst, sem in tiled:
                pltpu.make_async_copy(src.at[:, cols], dst.at[p], sem).start()

        _attend_pair(p, xs_ref, wq_ref, kv_ref)
        return carry

    lax.fori_loop(0, NP, pair_step, 0)

    for copy in late:
        copy.wait()
    for _, dst, sem in tiled:
        wait_filled(dst, sem)

    for half in range(2):
        def mix_step(c, carry):
            _mix_step(c, half, kv_ref, wo_ref, x_ref, ak_ref, av_ref, hk_ref, shift_ref,
                      skip_ref, gate_ref, fwd_ref, inv_ref, uf_ref, hf_ref, held_ref, out_ref)
            for k in range(NC // 2):
                @pl.when(c == k)
                def _():
                    for part in ((0,), (1, 2))[half]:
                        out_copy(k, part).start()

            return carry

        lax.fori_loop(0, NC // 2, mix_step, 0)

    for c in range(NC // 2):
        for part in range(3):
            out_copy(c, part).wait()


@jax.jit
def pallas_gated_mix__ssm_conv_h3__compressed_kv_cla__prompt_kernel(
    A_q: jax.Array,
    A_k: jax.Array,
    A_v: jax.Array,
    A_shift_k: jax.Array,
    A_ssm_k: jax.Array,
    A_ssm_D: jax.Array,
    B_x: jax.Array,
    B_c_kv: jax.Array,
    B_w_q: jax.Array,
    B_w_uk: jax.Array,
    B_w_uv: jax.Array,
    B_w_o: jax.Array,
    gate_w: jax.Array,
):
    del B_x
    fwd, inv = _dft_matrices()
    hbm = pl.BlockSpec(memory_space=pl.ANY)
    out = pl.pallas_call(
        _kernel,
        out_shape=jax.ShapeDtypeStruct((S, DM), BF16),
        in_specs=[hbm] * 14,
        out_specs=hbm,
        scratch_shapes=[
            pltpu.VMEM((S, DM), BF16),
            pltpu.VMEM((NC, S, T), BF16),
            pltpu.VMEM((NC, S, T), BF16),
            pltpu.VMEM((DM, S), BF16),
            pltpu.VMEM((S, DC), BF16),
            pltpu.VMEM((NP, DM, DH), U32),
            pltpu.VMEM((2 * NP, DC, DH), U32),
            pltpu.VMEM((NC, H * DH, T), BF16),
            pltpu.VMEM((7, S // 4, DC // 2), U32),
            pltpu.VMEM((7, S // 4, DM // 2), U32),
            pltpu.VMEM((S, T), F32),
            pltpu.VMEM((NP, 2 * S, DH), U32),
            pltpu.VMEM((NB, 2 * T, T), F32),
            pltpu.VMEM((NB, 2 * T, T), F32),
            pltpu.VMEM((NC // 2, S, T), F32),
            pltpu.VMEM((NC, S, T), BF16),
            pltpu.VMEM((2 * T, T), BF16),
            pltpu.VMEM((T, 2 * T), BF16),
            pltpu.VMEM((KS, DM), BF16),
            pltpu.VMEM((DM,), BF16),
            pltpu.VMEM((DM,), BF16),
            pltpu.SemaphoreType.DMA((NB // 2 + 14,)),
            pltpu.SemaphoreType.DMA((3 * NC // 2,)),
        ],
        compiler_params=pltpu.CompilerParams(vmem_limit_bytes=124 * 2**20),
    )(
        A_q.reshape(S, DM), A_k.reshape(S, DM), A_v.reshape(S, DM), A_shift_k.T,
        A_ssm_k, A_ssm_D, B_c_kv.reshape(S, DC), B_w_q, B_w_uk, B_w_uv,
        B_w_o.reshape(H * DH, DM), gate_w, fwd, inv,
    )
    return out.reshape(1, S, DM)
```

```python
import functools

import jax
import jax.numpy as jnp
import numpy as np
from jax import lax
import jax.experimental.pallas as pl
import jax.experimental.pallas.tpu as pltpu

S = 2048
DM = 1024
H = 32
DH = 128
DC = 512
KS = 4
T = 128
W = T // 2
NB = S // T
NP = H // 2
NC = DM // T
LEAD = 6

F32 = jnp.float32
BF16 = jnp.bfloat16
U32 = jnp.uint32
NT = (((1,), (1,)), ((), ()))
LOG2E = float(np.log2(np.e))


def _dft_matrices():
    ks = np.concatenate([np.arange(0, T, 2), np.arange(1, T, 2)]).reshape(NB, 8)
    n = np.arange(T)
    theta = 2.0 * np.pi * (ks[:, :, None] + 0.5) * n[None, None, :] / (2 * T)
    fwd = np.concatenate([np.cos(theta), -np.sin(theta)], axis=1).reshape(2 * T, T)
    return fwd.astype(BF16), (fwd.T / T).astype(BF16)


def _mm(a, b):
    return jnp.dot(a, b, preferred_element_type=F32)


def _pack(v):
    return pltpu.pack_elementwise([v[:W], v[W:]], packed_dtype=BF16)


def _unpack(words):
    return pltpu.bitcast(words, BF16)


def _halves(words):
    return [pltpu.unpack_elementwise(words, index=i, packed_dtype=BF16, unpacked_dtype=F32)
            for i in range(2)]


def _zero(i):
    return lax.shift_right_logical(i, 8)


def _zero_after(values, i):
    bits = functools.reduce(jnp.bitwise_or, [pltpu.bitcast(v, U32) for v in values])
    return bits & jnp.full(bits.shape, _zero(i), jnp.int32).astype(U32)


def _left(a11, a12, a21, a22):
    return [a11 + a22, a21 + a22, a11, a22, a11 + a12, a21 - a11, a12 - a22]


def _right(b):
    return [b(0, 0, 0) + b(0, 1, 1), b(1, 0, 0), b(2, 0, 1) - b(2, 1, 1),
            b(3, 1, 0) - b(3, 0, 0), b(4, 1, 1), b(5, 0, 0) + b(5, 0, 1),
            b(6, 1, 0) + b(6, 1, 1)]


def _combine(m):
    return (m[0] + m[3] - m[4] + m[6], m[2] + m[4], m[1] + m[3], m[0] - m[1] + m[2] + m[5])


def _pair_weights(words):
    half = words.shape[0] // 2
    heads = _halves(words)
    return [v.astype(BF16)
            for v in _right(lambda i, r, c: heads[c][r * half:(r + 1) * half])]


def _store_left(src_ref, cols, dst_ref, e, r0, r1):
    half = src_ref.shape[1] // 2
    parts = []
    for j in range(2):
        rows = pl.ds(pl.multiple_of((2 * e + j) * T + r0, 32), r1 - r0)
        for c0 in (0, half):
            v = src_ref[rows, c0 + cols.start:c0 + cols.stop]
            parts.append(_halves(pltpu.bitcast(v, U32)))
    stored = []
    for odd in range(2):
        rows = pl.ds(pl.multiple_of(e * W + odd * (W // 2) + r0 // 4, 8), (r1 - r0) // 4)
        for i, v in enumerate(_left(*[part[odd] for part in parts])):
            stored.append(pltpu.bitcast(v.astype(BF16), U32))
            dst_ref[i, rows, cols] = stored[-1]
    return stored


def _project_kv(t, order, cs_ref, wkv_ref, kv_ref, meanwhile):
    base = pl.multiple_of((t >> 2) * S, S)
    w = [_pair_weights(wkv_ref[t * 4 + b]) for b in range(4)]
    for b, quarter in order:
        e = 2 * quarter
        zero = meanwhile(b, quarter)
        left = [cs_ref[i, e * W:(e + 2) * W, :] for i in range(7)]
        if zero is not None:
            left[2] = jnp.concatenate(
                [left[2][:8] | jnp.concatenate([zero, zero], axis=1), left[2][8:]], axis=0)
        c = _combine([_mm(_unpack(left[i]), w[b][i]) for i in range(7)])
        for k in range(2):
            for odd in range(2):
                for head in range(2):
                    r0 = head * (S // 2) + (2 * (e + k) + odd) * W
                    kv_ref[(t & 3) * 4 + b, pl.ds(base + r0, W), :] = _pack(
                        c[2 * odd + head][k * T:(k + 1) * T])


def _operand_row(e, i):
    return (i // 2) * (S // 2) + (2 * e + i % 2) * W


def _attend_pair(p, xs_ref, wq_ref, kv_ref):
    row = lax.broadcasted_iota(jnp.int32, (T, T), 0)
    col = lax.broadcasted_iota(jnp.int32, (T, T), 1)
    causal = col <= jnp.where(row < W, 2 * row, 2 * (row - W) + 1)
    w = _pair_weights(wq_ref[p])
    q, s, ctx = {}, {}, {}

    def blocks(region, n):
        r0 = region * (S // 2)
        return _unpack(kv_ref[p, r0:r0 + n * W, :])

    def queries(e):
        c = _combine([_mm(_unpack(xs_ref[i, e * W:(e + 1) * W, :]), w[i]) for i in range(7)])
        for odd in range(2):
            for head in range(2):
                q[2 * e + odd, head] = (c[2 * odd + head] * (DH ** -0.5 * LOG2E)).astype(BF16)

    def scores(r, head):
        d = lax.dot_general(q.pop((r, head)), blocks(head, r + 1), NT,
                            preferred_element_type=F32)
        tiles = [d[:, j * T:(j + 1) * T] for j in range(r + 1)]
        tiles[r] = jnp.where(causal, tiles[r], -1e9 * LOG2E)
        top = jnp.max(functools.reduce(jnp.maximum, tiles), axis=1, keepdims=True)
        s[r, head] = tiles, top

    def context(r, head):
        tiles, top = s.pop((r, head))
        top = jnp.broadcast_to(top, (T, T))
        tiles = [jnp.exp2(v - top) for v in tiles]
        total = tiles[0]
        for j in range(1, r + 1):
            total = total + tiles[j]
            tiles[j] = jnp.minimum(tiles[j], total)
        o = _mm(jnp.concatenate(tiles, axis=1).astype(BF16), blocks(2 + head, r + 1))
        total = jnp.sum(total, axis=1, keepdims=True)
        inv = pltpu.reciprocal(total, approx=True)
        inv = inv * (2.0 - total * inv)
        ctx[r, head] = o * inv

    def emit(e):
        ops = _left(*[ctx.pop((2 * e + odd, head)) for odd in range(2) for head in range(2)])
        for i in range(7):
            r0 = _operand_row(e, i)
            kv_ref[p, r0:r0 + W, :] = _pack(ops[i])

    order = [(r, head) for r in range(NB - 1, -1, -1) for head in range(2)]
    scored, lead = 0, 0
    for r, head in order:
        while scored < len(order) and lead < LEAD + r + 1:
            if order[scored] not in q:
                queries(order[scored][0] // 2)
            scores(*order[scored])
            lead += order[scored][0] + 1
            scored += 1
        context(r, head)
        lead -= r + 1
        if head == 1 and r % 2 == 0:
            emit(r // 2)


def _mix_step(c, half, kv_ref, wo_ref, x_ref, ak_ref, av_ref, hk_ref, shift_ref, skip_ref,
              gate_ref, fwd_ref, inv_ref, uf_ref, hf_ref, held_ref, out_ref):
    tile = 2 * c + half
    own = pl.ds(pl.multiple_of(tile * T, T), T)
    fwd = fwd_ref[...]
    inv = inv_ref[...]
    skip = skip_ref[pl.ds(pl.multiple_of(c * 2 * T, 2 * T), 2 * T)]
    skip = skip.astype(F32).reshape(1, 2 * T)[:, half * T:(half + 1) * T]

    taps = shift_ref[:, own].astype(F32)
    keys = ak_ref[tile].astype(F32)
    shifted = keys * taps[KS - 1:KS]
    for t in range(KS - 2, -1, -1):
        shifted = jnp.concatenate([jnp.zeros((1, T), F32), shifted[:-1]], axis=0)
        shifted = shifted + keys * taps[t:t + 1]

    def heads(i, odd, n):
        at = 2 * c + n + _zero(c >> i)
        return jnp.concatenate([wo_ref[at, h * DH:(h + 1) * DH, :].astype(F32)
                                for h in range(odd, H, 2)], axis=0)

    w = [v.astype(BF16) for v in _right(heads)]
    plain, u, z, parts, due = [], {}, {}, {}, {}

    def deliver(j, n, v):
        blk = slice(j * T, (j + 1) * T)
        if n == half and j // 8 == half:
            if (j, n) not in parts:
                parts[j, n] = v
                return
            v = v + parts.pop((j, n))
        elif half == 0:
            held_ref[c, blk, :] = v
            return
        else:
            v = v + held_ref[c, blk, :]
        out_ref[2 * c + n, blk, :] = v.astype(BF16)

    def spectra(j):
        blk = slice(j * T, (j + 1) * T)
        cur = lax.dot_general(fwd, hk_ref[own, blk], NT, preferred_element_type=F32)
        for f in range(NB):
            re, im = slice(16 * f, 16 * f + 8), slice(16 * f + 8, 16 * f + 16)
            if j == 0:
                hr, hi = cur[re], cur[im]
            elif f < NB // 2:
                hr, hi = cur[re] - plain[-1][im], cur[im] + plain[-1][re]
            else:
                hr, hi = cur[re] + plain[-1][im], cur[im] - plain[-1][re]
            hf_ref[j, re, :] = hr
            hf_ref[j, im, :] = hi
        plain.append(cur)
        u[j] = (shifted[blk] * av_ref[tile, blk, :].astype(F32)).astype(BF16)
        uf_ref[j] = _mm(fwd, u[j])

    def multiply(i0, start, step):
        base = _zero(c >> i0)
        rows = {i0: [], i0 + 1: []}
        for f in range(NB):
            re, im = slice(16 * f, 16 * f + 8), slice(16 * f + 8, 16 * f + 16)
            acc = {}
            for j in range(i0 + 2):
                ur, ui = uf_ref[base + j, re, :], uf_ref[base + j, im, :]
                for i in range(max(i0, j), i0 + 2):
                    hr, hi = hf_ref[i - j, re, :], hf_ref[i - j, im, :]
                    pr, pi = ur * hr - ui * hi, ur * hi + ui * hr
                    acc[i] = (pr, pi) if j == 0 else (acc[i][0] + pr, acc[i][1] + pi)
            for i in rows:
                rows[i] += acc[i]
            due[int(start + f * step)] = _zero_after(acc[i0] + acc[i0 + 1], c)
        for i in rows:
            z[i] = jnp.concatenate(rows[i], axis=0).astype(BF16)

    def convolved(i):
        blk = slice(i * T, (i + 1) * T)
        y = _mm(inv, z.pop(i)) + u.pop(i).astype(F32) * skip
        deliver(i, half, gate_ref[blk, :] * (x_ref[blk, own].astype(F32) * y))

    def product(e, i):
        r0 = _operand_row(e, i)
        left = [kv_ref[p, r0:r0 + W, :] for p in range(NP)]
        for p in range(0, NP, 4):
            at = 32 * i + 2 * p
            if any(at + k in due for k in range(8)):
                rows = [left[p][8 * k:8 * k + 8] for k in range(8)]
                left[p] = jnp.concatenate(
                    [v | due.pop(at + k) if at + k in due else v for k, v in enumerate(rows)],
                    axis=0)
        return _mm(_unpack(jnp.concatenate(left, axis=1)), w[i])

    groups = [(0, 2), (4, 14), (6, 12), (8, 10)] if half == 0 else [
        (0, 2), (8, 10), (12, 6), (14, 4)]
    for j in range(4):
        spectra(j)
    for step, pair in enumerate(groups):
        e = 4 * half + step
        pace = ((64, 3), (130, 4)) if step == 0 else ((4, 7.5), (130, 5.8))
        m = []
        for k, i0 in enumerate(pair):
            multiply(i0, *pace[k])
            for _ in range(4 - k):
                m.append(product(e, len(m)))
                for j in range(len(plain), min(len(plain) + 2, NB)):
                    spectra(j)
            convolved(i0)
            convolved(i0 + 1)
        b = _combine(m)
        for odd in range(2):
            j = 2 * e + odd
            for n in range(2):
                deliver(j, n, (1.0 - gate_ref[j * T:(j + 1) * T, :]) * b[2 * odd + n])


def _kernel(x_hbm, ak_hbm, av_hbm, shift_hbm, hk_hbm, skip_hbm, c_hbm, wq_hbm, wuk_hbm,
            wuv_hbm, wo_hbm, gw_hbm, fwd_hbm, inv_hbm, out_hbm,
            x_ref, ak_ref, av_ref, hk_ref, c_ref, wq_ref, wkv_ref, wo_ref, cs_ref, xs_ref,
            gate_ref, kv_ref, uf_ref, hf_ref, held_ref, out_ref, fwd_ref, inv_ref, shift_ref,
            skip_ref, gw_ref, in_sem, out_sem):
    steps = NB // 2
    wq_sem = in_sem.at[steps]
    first, rest = pl.ds(0, 2 * T), pl.ds(2 * T, S - 2 * T)
    upper, lower = pl.ds(0, S // 2), pl.ds(S // 2, S // 2)
    whole = [(c_hbm.at[upper], c_ref.at[upper]), (c_hbm.at[lower], c_ref.at[lower]),
             (gw_hbm, gw_ref), (x_hbm.at[first], x_ref.at[first]),
             (x_hbm.at[rest], x_ref.at[rest]), (hk_hbm, hk_ref), (shift_hbm, shift_ref),
             (skip_hbm, skip_ref), (fwd_hbm, fwd_ref), (inv_hbm, inv_ref)]
    c_upper, c_lower, gw_copy, x_first, x_rest, *late = [
        pltpu.make_async_copy(src, dst, in_sem.at[steps + 1 + k])
        for k, (src, dst) in enumerate(whole)]
    tiled = [(src, dst, in_sem.at[steps + 1 + len(whole) + k])
             for k, (src, dst) in enumerate(
                 [(wo_hbm, wo_ref), (ak_hbm, ak_ref), (av_hbm, av_ref)])]

    def pair_copy(w_hbm, p, dst, sem):
        return pltpu.make_async_copy(w_hbm.bitcast(U32).at[:, p, :], dst, sem)

    def wait_filled(buf, sem):
        pltpu.make_async_copy(buf, buf, sem).wait()

    def fetch_group(t):
        for b in range(4):
            pair_copy(wuk_hbm if t < 4 else wuv_hbm, (t % 4) * 4 + b,
                      wkv_ref.at[t * 4 + b], in_sem.at[t]).start()

    def fetch_ahead(t):
        fetch_group(t + 1)
        if 1 <= t <= 4:
            for p in range(4 * t - 4, 4 * t):
                pair_copy(wq_hbm, p, wq_ref.at[p], wq_sem).start()

    def out_copy(c, part):
        rows, n = ((pl.ds(0, S // 2), 0), (pl.ds(S // 2, S // 2), 0), (pl.ds(0, S), 1))[part]
        return pltpu.make_async_copy(
            out_ref.at[2 * c + n, rows], out_hbm.at[rows, pl.ds((2 * c + n) * T, T)],
            out_sem.at[3 * c + part])

    def prepare_x(t, b, k):
        done = _store_left(x_ref, slice(b * T, (b + 1) * T), xs_ref, t, 32 * k, 32 * k + 32)
        rows = pl.ds(pl.multiple_of(t * 2 * T + (4 * b + k) * 16, 16), 16)
        gw = gw_ref[...].astype(F32).reshape(1, DM)
        logit = jnp.sum(x_ref[rows, :].astype(F32) * gw, axis=1, keepdims=True)
        g = jnp.broadcast_to(1.0 / (1.0 + jnp.exp(-logit)), (16, T))
        gate_ref[rows, :] = g
        return _zero_after(done + [g[:8], g[8:]], t)

    def prepare_c(e0):
        for e in range(e0, e0 + steps // 2):
            _store_left(c_ref, slice(0, DC // 2), cs_ref, e, 0, T)

    def first_step(t, carry):
        def meanwhile(b, quarter):
            if (b, quarter) == (0, 1):
                c_lower.wait()
                x_first.wait()
                gw_copy.wait()
                prepare_c(steps // 2)
            if quarter >= 2:
                return prepare_x(t, b, 2 * quarter - 4) | prepare_x(t, b, 2 * quarter - 3)

        c_upper.wait()
        prepare_c(0)
        wait_filled(wkv_ref.at[pl.ds(0, 4)], in_sem.at[0])
        _project_kv(t, [(b, quarter) for quarter in range(4) for b in range(4)],
                    cs_ref, wkv_ref, kv_ref, meanwhile)
        return carry

    def kv_step(t, carry):
        for k in range(1, steps - 1):
            pl.when(t == k)(functools.partial(fetch_ahead, k))
        pl.when(t == 1)(x_rest.wait)
        wait_filled(wkv_ref.at[pl.ds(t * 4, 4)], in_sem.at[t])
        _project_kv(t, [(b, quarter) for b in range(4) for quarter in range(4)],
                    cs_ref, wkv_ref, kv_ref, functools.partial(prepare_x, t))
        return carry

    c_upper.start()
    fetch_group(0)
    c_lower.start()
    x_first.start()
    gw_copy.start()
    fetch_group(1)
    x_rest.start()
    first_step(jnp.int32(0), 0)
    lax.fori_loop(1, steps, kv_step, 0)

    for copy in late:
        copy.start()
    wait_filled(wq_ref, wq_sem)

    def pair_step(p, carry):
        @pl.when(p < NC)
        def _():
            cols = pl.ds(pl.multiple_of(p * T, T), T)
            for src, dst, sem in tiled:
                pltpu.make_async_copy(src.at[:, cols], dst.at[p], sem).start()

        _attend_pair(p, xs_ref, wq_ref, kv_ref)
        return carry

    lax.fori_loop(0, NP, pair_step, 0)

    for copy in late:
        copy.wait()
    for _, dst, sem in tiled:
        wait_filled(dst, sem)

    for half in range(2):
        def mix_step(c, carry):
            _mix_step(c, half, kv_ref, wo_ref, x_ref, ak_ref, av_ref, hk_ref, shift_ref,
                      skip_ref, gate_ref, fwd_ref, inv_ref, uf_ref, hf_ref, held_ref, out_ref)
            for k in range(NC // 2):
                @pl.when(c == k)
                def _():
                    for part in ((0,), (1, 2))[half]:
                        out_copy(k, part).start()

            return carry

        lax.fori_loop(0, NC // 2, mix_step, 0)

    for c in range(NC // 2):
        for part in range(3):
            out_copy(c, part).wait()


@jax.jit
def pallas_gated_mix__ssm_conv_h3__compressed_kv_cla__prompt_kernel(
    A_q: jax.Array,
    A_k: jax.Array,
    A_v: jax.Array,
    A_shift_k: jax.Array,
    A_ssm_k: jax.Array,
    A_ssm_D: jax.Array,
    B_x: jax.Array,
    B_c_kv: jax.Array,
    B_w_q: jax.Array,
    B_w_uk: jax.Array,
    B_w_uv: jax.Array,
    B_w_o: jax.Array,
    gate_w: jax.Array,
):
    del B_x
    fwd, inv = _dft_matrices()
    hbm = pl.BlockSpec(memory_space=pl.ANY)
    out = pl.pallas_call(
        _kernel,
        out_shape=jax.ShapeDtypeStruct((S, DM), BF16),
        in_specs=[hbm] * 14,
        out_specs=hbm,
        scratch_shapes=[
            pltpu.VMEM((S, DM), BF16),
            pltpu.VMEM((NC, S, T), BF16),
            pltpu.VMEM((NC, S, T), BF16),
            pltpu.VMEM((DM, S), BF16),
            pltpu.VMEM((S, DC), BF16),
            pltpu.VMEM((NP, DM, DH), U32),
            pltpu.VMEM((2 * NP, DC, DH), U32),
            pltpu.VMEM((NC, H * DH, T), BF16),
            pltpu.VMEM((7, S // 4, DC // 2), U32),
            pltpu.VMEM((7, S // 4, DM // 2), U32),
            pltpu.VMEM((S, T), F32),
            pltpu.VMEM((NP, 2 * S, DH), U32),
            pltpu.VMEM((NB, 2 * T, T), F32),
            pltpu.VMEM((NB, 2 * T, T), F32),
            pltpu.VMEM((NC // 2, S, T), F32),
            pltpu.VMEM((NC, S, T), BF16),
            pltpu.VMEM((2 * T, T), BF16),
            pltpu.VMEM((T, 2 * T), BF16),
            pltpu.VMEM((KS, DM), BF16),
            pltpu.VMEM((DM,), BF16),
            pltpu.VMEM((DM,), BF16),
            pltpu.SemaphoreType.DMA((NB // 2 + 14,)),
            pltpu.SemaphoreType.DMA((3 * NC // 2,)),
        ],
        compiler_params=pltpu.CompilerParams(vmem_limit_bytes=124 * 2**20),
    )(
        A_q.reshape(S, DM), A_k.reshape(S, DM), A_v.reshape(S, DM), A_shift_k.T,
        A_ssm_k, A_ssm_D, B_c_kv.reshape(S, DC), B_w_q, B_w_uk, B_w_uv,
        B_w_o.reshape(H * DH, DM), gate_w, fwd, inv,
    )
    return out.reshape(1, S, DM)
```

```python
import functools

import jax
import jax.numpy as jnp
import numpy as np
from jax import lax
import jax.experimental.pallas as pl
import jax.experimental.pallas.tpu as pltpu

S = 2048
DM = 1024
H = 32
DH = 128
DC = 512
KS = 4
T = 128
W = T // 2
NB = S // T
NP = H // 2
NC = DM // T
LEAD = 6

F32 = jnp.float32
BF16 = jnp.bfloat16
U32 = jnp.uint32
NT = (((1,), (1,)), ((), ()))
LOG2E = float(np.log2(np.e))


def _dft_matrices():
    ks = np.concatenate([np.arange(0, T, 2), np.arange(1, T, 2)]).reshape(NB, 8)
    omega = 2.0 * np.pi * (ks[:, :, None] + 0.5) / (2 * T)

    def forward(n):
        return np.concatenate([np.cos(omega * n), -np.sin(omega * n)], axis=1).reshape(2 * T, T)

    theta = (omega * (np.arange(W) + 0.5)).reshape(T, W).T
    inverse = np.concatenate([np.cos(theta), np.sin(theta)], axis=0) / T
    n = np.arange(T)
    return np.concatenate([forward(n), forward(n - (T - 1) / 2), inverse], axis=0).astype(BF16)


def _reverse_rows(v):
    row = lax.broadcasted_iota(jnp.int32, (8, T), 0)
    out = []
    for r0 in range(v.shape[0] - 8, -8, -8):
        part = pltpu.roll(v[r0:r0 + 8], 4, 0)
        for bit in (2, 1):
            part = jnp.where((row & bit) != 0, pltpu.roll(part, bit, 0),
                             pltpu.roll(part, 8 - bit, 0))
        out.append(part)
    return jnp.concatenate(out, axis=0)


def _mm(a, b):
    return jnp.dot(a, b, preferred_element_type=F32)


def _pack(v):
    return pltpu.pack_elementwise([v[:W], v[W:]], packed_dtype=BF16)


def _unpack(words):
    return pltpu.bitcast(words, BF16)


def _halves(words):
    return [pltpu.unpack_elementwise(words, index=i, packed_dtype=BF16, unpacked_dtype=F32)
            for i in range(2)]


def _zero(i):
    return lax.shift_right_logical(i, 8)


def _zero_after(values, i):
    bits = functools.reduce(jnp.bitwise_or, [pltpu.bitcast(v, U32) for v in values])
    return bits & jnp.full(bits.shape, _zero(i), jnp.int32).astype(U32)


def _left(a11, a12, a21, a22):
    return [a11 + a22, a21 + a22, a11, a22, a11 + a12, a21 - a11, a12 - a22]


def _right(b):
    return [b(0, 0, 0) + b(0, 1, 1), b(1, 0, 0), b(2, 0, 1) - b(2, 1, 1),
            b(3, 1, 0) - b(3, 0, 0), b(4, 1, 1), b(5, 0, 0) + b(5, 0, 1),
            b(6, 1, 0) + b(6, 1, 1)]


def _combine(m):
    return (m[0] + m[3] - m[4] + m[6], m[2] + m[4], m[1] + m[3], m[0] - m[1] + m[2] + m[5])


def _pair_weights(words):
    half = words.shape[0] // 2
    heads = _halves(words)
    return [v.astype(BF16)
            for v in _right(lambda i, r, c: heads[c][r * half:(r + 1) * half])]


def _store_left(src_ref, cols, dst_ref, e, r0, r1):
    half = src_ref.shape[1] // 2
    parts = []
    for j in range(2):
        rows = pl.ds(pl.multiple_of((2 * e + j) * T + r0, 32), r1 - r0)
        for c0 in (0, half):
            v = src_ref[rows, c0 + cols.start:c0 + cols.stop]
            parts.append(_halves(pltpu.bitcast(v, U32)))
    stored = []
    for odd in range(2):
        rows = pl.ds(pl.multiple_of(e * W + odd * (W // 2) + r0 // 4, 8), (r1 - r0) // 4)
        for i, v in enumerate(_left(*[part[odd] for part in parts])):
            stored.append(pltpu.bitcast(v.astype(BF16), U32))
            dst_ref[i, rows, cols] = stored[-1]
    return stored


def _project_kv(t, order, cs_ref, wkv_ref, kv_ref, meanwhile):
    base = pl.multiple_of((t >> 2) * S, S)
    w = [_pair_weights(wkv_ref[t * 4 + b]) for b in range(4)]
    for b, quarter in order:
        e = 2 * quarter
        zero = meanwhile(b, quarter)
        left = [cs_ref[i, e * W:(e + 2) * W, :] for i in range(7)]
        if zero is not None:
            left[2] = jnp.concatenate(
                [left[2][:8] | jnp.concatenate([zero, zero], axis=1), left[2][8:]], axis=0)
        c = _combine([_mm(_unpack(left[i]), w[b][i]) for i in range(7)])
        for k in range(2):
            for odd in range(2):
                for head in range(2):
                    r0 = head * (S // 2) + (2 * (e + k) + odd) * W
                    kv_ref[(t & 3) * 4 + b, pl.ds(base + r0, W), :] = _pack(
                        c[2 * odd + head][k * T:(k + 1) * T])


def _operand_row(e, i):
    return (i // 2) * (S // 2) + (2 * e + i % 2) * W


def _attend_pair(p, xs_ref, wq_ref, kv_ref):
    row = lax.broadcasted_iota(jnp.int32, (T, T), 0)
    col = lax.broadcasted_iota(jnp.int32, (T, T), 1)
    causal = col <= jnp.where(row < W, 2 * row, 2 * (row - W) + 1)
    w = _pair_weights(wq_ref[p])
    q, s, ctx = {}, {}, {}

    def blocks(region, n):
        r0 = region * (S // 2)
        return _unpack(kv_ref[p, r0:r0 + n * W, :])

    def queries(e):
        c = _combine([_mm(_unpack(xs_ref[i, e * W:(e + 1) * W, :]), w[i]) for i in range(7)])
        for odd in range(2):
            for head in range(2):
                q[2 * e + odd, head] = (c[2 * odd + head] * (DH ** -0.5 * LOG2E)).astype(BF16)

    def scores(r, head):
        d = lax.dot_general(q.pop((r, head)), blocks(head, r + 1), NT,
                            preferred_element_type=F32)
        tiles = [d[:, j * T:(j + 1) * T] for j in range(r + 1)]
        tiles[r] = jnp.where(causal, tiles[r], -1e9 * LOG2E)
        top = jnp.max(functools.reduce(jnp.maximum, tiles), axis=1, keepdims=True)
        s[r, head] = tiles, top

    def context(r, head):
        tiles, top = s.pop((r, head))
        top = jnp.broadcast_to(top, (T, T))
        tiles = [jnp.exp2(v - top) for v in tiles]
        total = tiles[0]
        for j in range(1, r + 1):
            total = total + tiles[j]
            tiles[j] = jnp.minimum(tiles[j], total)
        o = _mm(jnp.concatenate(tiles, axis=1).astype(BF16), blocks(2 + head, r + 1))
        total = jnp.sum(total, axis=1, keepdims=True)
        inv = pltpu.reciprocal(total, approx=True)
        inv = inv * (2.0 - total * inv)
        ctx[r, head] = o * inv

    def emit(e):
        ops = _left(*[ctx.pop((2 * e + odd, head)) for odd in range(2) for head in range(2)])
        for i in range(7):
            r0 = _operand_row(e, i)
            kv_ref[p, r0:r0 + W, :] = _pack(ops[i])

    order = [(r, head) for r in range(NB - 1, -1, -1) for head in range(2)]
    scored, lead = 0, 0
    for r, head in order:
        while scored < len(order) and lead < LEAD + r + 1:
            if order[scored] not in q:
                queries(order[scored][0] // 2)
            scores(*order[scored])
            lead += order[scored][0] + 1
            scored += 1
        context(r, head)
        lead -= r + 1
        if head == 1 and r % 2 == 0:
            emit(r // 2)


def _mix_step(c, half, kv_ref, wo_ref, x_ref, ak_ref, av_ref, hk_ref, shift_ref, skip_ref,
              gate_ref, dft_ref, uf_ref, hf_ref, held_ref, out_ref):
    tile = 2 * c + half
    own = pl.ds(pl.multiple_of(tile * T, T), T)
    fwd, fwd_mid = dft_ref[0:2 * T, :], dft_ref[2 * T:4 * T, :]
    cos, sin = dft_ref[4 * T:4 * T + W, :], dft_ref[4 * T + W:, :]
    skip = skip_ref[pl.ds(pl.multiple_of(c * 2 * T, 2 * T), 2 * T)]
    skip = skip.astype(F32).reshape(1, 2 * T)[:, half * T:(half + 1) * T]

    taps = shift_ref[:, own].astype(F32)
    keys = ak_ref[tile].astype(F32)
    shifted = keys * taps[KS - 1:KS]
    for t in range(KS - 2, -1, -1):
        shifted = jnp.concatenate([jnp.zeros((1, T), F32), shifted[:-1]], axis=0)
        shifted = shifted + keys * taps[t:t + 1]

    def heads(i, odd, n):
        at = 2 * c + n + _zero(c >> i)
        return jnp.concatenate([wo_ref[at, h * DH:(h + 1) * DH, :].astype(F32)
                                for h in range(odd, H, 2)], axis=0)

    w = [v.astype(BF16) for v in _right(heads)]
    plain, u, z, parts, due = [], {}, {}, {}, {}

    def deliver(j, n, v):
        blk = slice(j * T, (j + 1) * T)
        if n == half and j // 8 == half:
            if (j, n) not in parts:
                parts[j, n] = v
                return
            v = v + parts.pop((j, n))
        elif half == 0:
            held_ref[c, blk, :] = v
            return
        else:
            v = v + held_ref[c, blk, :]
        out_ref[2 * c + n, blk, :] = v.astype(BF16)

    def spectra(j):
        blk = slice(j * T, (j + 1) * T)
        cur = lax.dot_general(fwd_mid, hk_ref[own, blk], NT, preferred_element_type=F32)
        for f in range(NB):
            re, im = slice(16 * f, 16 * f + 8), slice(16 * f + 8, 16 * f + 16)
            if j == 0:
                hr, hi = cur[re], cur[im]
            elif f < NB // 2:
                hr, hi = cur[re] - plain[-1][im], cur[im] + plain[-1][re]
            else:
                hr, hi = cur[re] + plain[-1][im], cur[im] - plain[-1][re]
            hf_ref[j, re, :] = hr
            hf_ref[j, im, :] = hi
        plain.append(cur)
        u[j] = (shifted[blk] * av_ref[tile, blk, :].astype(F32)).astype(BF16)
        uf_ref[j] = _mm(fwd, u[j])

    def multiply(i0, start, step):
        base = _zero(c >> i0)
        rows = {i0: [], i0 + 1: []}
        for f in range(NB):
            re, im = slice(16 * f, 16 * f + 8), slice(16 * f + 8, 16 * f + 16)
            acc = {}
            for j in range(i0 + 2):
                ur, ui = uf_ref[base + j, re, :], uf_ref[base + j, im, :]
                for i in range(max(i0, j), i0 + 2):
                    hr, hi = hf_ref[i - j, re, :], hf_ref[i - j, im, :]
                    pr, pi = ur * hr - ui * hi, ur * hi + ui * hr
                    acc[i] = (pr, pi) if j == 0 else (acc[i][0] + pr, acc[i][1] + pi)
            for i in rows:
                rows[i].append(acc[i])
            due[int(start + f * step)] = _zero_after(acc[i0] + acc[i0 + 1], c)
        for i in rows:
            z[i] = [jnp.concatenate(part, axis=0).astype(BF16) for part in zip(*rows[i])]

    def convolved(i):
        blk = slice(i * T, (i + 1) * T)
        re, im = z.pop(i)
        even, odd = _mm(cos, re), _mm(sin, im)
        y = jnp.concatenate([_reverse_rows(even + odd), even - odd], axis=0)
        y = y + u.pop(i).astype(F32) * skip
        deliver(i, half, gate_ref[blk, :] * (x_ref[blk, own].astype(F32) * y))

    def product(e, i):
        r0 = _operand_row(e, i)
        left = [kv_ref[p, r0:r0 + W, :] for p in range(NP)]
        for p in range(0, NP, 4):
            at = 32 * i + 2 * p
            if any(at + k in due for k in range(8)):
                rows = [left[p][8 * k:8 * k + 8] for k in range(8)]
                left[p] = jnp.concatenate(
                    [v | due.pop(at + k) if at + k in due else v for k, v in enumerate(rows)],
                    axis=0)
        return _mm(_unpack(jnp.concatenate(left, axis=1)), w[i])

    groups = [(0, 2), (4, 14), (6, 12), (8, 10)] if half == 0 else [
        (0, 2), (8, 10), (12, 6), (14, 4)]
    for j in range(4):
        spectra(j)
    for step, pair in enumerate(groups):
        e = 4 * half + step
        pace = ((64, 3), (130, 4)) if step == 0 else ((4, 7.5), (130, 5.8))
        m = []
        for k, i0 in enumerate(pair):
            multiply(i0, *pace[k])
            for _ in range(4 - k):
                m.append(product(e, len(m)))
                for j in range(len(plain), min(len(plain) + 2, NB)):
                    spectra(j)
            convolved(i0)
            convolved(i0 + 1)
        b = _combine(m)
        for odd in range(2):
            j = 2 * e + odd
            for n in range(2):
                deliver(j, n, (1.0 - gate_ref[j * T:(j + 1) * T, :]) * b[2 * odd + n])


def _kernel(x_hbm, ak_hbm, av_hbm, shift_hbm, hk_hbm, skip_hbm, c_hbm, wq_hbm, wuk_hbm,
            wuv_hbm, wo_hbm, gw_hbm, dft_hbm, out_hbm,
            x_ref, ak_ref, av_ref, hk_ref, c_ref, wq_ref, wkv_ref, wo_ref, cs_ref, xs_ref,
            gate_ref, kv_ref, uf_ref, hf_ref, held_ref, out_ref, dft_ref, shift_ref,
            skip_ref, gw_ref, in_sem, out_sem):
    steps = NB // 2
    wq_sem = in_sem.at[steps]
    first, rest = pl.ds(0, 2 * T), pl.ds(2 * T, S - 2 * T)
    upper, lower = pl.ds(0, S // 2), pl.ds(S // 2, S // 2)
    whole = [(c_hbm.at[upper], c_ref.at[upper]), (c_hbm.at[lower], c_ref.at[lower]),
             (gw_hbm, gw_ref), (x_hbm.at[first], x_ref.at[first]),
             (x_hbm.at[rest], x_ref.at[rest]), (hk_hbm, hk_ref), (shift_hbm, shift_ref),
             (skip_hbm, skip_ref), (dft_hbm, dft_ref)]
    c_upper, c_lower, gw_copy, x_first, x_rest, *late = [
        pltpu.make_async_copy(src, dst, in_sem.at[steps + 1 + k])
        for k, (src, dst) in enumerate(whole)]
    tiled = [(src, dst, in_sem.at[steps + 1 + len(whole) + k])
             for k, (src, dst) in enumerate(
                 [(wo_hbm, wo_ref), (ak_hbm, ak_ref), (av_hbm, av_ref)])]

    def pair_copy(w_hbm, p, dst, sem):
        return pltpu.make_async_copy(w_hbm.bitcast(U32).at[:, p, :], dst, sem)

    def wait_filled(buf, sem):
        pltpu.make_async_copy(buf, buf, sem).wait()

    def fetch_group(t):
        for b in range(4):
            pair_copy(wuk_hbm if t < 4 else wuv_hbm, (t % 4) * 4 + b,
                      wkv_ref.at[t * 4 + b], in_sem.at[t]).start()

    def fetch_ahead(t):
        fetch_group(t + 1)
        if 1 <= t <= 4:
            for p in range(4 * t - 4, 4 * t):
                pair_copy(wq_hbm, p, wq_ref.at[p], wq_sem).start()

    def out_copy(c, part):
        rows, n = ((pl.ds(0, S // 2), 0), (pl.ds(S // 2, S // 2), 0), (pl.ds(0, S), 1))[part]
        return pltpu.make_async_copy(
            out_ref.at[2 * c + n, rows], out_hbm.at[rows, pl.ds((2 * c + n) * T, T)],
            out_sem.at[3 * c + part])

    def prepare_x(t, b, k):
        done = _store_left(x_ref, slice(b * T, (b + 1) * T), xs_ref, t, 32 * k, 32 * k + 32)
        rows = pl.ds(pl.multiple_of(t * 2 * T + (4 * b + k) * 16, 16), 16)
        gw = gw_ref[...].astype(F32).reshape(1, DM)
        logit = jnp.sum(x_ref[rows, :].astype(F32) * gw, axis=1, keepdims=True)
        g = jnp.broadcast_to(1.0 / (1.0 + jnp.exp(-logit)), (16, T))
        gate_ref[rows, :] = g
        return _zero_after(done + [g[:8], g[8:]], t)

    def prepare_c(e0):
        for e in range(e0, e0 + steps // 2):
            _store_left(c_ref, slice(0, DC // 2), cs_ref, e, 0, T)

    def first_step(t, carry):
        def meanwhile(b, quarter):
            if (b, quarter) == (0, 1):
                c_lower.wait()
                x_first.wait()
                gw_copy.wait()
                prepare_c(steps // 2)
            if quarter >= 2:
                return prepare_x(t, b, 2 * quarter - 4) | prepare_x(t, b, 2 * quarter - 3)

        c_upper.wait()
        prepare_c(0)
        wait_filled(wkv_ref.at[pl.ds(0, 4)], in_sem.at[0])
        _project_kv(t, [(b, quarter) for quarter in range(4) for b in range(4)],
                    cs_ref, wkv_ref, kv_ref, meanwhile)
        return carry

    def kv_step(t, carry):
        for k in range(1, steps - 1):
            pl.when(t == k)(functools.partial(fetch_ahead, k))
        pl.when(t == 1)(x_rest.wait)
        wait_filled(wkv_ref.at[pl.ds(t * 4, 4)], in_sem.at[t])
        _project_kv(t, [(b, quarter) for b in range(4) for quarter in range(4)],
                    cs_ref, wkv_ref, kv_ref, functools.partial(prepare_x, t))
        return carry

    c_upper.start()
    fetch_group(0)
    c_lower.start()
    x_first.start()
    gw_copy.start()
    fetch_group(1)
    x_rest.start()
    first_step(jnp.int32(0), 0)
    lax.fori_loop(1, steps, kv_step, 0)

    for copy in late:
        copy.start()
    wait_filled(wq_ref, wq_sem)

    def pair_step(p, carry):
        @pl.when(p < NC)
        def _():
            cols = pl.ds(pl.multiple_of(p * T, T), T)
            for src, dst, sem in tiled:
                pltpu.make_async_copy(src.at[:, cols], dst.at[p], sem).start()

        _attend_pair(p, xs_ref, wq_ref, kv_ref)
        return carry

    lax.fori_loop(0, NP, pair_step, 0)

    for copy in late:
        copy.wait()
    for _, dst, sem in tiled:
        wait_filled(dst, sem)

    for half in range(2):
        def mix_step(c, carry):
            _mix_step(c, half, kv_ref, wo_ref, x_ref, ak_ref, av_ref, hk_ref, shift_ref,
                      skip_ref, gate_ref, dft_ref, uf_ref, hf_ref, held_ref, out_ref)
            for k in range(NC // 2):
                @pl.when(c == k)
                def _():
                    for part in ((0,), (1, 2))[half]:
                        out_copy(k, part).start()

            return carry

        lax.fori_loop(0, NC // 2, mix_step, 0)

    for c in range(NC // 2):
        for part in range(3):
            out_copy(c, part).wait()


@jax.jit
def pallas_gated_mix__ssm_conv_h3__compressed_kv_cla__prompt_kernel(
    A_q: jax.Array,
    A_k: jax.Array,
    A_v: jax.Array,
    A_shift_k: jax.Array,
    A_ssm_k: jax.Array,
    A_ssm_D: jax.Array,
    B_x: jax.Array,
    B_c_kv: jax.Array,
    B_w_q: jax.Array,
    B_w_uk: jax.Array,
    B_w_uv: jax.Array,
    B_w_o: jax.Array,
    gate_w: jax.Array,
):
    del B_x
    hbm = pl.BlockSpec(memory_space=pl.ANY)
    out = pl.pallas_call(
        _kernel,
        out_shape=jax.ShapeDtypeStruct((S, DM), BF16),
        in_specs=[hbm] * 13,
        out_specs=hbm,
        scratch_shapes=[
            pltpu.VMEM((S, DM), BF16),
            pltpu.VMEM((NC, S, T), BF16),
            pltpu.VMEM((NC, S, T), BF16),
            pltpu.VMEM((DM, S), BF16),
            pltpu.VMEM((S, DC), BF16),
            pltpu.VMEM((NP, DM, DH), U32),
            pltpu.VMEM((2 * NP, DC, DH), U32),
            pltpu.VMEM((NC, H * DH, T), BF16),
            pltpu.VMEM((7, S // 4, DC // 2), U32),
            pltpu.VMEM((7, S // 4, DM // 2), U32),
            pltpu.VMEM((S, T), F32),
            pltpu.VMEM((NP, 2 * S, DH), U32),
            pltpu.VMEM((NB, 2 * T, T), F32),
            pltpu.VMEM((NB, 2 * T, T), F32),
            pltpu.VMEM((NC // 2, S, T), F32),
            pltpu.VMEM((NC, S, T), BF16),
            pltpu.VMEM((5 * T, T), BF16),
            pltpu.VMEM((KS, DM), BF16),
            pltpu.VMEM((DM,), BF16),
            pltpu.VMEM((DM,), BF16),
            pltpu.SemaphoreType.DMA((NB // 2 + 13,)),
            pltpu.SemaphoreType.DMA((3 * NC // 2,)),
        ],
        compiler_params=pltpu.CompilerParams(vmem_limit_bytes=124 * 2**20),
    )(
        A_q.reshape(S, DM), A_k.reshape(S, DM), A_v.reshape(S, DM), A_shift_k.T,
        A_ssm_k, A_ssm_D, B_c_kv.reshape(S, DC), B_w_q, B_w_uk, B_w_uv,
        B_w_o.reshape(H * DH, DM), gate_w, _dft_matrices(),
    )
    return out.reshape(1, S, DM)
```

```python
import functools

import jax
import jax.numpy as jnp
import numpy as np
from jax import lax
import jax.experimental.pallas as pl
import jax.experimental.pallas.tpu as pltpu

S = 2048
DM = 1024
H = 32
DH = 128
DC = 512
KS = 4
T = 128
W = T // 2
NB = S // T
NP = H // 2
NC = DM // T
LEAD = 6

F32 = jnp.float32
BF16 = jnp.bfloat16
U32 = jnp.uint32
NT = (((1,), (1,)), ((), ()))
LOG2E = float(np.log2(np.e))


def _dft_matrices():
    ks = np.concatenate([np.arange(0, T, 2), np.arange(1, T, 2)]).reshape(NB, 8)
    omega = 2.0 * np.pi * (ks[:, :, None] + 0.5) / (2 * T)

    def forward(n):
        return np.concatenate([np.cos(omega * n), -np.sin(omega * n)], axis=1).reshape(2 * T, T)

    theta = (omega * (np.arange(W) + 0.5)).reshape(T, W).T
    inverse = np.concatenate([np.cos(theta), np.sin(theta)], axis=0) / T
    n = np.arange(T)
    return np.concatenate([forward(n), forward(n - (T - 1) / 2), inverse], axis=0).astype(BF16)


def _reverse_rows(v):
    row = lax.broadcasted_iota(jnp.int32, (8, T), 0)
    out = []
    for r0 in range(v.shape[0] - 8, -8, -8):
        part = pltpu.roll(v[r0:r0 + 8], 4, 0)
        for bit in (2, 1):
            part = jnp.where((row & bit) != 0, pltpu.roll(part, bit, 0),
                             pltpu.roll(part, 8 - bit, 0))
        out.append(part)
    return jnp.concatenate(out, axis=0)


def _mm(a, b):
    return jnp.dot(a, b, preferred_element_type=F32)


def _pack(v):
    return pltpu.pack_elementwise([v[:W], v[W:]], packed_dtype=BF16)


def _unpack(words):
    return pltpu.bitcast(words, BF16)


def _halves(words):
    return [pltpu.unpack_elementwise(words, index=i, packed_dtype=BF16, unpacked_dtype=F32)
            for i in range(2)]


def _zero(i):
    return lax.shift_right_logical(i, 8)


def _zero_after(values, i):
    bits = functools.reduce(jnp.bitwise_or, [pltpu.bitcast(v, U32) for v in values])
    return bits & jnp.full(bits.shape, _zero(i), jnp.int32).astype(U32)


def _left(a11, a12, a21, a22):
    return [a11 + a22, a21 + a22, a11, a22, a11 + a12, a21 - a11, a12 - a22]


def _right(b):
    return [b(0, 0, 0) + b(0, 1, 1), b(1, 0, 0), b(2, 0, 1) - b(2, 1, 1),
            b(3, 1, 0) - b(3, 0, 0), b(4, 1, 1), b(5, 0, 0) + b(5, 0, 1),
            b(6, 1, 0) + b(6, 1, 1)]


def _combine(m):
    return (m[0] + m[3] - m[4] + m[6], m[2] + m[4], m[1] + m[3], m[0] - m[1] + m[2] + m[5])


def _pair_weights(words):
    half = words.shape[0] // 2
    heads = _halves(words)
    return [v.astype(BF16)
            for v in _right(lambda i, r, c: heads[c][r * half:(r + 1) * half])]


def _store_left(src_ref, cols, dst_ref, e, r0, r1):
    half = src_ref.shape[1] // 2
    parts = []
    for j in range(2):
        rows = pl.ds(pl.multiple_of((2 * e + j) * T + r0, 32), r1 - r0)
        for c0 in (0, half):
            v = src_ref[rows, c0 + cols.start:c0 + cols.stop]
            parts.append(_halves(pltpu.bitcast(v, U32)))
    stored = []
    for odd in range(2):
        rows = pl.ds(pl.multiple_of(e * W + odd * (W // 2) + r0 // 4, 8), (r1 - r0) // 4)
        for i, v in enumerate(_left(*[part[odd] for part in parts])):
            stored.append(pltpu.bitcast(v.astype(BF16), U32))
            dst_ref[i, rows, cols] = stored[-1]
    return stored


def _project_kv(t, order, cs_ref, wkv_ref, kv_ref, meanwhile):
    base = pl.multiple_of((t >> 2) * S, S)
    w = [_pair_weights(wkv_ref[t * 4 + b]) for b in range(4)]
    for b, quarter in order:
        e = 2 * quarter
        zero = meanwhile(b, quarter)
        left = [cs_ref[i, e * W:(e + 2) * W, :] for i in range(7)]
        if zero is not None:
            left[2] = jnp.concatenate(
                [left[2][:8] | jnp.concatenate([zero, zero], axis=1), left[2][8:]], axis=0)
        c = _combine([_mm(_unpack(left[i]), w[b][i]) for i in range(7)])
        for k in range(2):
            for odd in range(2):
                for head in range(2):
                    r0 = head * (S // 2) + (2 * (e + k) + odd) * W
                    kv_ref[(t & 3) * 4 + b, pl.ds(base + r0, W), :] = _pack(
                        c[2 * odd + head][k * T:(k + 1) * T])


def _operand_row(e, i):
    return (i // 2) * (S // 2) + (2 * e + i % 2) * W


def _attend_pair(p, xs_ref, wq_ref, kv_ref):
    row = lax.broadcasted_iota(jnp.int32, (T, T), 0)
    col = lax.broadcasted_iota(jnp.int32, (T, T), 1)
    causal = col <= jnp.where(row < W, 2 * row, 2 * (row - W) + 1)
    w = _pair_weights(wq_ref[p])
    q, s, ctx = {}, {}, {}

    def blocks(region, n):
        r0 = region * (S // 2)
        return _unpack(kv_ref[p, r0:r0 + n * W, :])

    def queries(e):
        c = _combine([_mm(_unpack(xs_ref[i, e * W:(e + 1) * W, :]), w[i]) for i in range(7)])
        for odd in range(2):
            for head in range(2):
                q[2 * e + odd, head] = (c[2 * odd + head] * (DH ** -0.5 * LOG2E)).astype(BF16)

    def scores(r, head):
        d = lax.dot_general(q.pop((r, head)), blocks(head, r + 1), NT,
                            preferred_element_type=F32)
        tiles = [d[:, j * T:(j + 1) * T] for j in range(r + 1)]
        tiles[r] = jnp.where(causal, tiles[r], -1e9 * LOG2E)
        top = jnp.max(functools.reduce(jnp.maximum, tiles), axis=1, keepdims=True)
        s[r, head] = tiles, top

    def context(r, head):
        tiles, top = s.pop((r, head))
        top = jnp.broadcast_to(top, (T, T))
        tiles = [jnp.exp2(v - top) for v in tiles]
        total = tiles[0]
        for j in range(1, r + 1):
            total = total + tiles[j]
            tiles[j] = jnp.minimum(tiles[j], total)
        o = _mm(jnp.concatenate(tiles, axis=1).astype(BF16), blocks(2 + head, r + 1))
        total = jnp.sum(total, axis=1, keepdims=True)
        inv = pltpu.reciprocal(total, approx=True)
        inv = inv * (2.0 - total * inv)
        ctx[r, head] = o * inv

    def emit(e):
        ops = _left(*[ctx.pop((2 * e + odd, head)) for odd in range(2) for head in range(2)])
        for i in range(7):
            r0 = _operand_row(e, i)
            kv_ref[p, r0:r0 + W, :] = _pack(ops[i])

    order = [(r, head) for r in range(NB - 1, -1, -1) for head in range(2)]
    scored, lead = 0, 0
    for r, head in order:
        while scored < len(order) and lead < LEAD + r + 1:
            if order[scored] not in q:
                queries(order[scored][0] // 2)
            scores(*order[scored])
            lead += order[scored][0] + 1
            scored += 1
        context(r, head)
        lead -= r + 1
        if head == 1 and r % 2 == 0:
            emit(r // 2)


def _mix_step(c, half, kv_ref, wo_ref, x_ref, ak_ref, av_ref, hk_ref, shift_ref, skip_ref,
              gate_ref, dft_ref, uf_ref, hf_ref, held_ref, out_ref):
    tile = 2 * c + half
    own = pl.ds(pl.multiple_of(tile * T, T), T)
    fwd, fwd_mid = dft_ref[0:2 * T, :], dft_ref[2 * T:4 * T, :]
    cos, sin = dft_ref[4 * T:4 * T + W, :], dft_ref[4 * T + W:, :]
    skip = skip_ref[pl.ds(pl.multiple_of(c * 2 * T, 2 * T), 2 * T)]
    skip = skip.astype(F32).reshape(1, 2 * T)[:, half * T:(half + 1) * T]

    taps = shift_ref[:, own].astype(F32)
    keys = ak_ref[tile].astype(F32)
    shifted = keys * taps[KS - 1:KS]
    for t in range(KS - 2, -1, -1):
        shifted = jnp.concatenate([jnp.zeros((1, T), F32), shifted[:-1]], axis=0)
        shifted = shifted + keys * taps[t:t + 1]

    def heads(i, odd, n):
        at = 2 * c + n + _zero(c >> i)
        return jnp.concatenate([wo_ref[at, h * DH:(h + 1) * DH, :].astype(F32)
                                for h in range(odd, H, 2)], axis=0)

    w = [v.astype(BF16) for v in _right(heads)]
    plain, u, z, parts, due = [], {}, {}, {}, {}

    def deliver(j, n, v):
        blk = slice(j * T, (j + 1) * T)
        if n == half and j // 8 == half:
            if (j, n) not in parts:
                parts[j, n] = v
                return
            v = v + parts.pop((j, n))
        elif half == 0:
            held_ref[c, blk, :] = v
            return
        else:
            v = v + held_ref[c, blk, :]
        out_ref[2 * c + n, blk, :] = v.astype(BF16)

    def spectra(j):
        blk = slice(j * T, (j + 1) * T)
        cur = lax.dot_general(fwd_mid, hk_ref[own, blk], NT, preferred_element_type=F32)
        for f in range(NB):
            re, im = slice(16 * f, 16 * f + 8), slice(16 * f + 8, 16 * f + 16)
            if j == 0:
                hr, hi = cur[re], cur[im]
            elif f < NB // 2:
                hr, hi = cur[re] - plain[-1][im], cur[im] + plain[-1][re]
            else:
                hr, hi = cur[re] + plain[-1][im], cur[im] - plain[-1][re]
            hf_ref[j, re, :] = hr
            hf_ref[j, im, :] = hi
        plain.append(cur)
        u[j] = (shifted[blk] * av_ref[tile, blk, :].astype(F32)).astype(BF16)
        uf_ref[j] = _mm(fwd, u[j])

    def multiply(i0, start, step):
        base = _zero(c >> i0)
        rows = {i0: [], i0 + 1: []}
        for f in range(NB):
            re, im = slice(16 * f, 16 * f + 8), slice(16 * f + 8, 16 * f + 16)
            acc = {}
            for j in range(i0 + 2):
                ur, ui = uf_ref[base + j, re, :], uf_ref[base + j, im, :]
                for i in range(max(i0, j), i0 + 2):
                    hr, hi = hf_ref[base + i - j, re, :], hf_ref[base + i - j, im, :]
                    pr, pi = ur * hr - ui * hi, ur * hi + ui * hr
                    acc[i] = (pr, pi) if j == 0 else (acc[i][0] + pr, acc[i][1] + pi)
            for i in rows:
                rows[i].append(acc[i])
            due[int(start + f * step)] = _zero_after(acc[i0] + acc[i0 + 1], c)
        for i in rows:
            z[i] = [jnp.concatenate(part, axis=0).astype(BF16) for part in zip(*rows[i])]

    def convolved(i):
        blk = slice(i * T, (i + 1) * T)
        re, im = z.pop(i)
        even, odd = _mm(cos, re), _mm(sin, im)
        y = jnp.concatenate([_reverse_rows(even + odd), even - odd], axis=0)
        y = y + u.pop(i).astype(F32) * skip
        deliver(i, half, gate_ref[blk, :] * (x_ref[blk, own].astype(F32) * y))

    def product(e, i):
        r0 = _operand_row(e, i)
        left = [kv_ref[p, r0:r0 + W, :] for p in range(NP)]
        for p in range(0, NP, 4):
            at = 32 * i + 2 * p
            if any(at + k in due for k in range(8)):
                rows = [left[p][8 * k:8 * k + 8] for k in range(8)]
                left[p] = jnp.concatenate(
                    [v | due.pop(at + k) if at + k in due else v for k, v in enumerate(rows)],
                    axis=0)
        return _mm(_unpack(jnp.concatenate(left, axis=1)), w[i])

    for j in range(NB):
        spectra(j)
    for step in range(4):
        e = 4 * half + step
        pace = ((50, 4.5), (135, 5.5)) if step == 0 else ((4, 7.5), (130, 5.8))
        m = []
        for k, i0 in enumerate((2 * e, NB - 2 - 2 * e)):
            multiply(i0, *pace[k])
            for _ in range(4 - k):
                m.append(product(e, len(m)))
            convolved(i0)
            convolved(i0 + 1)
        b = _combine(m)
        for odd in range(2):
            j = 2 * e + odd
            for n in range(2):
                deliver(j, n, (1.0 - gate_ref[j * T:(j + 1) * T, :]) * b[2 * odd + n])


def _kernel(x_hbm, ak_hbm, av_hbm, shift_hbm, hk_hbm, skip_hbm, c_hbm, wq_hbm, wuk_hbm,
            wuv_hbm, wo_hbm, gw_hbm, dft_hbm, out_hbm,
            x_ref, ak_ref, av_ref, hk_ref, c_ref, wq_ref, wkv_ref, wo_ref, cs_ref, xs_ref,
            gate_ref, kv_ref, uf_ref, hf_ref, held_ref, out_ref, dft_ref, shift_ref,
            skip_ref, gw_ref, in_sem, out_sem):
    steps = NB // 2
    wq_sem = in_sem.at[steps]
    first, rest = pl.ds(0, 2 * T), pl.ds(2 * T, S - 2 * T)
    upper, lower = pl.ds(0, S // 2), pl.ds(S // 2, S // 2)
    whole = [(c_hbm.at[upper], c_ref.at[upper]), (c_hbm.at[lower], c_ref.at[lower]),
             (gw_hbm, gw_ref), (x_hbm.at[first], x_ref.at[first]),
             (x_hbm.at[rest], x_ref.at[rest]), (hk_hbm, hk_ref), (shift_hbm, shift_ref),
             (skip_hbm, skip_ref), (dft_hbm, dft_ref)]
    c_upper, c_lower, gw_copy, x_first, x_rest, *late = [
        pltpu.make_async_copy(src, dst, in_sem.at[steps + 1 + k])
        for k, (src, dst) in enumerate(whole)]
    tiled = [(src, dst, in_sem.at[steps + 1 + len(whole) + k])
             for k, (src, dst) in enumerate(
                 [(wo_hbm, wo_ref), (ak_hbm, ak_ref), (av_hbm, av_ref)])]

    def pair_copy(w_hbm, p, dst, sem):
        return pltpu.make_async_copy(w_hbm.bitcast(U32).at[:, p, :], dst, sem)

    def wait_filled(buf, sem):
        pltpu.make_async_copy(buf, buf, sem).wait()

    def fetch_group(t):
        for b in range(4):
            pair_copy(wuk_hbm if t < 4 else wuv_hbm, (t % 4) * 4 + b,
                      wkv_ref.at[t * 4 + b], in_sem.at[t]).start()

    def fetch_ahead(t):
        fetch_group(t + 1)
        if 1 <= t <= 4:
            for p in range(4 * t - 4, 4 * t):
                pair_copy(wq_hbm, p, wq_ref.at[p], wq_sem).start()

    def out_copy(c, part):
        rows, n = ((pl.ds(0, S // 2), 0), (pl.ds(S // 2, S // 2), 0), (pl.ds(0, S), 1))[part]
        return pltpu.make_async_copy(
            out_ref.at[2 * c + n, rows], out_hbm.at[rows, pl.ds((2 * c + n) * T, T)],
            out_sem.at[3 * c + part])

    def prepare_x(t, b, k):
        done = _store_left(x_ref, slice(b * T, (b + 1) * T), xs_ref, t, 32 * k, 32 * k + 32)
        rows = pl.ds(pl.multiple_of(t * 2 * T + (4 * b + k) * 16, 16), 16)
        gw = gw_ref[...].astype(F32).reshape(1, DM)
        logit = jnp.sum(x_ref[rows, :].astype(F32) * gw, axis=1, keepdims=True)
        g = jnp.broadcast_to(1.0 / (1.0 + jnp.exp(-logit)), (16, T))
        gate_ref[rows, :] = g
        return _zero_after(done + [g[:8], g[8:]], t)

    def prepare_c(e0):
        for e in range(e0, e0 + steps // 2):
            _store_left(c_ref, slice(0, DC // 2), cs_ref, e, 0, T)

    def first_step(t, carry):
        def meanwhile(b, quarter):
            if (b, quarter) == (0, 1):
                c_lower.wait()
                x_first.wait()
                gw_copy.wait()
                prepare_c(steps // 2)
            if quarter >= 2:
                return prepare_x(t, b, 2 * quarter - 4) | prepare_x(t, b, 2 * quarter - 3)

        c_upper.wait()
        prepare_c(0)
        wait_filled(wkv_ref.at[pl.ds(0, 4)], in_sem.at[0])
        _project_kv(t, [(b, quarter) for quarter in range(4) for b in range(4)],
                    cs_ref, wkv_ref, kv_ref, meanwhile)
        return carry

    def kv_step(t, carry):
        for k in range(1, steps - 1):
            pl.when(t == k)(functools.partial(fetch_ahead, k))
        pl.when(t == 1)(x_rest.wait)
        wait_filled(wkv_ref.at[pl.ds(t * 4, 4)], in_sem.at[t])
        _project_kv(t, [(b, quarter) for b in range(4) for quarter in range(4)],
                    cs_ref, wkv_ref, kv_ref, functools.partial(prepare_x, t))
        return carry

    c_upper.start()
    fetch_group(0)
    c_lower.start()
    x_first.start()
    gw_copy.start()
    fetch_group(1)
    x_rest.start()
    first_step(jnp.int32(0), 0)
    lax.fori_loop(1, steps, kv_step, 0)

    for copy in late:
        copy.start()
    wait_filled(wq_ref, wq_sem)

    def pair_step(p, carry):
        @pl.when(p < NC)
        def _():
            cols = pl.ds(pl.multiple_of(p * T, T), T)
            for src, dst, sem in tiled:
                pltpu.make_async_copy(src.at[:, cols], dst.at[p], sem).start()

        _attend_pair(p, xs_ref, wq_ref, kv_ref)
        return carry

    lax.fori_loop(0, NP, pair_step, 0)

    for copy in late:
        copy.wait()
    for _, dst, sem in tiled:
        wait_filled(dst, sem)

    for half in range(2):
        def mix_step(c, carry):
            _mix_step(c, half, kv_ref, wo_ref, x_ref, ak_ref, av_ref, hk_ref, shift_ref,
                      skip_ref, gate_ref, dft_ref, uf_ref, hf_ref, held_ref, out_ref)
            for k in range(NC // 2):
                @pl.when(c == k)
                def _():
                    for part in ((0,), (1, 2))[half]:
                        out_copy(k, part).start()

            return carry

        lax.fori_loop(0, NC // 2, mix_step, 0)

    for c in range(NC // 2):
        for part in range(3):
            out_copy(c, part).wait()


@jax.jit
def pallas_gated_mix__ssm_conv_h3__compressed_kv_cla__prompt_kernel(
    A_q: jax.Array,
    A_k: jax.Array,
    A_v: jax.Array,
    A_shift_k: jax.Array,
    A_ssm_k: jax.Array,
    A_ssm_D: jax.Array,
    B_x: jax.Array,
    B_c_kv: jax.Array,
    B_w_q: jax.Array,
    B_w_uk: jax.Array,
    B_w_uv: jax.Array,
    B_w_o: jax.Array,
    gate_w: jax.Array,
):
    del B_x
    hbm = pl.BlockSpec(memory_space=pl.ANY)
    out = pl.pallas_call(
        _kernel,
        out_shape=jax.ShapeDtypeStruct((S, DM), BF16),
        in_specs=[hbm] * 13,
        out_specs=hbm,
        scratch_shapes=[
            pltpu.VMEM((S, DM), BF16),
            pltpu.VMEM((NC, S, T), BF16),
            pltpu.VMEM((NC, S, T), BF16),
            pltpu.VMEM((DM, S), BF16),
            pltpu.VMEM((S, DC), BF16),
            pltpu.VMEM((NP, DM, DH), U32),
            pltpu.VMEM((2 * NP, DC, DH), U32),
            pltpu.VMEM((NC, H * DH, T), BF16),
            pltpu.VMEM((7, S // 4, DC // 2), U32),
            pltpu.VMEM((7, S // 4, DM // 2), U32),
            pltpu.VMEM((S, T), F32),
            pltpu.VMEM((NP, 2 * S, DH), U32),
            pltpu.VMEM((NB, 2 * T, T), F32),
            pltpu.VMEM((NB, 2 * T, T), F32),
            pltpu.VMEM((NC // 2, S, T), F32),
            pltpu.VMEM((NC, S, T), BF16),
            pltpu.VMEM((5 * T, T), BF16),
            pltpu.VMEM((KS, DM), BF16),
            pltpu.VMEM((DM,), BF16),
            pltpu.VMEM((DM,), BF16),
            pltpu.SemaphoreType.DMA((NB // 2 + 13,)),
            pltpu.SemaphoreType.DMA((3 * NC // 2,)),
        ],
        compiler_params=pltpu.CompilerParams(vmem_limit_bytes=124 * 2**20),
    )(
        A_q.reshape(S, DM), A_k.reshape(S, DM), A_v.reshape(S, DM), A_shift_k.T,
        A_ssm_k, A_ssm_D, B_c_kv.reshape(S, DC), B_w_q, B_w_uk, B_w_uv,
        B_w_o.reshape(H * DH, DM), gate_w, _dft_matrices(),
    )
    return out.reshape(1, S, DM)
```
